```python
import jax
import jax.numpy as jnp

def _softmax(x, axis=-1):
    return jax.nn.softmax(x, axis=axis)
def _gelu(x):
    return jax.nn.gelu(x, approximate=True)
def _silu(x):
    return jax.nn.silu(x)
def _sigmoid(x):
    return jax.nn.sigmoid(x)
def _layernorm(x, axis=-1, eps=1e-5):
    m = jnp.mean(x, axis=axis, keepdims=True)
    v = jnp.var(x, axis=axis, keepdims=True)
    return (x - m) / jnp.sqrt(v + eps)
def _scatter_add(tgt, idx, src, axis=0):
    return tgt.at[idx].add(src)
def _segment_sum(src, seg, n):
    return jax.ops.segment_sum(src, seg, n)
class _Rng:
    def __init__(self, key):
        self._k = key
    def _next(self):
        self._k, sub = jax.random.split(self._k)
        return sub
    def normal(self, shape):
        return jax.random.normal(self._next(), shape, dtype=jnp.bfloat16)
    def randint(self, lo, hi, shape):
        return jax.random.randint(self._next(), shape, lo, hi, dtype=jnp.int32)
    def uniform(self, shape, lo=0.0, hi=1.0):
        return jax.random.uniform(self._next(), shape, jnp.bfloat16, lo, hi)
    def permutation(self, n):
        return jax.random.permutation(self._next(), n)


kernel_name = 'interleave_layers__sliding_block_cached__dense_activation_gelu__decode'

def setup_inputs():
    _rng = _Rng(jax.random.key(int.from_bytes(__import__("os").urandom(4), "little")))
    _w = (lambda a: (lambda t: t.astype(jnp.bfloat16) if jnp.issubdtype(t.dtype, jnp.floating) else t)(jnp.asarray(a)))
    def _A_setup():
        B, Sq, D = 1, 1, 640
        Hq, Hkv, Sk, Dh = 32, 32, 32768, 192
        assert Hq % Hkv == 0, (Hq, Hkv)
        return {
            "x": _w((lambda *s: _rng.normal(s) * 0.05)(B, Sq, D)),
            "k_cache": _w((lambda *s: _rng.normal(s) * 0.05)(B, Hkv, Sk, Dh)),
            "v_cache": _w((lambda *s: _rng.normal(s) * 0.05)(B, Hkv, Sk, Dh)),
            "wq": _w((lambda *s: _rng.normal(s) * 0.05)(D, Hq * Dh) * (D ** -0.5)),
            "wo": _w((lambda *s: _rng.normal(s) * 0.05)(Hq * Dh, D) * ((Hq * Dh) ** -0.5)),
        }
    _A_in = _A_setup()

    def _B_setup():
        B, S, D, F = 1, 1, 640, 1536
        return {
            "x": _w((lambda *s: _rng.normal(s) * 0.05)(B, S, D)),
            "w1": _w((lambda *s: _rng.normal(s) * 0.05)(D, F) * (D ** -0.5)),
            "b1": _w((lambda *s: _rng.normal(s) * 0.05)(F) * 0.01),
            "w2": _w((lambda *s: _rng.normal(s) * 0.05)(F, D) * (F ** -0.5)),
            "b2": _w((lambda *s: _rng.normal(s) * 0.05)(D) * 0.01),
        }
    _B_in = _B_setup()

    return {
        "A_x": _A_in["x"],
        "A_k_cache": _A_in["k_cache"],
        "A_v_cache": _A_in["v_cache"],
        "A_wq": _A_in["wq"],
        "A_wo": _A_in["wo"],
        "B_x": _B_in["x"],
        "B_w1": _B_in["w1"],
        "B_b1": _B_in["b1"],
        "B_w2": _B_in["w2"],
        "B_b2": _B_in["b2"],
    }

def reference(A_x, A_k_cache, A_v_cache, A_wq, A_wo, B_x, B_w1, B_b1, B_w2, B_b2):
    def _A_ref(x, k_cache, v_cache, wq, wo):
        B, Sq, D = x.shape
        Hq, Dh = 32, 192
        Hkv, Sk = k_cache.shape[1], k_cache.shape[2]
        W = min(4096, max(256, Sk // 4))
        rep = Hq // Hkv
        q = (lambda x, *d: x.transpose(*d))((x @ wq).reshape(B, Sq, Hq, Dh), 0, 2, 1, 3)
        k = jnp.repeat(k_cache[:, :, Sk - W:, :], rep, axis=1)
        v = jnp.repeat(v_cache[:, :, Sk - W:, :], rep, axis=1)
        scores = jnp.einsum("bhqd,bhkd->bhqk", q, k) * (Dh ** -0.5)
        p = _softmax(scores, axis=-1)
        o = jnp.einsum("bhqk,bhkd->bhqd", p, v)
        return (lambda x, *d: x.transpose(*d))(o, 0, 2, 1, 3).reshape(B, Sq, Hq * Dh) @ wo

    def _B_ref(x, w1, b1, w2, b2):
        h = jnp.einsum("bsd,df->bsf", x, w1) + b1
        h = _gelu(h)
        return jnp.einsum("bsf,fd->bsd", h, w2) + b2

    x = A_x
    x = x + _A_ref(_layernorm(x, axis=-1), A_k_cache, A_v_cache, A_wq, A_wo)
    x = x + _B_ref(_layernorm(x, axis=-1), B_w1, B_b1, B_w2, B_b2)
    x = x + _A_ref(_layernorm(x, axis=-1), A_k_cache, A_v_cache, A_wq, A_wo)
    x = x + _B_ref(_layernorm(x, axis=-1), B_w1, B_b1, B_w2, B_b2)
    return x
```

```python
import math

import jax
import jax.numpy as jnp
from jax import lax
import jax.experimental.pallas as pl
import jax.experimental.pallas.tpu as pltpu

F32 = jnp.float32
BF16 = jnp.bfloat16
U32 = jnp.uint32

LANES = 128
ROWS = 8


def _layernorm(x, eps=1e-5):
    m = jnp.mean(x, axis=-1, keepdims=True)
    c = x - m
    v = jnp.mean(c * c, axis=-1, keepdims=True)
    return c / jnp.sqrt(v + eps)


def _round_bf16(x):
    return x.astype(BF16).astype(F32)


def _gelu_tanh(x):
    c = math.sqrt(2.0 / math.pi)
    return 0.5 * x * (1.0 + jnp.tanh(c * (x + 0.044715 * (x * x * x))))


@jax.jit
def pallas_interleave_layers__sliding_block_cached__dense_activation_gelu__decode_kernel(
    A_x: jax.Array,
    A_k_cache: jax.Array,
    A_v_cache: jax.Array,
    A_wq: jax.Array,
    A_wo: jax.Array,
    B_x: jax.Array,
    B_w1: jax.Array,
    B_b1: jax.Array,
    B_w2: jax.Array,
    B_b2: jax.Array,
):
    B, SQ, D = A_x.shape
    _, H, SK, DH = A_k_cache.shape
    FF = B_w1.shape[1]
    assert B == 1 and SQ == 1 and A_wq.shape[1] == H * DH and H % 4 == 0
    W = min(4096, max(256, SK // 4))
    NP = H // 2
    PD = 2 * DH
    HW = DH // 2
    NT = W // LANES
    NG = NP // 2
    W2C = 4
    FC = FF // W2C
    NRING = 3
    exp_scale = float(DH) ** -0.5

    kt = jnp.transpose(A_k_cache, (0, 1, 3, 2)).reshape(NP, PD, SK)
    vt = jnp.transpose(A_v_cache, (0, 1, 3, 2)).reshape(NP, PD, SK)
    wo3 = A_wo.reshape(NP, PD, D)

    def kernel(x_hbm, k_hbm, v_hbm, wq_hbm, wo_hbm, w1_hbm, b1_hbm, w2_hbm, b2_hbm,
               o_ref,
               kbuf, vbuf, wqbuf, wobuf, w1buf, w2buf, xbuf, b1buf, b2buf,
               p0, p1, a0, a1, linv, sems):
        kb = kbuf.bitcast(BF16)
        vb = vbuf.bitcast(BF16)
        wqb = wqbuf.bitcast(BF16)
        wob = wobuf.bitcast(BF16)
        w1b = w1buf.bitcast(BF16)
        w2b = w2buf.bitcast(BF16)
        pbuf = (p0, p1)
        abuf = (a0, a1)

        S_SMALL, S_WQ, S_K0, S_WO, S_W1, S_W2 = 0, 1, 2, 3, 4, 5
        S_RING = S_W2 + W2C

        def k_copy(start, n, sem):
            return pltpu.make_async_copy(
                k_hbm.at[pl.ds(start, n), :, pl.ds(SK - W, W)], kb.at[pl.ds(start, n)], sem)

        def v_copy(start, n, sem):
            return pltpu.make_async_copy(
                v_hbm.at[pl.ds(start, n), :, pl.ds(SK - W, W)], vb.at[pl.ds(start, n)], sem)

        def group_copies(g, last):
            sem = sems.at[S_RING + g % NRING]
            return [k_copy(2 * g + 1, 1 if last else 2, sem), v_copy(2 * g, 2, sem)]

        small = [pltpu.make_async_copy(x_hbm, xbuf, sems.at[S_SMALL]),
                 pltpu.make_async_copy(b1_hbm, b1buf, sems.at[S_SMALL]),
                 pltpu.make_async_copy(b2_hbm, b2buf, sems.at[S_SMALL])]
        wq_cp = pltpu.make_async_copy(wq_hbm, wqb, sems.at[S_WQ])
        k0_cp = k_copy(0, 1, sems.at[S_K0])
        wo_cp = pltpu.make_async_copy(wo_hbm, wob, sems.at[S_WO])
        w1_cp = pltpu.make_async_copy(w1_hbm, w1b, sems.at[S_W1])
        w2_cps = [pltpu.make_async_copy(w2_hbm.at[pl.ds(c * FC, FC)], w2b.at[pl.ds(c * FC, FC)],
                                        sems.at[S_W2 + c]) for c in range(W2C)]

        wq_cp.start()
        for cp in small:
            cp.start()
        k0_cp.start()
        wo_cp.start()
        for g in range(NRING):
            for cp in group_copies(g, False):
                cp.start()

        row = lax.broadcasted_iota(jnp.int32, (ROWS, PD), 0)
        col = lax.broadcasted_iota(jnp.int32, (ROWS, PD), 1)
        first_head = col < DH
        diag = jnp.where(first_head, 0, 1) == row

        def q_proj(xn, i):
            off = pl.multiple_of(i * PD, LANES)
            q = jnp.dot(xn, wqb[:, pl.ds(off, PD)], preferred_element_type=F32)
            return jnp.where(diag, q, 0.0).astype(BF16)

        def scores(q, i, slot):
            s = jnp.dot(q, kb[i], preferred_element_type=F32)
            m = jnp.max(s, axis=1, keepdims=True)
            e = jnp.exp((s - m) * exp_scale)
            pbuf[slot][...] = e
            l = jnp.sum(e, axis=1, keepdims=True)
            linv[i] = jnp.broadcast_to(1.0 / l, (ROWS, LANES))

        def pv(i, slot):
            for j in range(2):
                lo_acc = hi_acc = None
                for t in range(NT):
                    pb = pbuf[slot][j:j + 1, t * LANES:(t + 1) * LANES]
                    u = vbuf[i, j * HW:(j + 1) * HW, t * LANES:(t + 1) * LANES]
                    lo = pltpu.bitcast(u << 16, F32) * pb
                    hi = pltpu.bitcast(u & U32(0xFFFF0000), F32) * pb
                    lo_acc = lo if lo_acc is None else lo_acc + lo
                    hi_acc = hi if hi_acc is None else hi_acc + hi
                abuf[slot][pl.ds(j * DH, HW, stride=2), :] = lo_acc
                abuf[slot][pl.ds(j * DH + 1, HW, stride=2), :] = hi_acc

        def o_proj(i, slot):
            o = jnp.sum(abuf[slot][...].T, axis=0, keepdims=True)
            inv = linv[i]
            reps = PD // LANES
            inv0 = jnp.concatenate([inv[0:1]] * reps, axis=1)
            inv1 = jnp.concatenate([inv[1:2]] * reps, axis=1)
            o = o * jnp.where(first_head[0:1], inv0, inv1)
            ob = jnp.broadcast_to(o, (ROWS, PD)).astype(BF16)
            return jnp.dot(ob, wob[i], preferred_element_type=F32)

        def attention(x, first):
            xn = _layernorm(x).astype(BF16)
            if first:
                wq_cp.wait()
            q0 = q_proj(xn, 0)
            q1 = q_proj(xn, 1)
            if first:
                k0_cp.wait()
            scores(q0, 0, 0)
            a1[...] = jnp.zeros(a1.shape, F32)
            if first:
                wo_cp.wait()

            def body(g, carry):
                q_odd, acc = carry
                if first:
                    @pl.when(g < NG - 1)
                    def _():
                        for cp in group_copies(g, False):
                            cp.wait()

                    @pl.when(g == NG - 1)
                    def _():
                        for cp in group_copies(NG - 1, True):
                            cp.wait()

                    @pl.when(g + NRING < NG - 1)
                    def _():
                        for cp in group_copies(g + NRING, False):
                            cp.start()

                    @pl.when(g + NRING == NG - 1)
                    def _():
                        for cp in group_copies(NG - 1, True):
                            cp.start()
                        w1_cp.start()
                        for cp in w2_cps:
                            cp.start()

                i0 = 2 * g
                i2 = jnp.minimum(i0 + 2, NP - 1)
                i3 = jnp.minimum(i0 + 3, NP - 1)
                im = jnp.maximum(i0 - 1, 0)
                scores(q_odd, i0 + 1, 1)
                q_even = q_proj(xn, i2)
                acc = acc + o_proj(im, 1)
                pv(i0, 0)
                scores(q_even, i2, 0)
                q_next = q_proj(xn, i3)
                acc = acc + o_proj(i0, 0)
                pv(i0 + 1, 1)
                return q_next, acc

            _, acc = lax.fori_loop(0, NG, body, (q1, jnp.zeros((ROWS, D), F32)))
            acc = acc + o_proj(NP - 1, 1)
            return _round_bf16(x + _round_bf16(acc))

        def ffn(x, first):
            xn = _layernorm(x).astype(BF16)
            if first:
                w1_cp.wait()
            b1 = b1buf[...].reshape(1, FF).astype(F32)
            b2 = b2buf[...].reshape(1, D).astype(F32)
            h = jnp.dot(xn, w1b[...], preferred_element_type=F32)
            h = _round_bf16(_round_bf16(h) + b1)
            h = _gelu_tanh(h).astype(BF16)
            y = None
            for c in range(W2C):
                if first:
                    w2_cps[c].wait()
                yc = jnp.dot(h[:, c * FC:(c + 1) * FC], w2b[c * FC:(c + 1) * FC, :],
                             preferred_element_type=F32)
                y = yc if y is None else y + yc
            y = _round_bf16(_round_bf16(y) + b2)
            return _round_bf16(x + y)

        for cp in small:
            cp.wait()
        x = jnp.broadcast_to(xbuf[0].astype(F32), (ROWS, D))
        x = attention(x, True)
        x = ffn(x, True)
        x = attention(x, False)
        x = ffn(x, False)
        o_ref[0] = x[0:1].astype(o_ref.dtype)

    any_spec = pl.BlockSpec(memory_space=pl.ANY)
    return pl.pallas_call(
        kernel,
        out_shape=jax.ShapeDtypeStruct((B, SQ, D), A_x.dtype),
        in_specs=[any_spec] * 9,
        out_specs=pl.BlockSpec(memory_space=pltpu.VMEM),
        scratch_shapes=[
            pltpu.VMEM((NP, DH, W), U32),
            pltpu.VMEM((NP, DH, W), U32),
            pltpu.VMEM((D // 2, H * DH), U32),
            pltpu.VMEM((NP, DH, D), U32),
            pltpu.VMEM((D // 2, FF), U32),
            pltpu.VMEM((FF // 2, D), U32),
            pltpu.VMEM((B, SQ, D), BF16),
            pltpu.VMEM((FF,), BF16),
            pltpu.VMEM((D,), BF16),
            pltpu.VMEM((ROWS, W), F32),
            pltpu.VMEM((ROWS, W), F32),
            pltpu.VMEM((PD, LANES), F32),
            pltpu.VMEM((PD, LANES), F32),
            pltpu.VMEM((NP, ROWS, LANES), F32),
            pltpu.SemaphoreType.DMA((5 + W2C + NRING,)),
        ],
        compiler_params=pltpu.CompilerParams(vmem_limit_bytes=124 * 1024 * 1024),
    )(A_x, kt, vt, A_wq, wo3, B_w1, B_b1, B_w2, B_b2)
```

```python
import math

import jax
import jax.numpy as jnp
from jax import lax
import jax.experimental.pallas as pl
import jax.experimental.pallas.tpu as pltpu

F32 = jnp.float32
BF16 = jnp.bfloat16
U32 = jnp.uint32

LANES = 128
ROWS = 8
PROWS = 16
NT_DIMS = (((1,), (1,)), ((), ()))


def _ln_stats(x, eps=1e-5):
    m = jnp.mean(x, axis=-1, keepdims=True)
    c = x - m
    v = jnp.mean(c * c, axis=-1, keepdims=True)
    return m, 1.0 / jnp.sqrt(v + eps)


def _ln_dot(x, m, r, w):
    lhs = jnp.concatenate([x, jnp.ones_like(x)], axis=0).astype(BF16)
    y = jnp.dot(lhs, w, preferred_element_type=F32)
    return (y[0:ROWS] - m * y[ROWS:PROWS]) * r


def _round_bf16(x):
    return x.astype(BF16).astype(F32)


def _gelu_tanh(x):
    c = math.sqrt(2.0 / math.pi)
    return 0.5 * x * (1.0 + jnp.tanh(c * (x + 0.044715 * (x * x * x))))


def _pack(x, y=None):
    y = jnp.zeros_like(x) if y is None else y
    return pltpu.bitcast(jnp.concatenate([x, y], axis=0).astype(BF16), U32)


def _unpack(u):
    return pltpu.bitcast(u, BF16)


@jax.jit
def pallas_interleave_layers__sliding_block_cached__dense_activation_gelu__decode_kernel(
    A_x: jax.Array,
    A_k_cache: jax.Array,
    A_v_cache: jax.Array,
    A_wq: jax.Array,
    A_wo: jax.Array,
    B_x: jax.Array,
    B_w1: jax.Array,
    B_b1: jax.Array,
    B_w2: jax.Array,
    B_b2: jax.Array,
):
    B, SQ, D = A_x.shape
    _, H, SK, DH = A_k_cache.shape
    FF = B_w1.shape[1]
    assert B == 1 and SQ == 1 and A_wq.shape[1] == H * DH and H % 4 == 0
    W = min(4096, max(256, SK // 4))
    NP = H // 2
    PD = 2 * DH
    HW = DH // 2
    NT = W // LANES
    KQ = D // LANES
    KP = PD // LANES
    W2C = 4
    FC = FF // W2C
    NRING = 3
    exp2_scale = float(DH) ** -0.5 * math.log2(math.e)

    NB = PD // PROWS
    kt = jnp.transpose(A_k_cache, (0, 1, 3, 2)).reshape(NP, NB, 2, ROWS, SK)
    vt = jnp.transpose(A_v_cache, (0, 1, 3, 2)).reshape(NP, NB, 2, ROWS, SK)
    wo3 = A_wo.reshape(NP, PD, D)

    pingpong = dict(
        qp=((KQ * ROWS, PD), F32),
        qpk=((ROWS, PD), U32),
        sp=((KP * ROWS, W), F32),
        p=((ROWS, W), F32),
        m=((ROWS, LANES), F32),
        l=((ROWS, LANES), F32),
        mx=((ROWS, LANES), F32),
        gpk=((ROWS, LANES), U32),
        gl=((PROWS, LANES), F32),
        den=((PROWS, LANES), F32),
        acca=((DH, LANES), U32),
        accb=((DH, LANES), U32),
        oraw=((PROWS, PD), F32),
        opk=((ROWS, PD), U32),
        op=((KP * ROWS, D), F32),
    )
    names = list(pingpong)

    def kernel(x_hbm, k_hbm, v_hbm, wq_hbm, wo_hbm, w1_hbm, b1_hbm, w2_hbm, b2_hbm,
               o_ref,
               kbuf, vbuf, wqbuf, wobuf, w1buf, w2buf, xbuf, b1buf, b2buf, xnpk, att, sems, *pp):
        bufs = {n: (pp[2 * k], pp[2 * k + 1]) for k, n in enumerate(names)}
        qp, qpk, sp, p, m, l, mx, gpk, gl, den, acca, accb, oraw, opk, op = (bufs[n] for n in names)
        kb = kbuf.bitcast(BF16)
        vb = vbuf.bitcast(BF16)
        wqb = wqbuf.bitcast(BF16)
        wob = wobuf.bitcast(BF16)
        w1b = w1buf.bitcast(BF16)
        w2b = w2buf.bitcast(BF16)

        S_SMALL, S_WQ, S_K0, S_WO, S_W1, S_W2 = 0, 1, 2, 3, 4, 5
        S_RING = S_W2 + W2C

        def window_copies(hbm, buf, start, n, sem):
            return [pltpu.make_async_copy(
                hbm.at[pl.ds(start, n), :, h, :, pl.ds(SK - W, W)],
                buf.at[pl.ds(start, n), :, pl.ds(h * ROWS, ROWS), :], sem) for h in range(2)]

        def group_copies(j, with_k):
            sem = sems.at[S_RING + j % NRING]
            return ((window_copies(k_hbm, kb, j + 2, 1, sem) if with_k else [])
                    + window_copies(v_hbm, vb, j, 1, sem))

        small = [pltpu.make_async_copy(x_hbm, xbuf, sems.at[S_SMALL]),
                 pltpu.make_async_copy(b1_hbm, b1buf, sems.at[S_SMALL]),
                 pltpu.make_async_copy(b2_hbm, b2buf, sems.at[S_SMALL])]
        wq_cp = pltpu.make_async_copy(wq_hbm, wqb, sems.at[S_WQ])
        k0_cps = window_copies(k_hbm, kb, 0, 2, sems.at[S_K0])
        wo_cp = pltpu.make_async_copy(wo_hbm, wob, sems.at[S_WO])
        w1_cp = pltpu.make_async_copy(w1_hbm, w1b, sems.at[S_W1])
        w2_cps = [pltpu.make_async_copy(w2_hbm.at[pl.ds(c * FC, FC)], w2b.at[pl.ds(c * FC, FC)],
                                        sems.at[S_W2 + c]) for c in range(W2C)]

        wq_cp.start()
        for cp in small:
            cp.start()
        for cp in k0_cps:
            cp.start()
        wo_cp.start()
        for j in range(NRING):
            for cp in group_copies(j, True):
                cp.start()

        row = lax.broadcasted_iota(jnp.int32, (ROWS, PD), 0)
        col = lax.broadcasted_iota(jnp.int32, (ROWS, PD), 1)
        first_head = col < DH
        diag = jnp.where(first_head, 0, 1) == row

        def tile(t):
            return slice(t * LANES, (t + 1) * LANES)

        def rows(t):
            return slice(t * ROWS, (t + 1) * ROWS)

        def mm(a, b_):
            return jnp.dot(a, b_, preferred_element_type=F32)[0:ROWS]

        def q_proj(i, b):
            off = pl.multiple_of(i * PD, LANES)
            for c in range(KQ):
                qp[b][rows(c)] = mm(_unpack(xnpk[:, tile(c)]), wqb[tile(c), pl.ds(off, PD)])

        def qk(i, b):
            for c in range(KP):
                sp[b][rows(c)] = mm(_unpack(qpk[b][:, tile(c)]), kb[i, rows(c)].reshape(LANES, W))

        def lane_combine(g_ref, acc_ref):
            return lax.dot_general(_unpack(g_ref[...]), _unpack(acc_ref[...]), NT_DIMS,
                                   preferred_element_type=F32)

        def o_proj(i, b):
            for c in range(KP):
                op[b][rows(c)] = mm(_unpack(opk[b][:, tile(c)]), wob[i, tile(c), :])

        def row_max(b):
            mx[b][...] = jnp.broadcast_to(jnp.max(m[b][...], axis=1, keepdims=True), (ROWS, LANES))

        def row_sum(b):
            return jnp.broadcast_to(jnp.sum(gl[b][...], axis=1, keepdims=True), (PROWS, LANES))

        def sum_rows(ref, n, cols=slice(None)):
            s = ref[rows(0), cols]
            for c in range(1, n):
                s = s + ref[rows(c), cols]
            return s

        def q_pack(b):
            qpk[b][...] = _pack(jnp.where(diag, sum_rows(qp[b], KQ), 0.0))

        def lane_weights(b):
            g = []
            for r in range(2):
                d = jnp.broadcast_to(m[b][r:r + 1] - mx[b][r:r + 1], (ROWS, LANES))
                g.append(_round_bf16(jnp.exp2(d * exp2_scale)))
                gl[b][rows(r)] = g[r] * l[b][r:r + 1]
            gpk[b][...] = _pack(g[0], g[1])

        def normalise(o, dn):
            inv = jnp.concatenate([1.0 / dn] * KP, axis=1)
            o = o * inv
            return _pack(jnp.where(first_head, o[0:ROWS], o[ROWS:PROWS]))

        def o_pack(b):
            opk[b][...] = normalise(oraw[b][...], den[b][...])

        def accumulate(b):
            att[...] += sum_rows(op[b], KP)

        def softmax_steps(b):
            mm_ = None
            for t in range(NT):
                s = sum_rows(sp[b], KP, tile(t))
                sp[b][rows(0), tile(t)] = s
                mm_ = s if mm_ is None else jnp.maximum(mm_, s)
                yield
            m[b][...] = mm_
            ll = None
            for t in range(NT):
                e = jnp.exp2((sp[b][rows(0), tile(t)] - mm_) * exp2_scale)
                p[b][:, tile(t)] = e
                ll = e if ll is None else ll + e
                if t == NT - 1:
                    l[b][...] = ll
                yield

        def pv_steps(i, b):
            G = 6 * ROWS
            DB = 1
            HB = HW // DB
            for j in range(2):
                for db in range(DB):
                    ng = HB // G
                    lo_acc = [None] * ng
                    hi_acc = [None] * ng
                    for t in range(NT):
                        pb = p[b][j:j + 1, tile(t)]
                        for g in range(ng):
                            r0 = j * HW + db * HB + g * G
                            u = vbuf[i, r0 // ROWS:(r0 + G) // ROWS, :, tile(t)].reshape(G, LANES)
                            lo = pltpu.bitcast(u << 16, F32) * pb
                            lo_acc[g] = lo if t == 0 else lo_acc[g] + lo
                            hi = pltpu.bitcast(u & U32(0xFFFF0000), F32) * pb
                            hi_acc[g] = hi if t == 0 else hi_acc[g] + hi
                            if t == NT - 1:
                                acca[b][r0:r0 + G, :] = pltpu.pack_elementwise(
                                    [lo_acc[g], hi_acc[g]], packed_dtype=BF16)
                        if (t * DB + db) % DB == DB - 1 or True:
                            if (db * NT + t) % DB == 0:
                                yield

        def step(j, b):
            nb = 1 - b

            def mxu():
                qk(jnp.minimum(j + 2, NP - 1), b)
                q_proj(jnp.minimum(j + 4, NP - 1), b)
                oraw[b][...] = lane_combine(gpk[b], accb[b])
                o_proj(jnp.maximum(j - 4, 0), b)

            def xlu():
                row_max(b)
                den[b][...] = row_sum(b)

            def front():
                small_stages = [lambda: lane_weights(nb), lambda: q_pack(nb), lambda: o_pack(nb),
                                lambda: accumulate(nb)]

                def copy_acc():
                    accb[nb][...] = acca[nb][...]
                small_stages.append(copy_acc)
                sm = softmax_steps(nb)
                for k, _ in enumerate(pv_steps(j, b)):
                    if k < len(small_stages):
                        small_stages[k]()
                    next(sm)
            front()
            mxu()
            xlu()

        def attention(x, first):
            mean, rstd = _ln_stats(x)
            xnpk[...] = _pack((x - mean) * rstd)
            for ref in (mx[1], m[1], gpk[0], accb[0], acca[1], oraw[1], opk[0], op[1], att):
                ref[...] = jnp.zeros(ref.shape, ref.dtype)
            for ref in (l[1], gl[0], den[1]):
                ref[...] = jnp.ones(ref.shape, ref.dtype)
            if first:
                wq_cp.wait()
            qpk[0][...] = _pack(jnp.where(diag, _ln_dot(x, mean, rstd, wqb[:, 0:PD]), 0.0))
            if first:
                for cp in k0_cps:
                    cp.wait()
            qk(0, 0)
            q_proj(1, 1)
            q_pack(1)
            qk(1, 1)
            q_proj(2, 0)
            q_pack(0)
            q_proj(3, 1)
            for _ in softmax_steps(0):
                pass
            if first:
                wo_cp.wait()

            def body(j, carry):
                if first:
                    @pl.when(j < NP - 2)
                    def _():
                        for cp in group_copies(j, True):
                            cp.wait()

                    @pl.when(j >= NP - 2)
                    def _():
                        for cp in group_copies(j, False):
                            cp.wait()

                    @pl.when(j + NRING < NP - 2)
                    def _():
                        for cp in group_copies(j + NRING, True):
                            cp.start()

                    @pl.when(jnp.logical_and(j + NRING >= NP - 2, j + NRING < NP))
                    def _():
                        for cp in group_copies(j + NRING, False):
                            cp.start()

                    @pl.when(j + NRING == NP - 1)
                    def _():
                        w1_cp.start()
                        for cp in w2_cps:
                            cp.start()

                for b in range(2):
                    @pl.when(j % 2 == b)
                    def _():
                        step(j, b)
                return carry

            lax.fori_loop(0, NP, body, 0)

            lane_weights(1)
            o2 = lane_combine(gpk[0], accb[0])
            o1 = lane_combine(gpk[1], acca[1])
            a = att[...] + sum_rows(op[1], KP)
            a = a + mm(_unpack(opk[0][...]), wob[NP - 4])
            a = a + mm(_unpack(normalise(oraw[1][...], den[1][...])), wob[NP - 3])
            a = a + mm(_unpack(normalise(o2, row_sum(0))), wob[NP - 2])
            a = a + mm(_unpack(normalise(o1, row_sum(1))), wob[NP - 1])
            return _round_bf16(x + _round_bf16(a))

        def ffn(x, first):
            mean, rstd = _ln_stats(x)
            if first:
                w1_cp.wait()
            b1 = b1buf[...].reshape(1, FF).astype(F32)
            b2 = b2buf[...].reshape(1, D).astype(F32)
            h = _ln_dot(x, mean, rstd, w1b[...])
            h = _round_bf16(_round_bf16(h) + b1)
            h = _gelu_tanh(h).astype(BF16)
            y = None
            for c in range(W2C):
                if first:
                    w2_cps[c].wait()
                yc = jnp.dot(h[:, c * FC:(c + 1) * FC], w2b[c * FC:(c + 1) * FC, :],
                             preferred_element_type=F32)
                y = yc if y is None else y + yc
            y = _round_bf16(_round_bf16(y) + b2)
            return _round_bf16(x + y)

        for cp in small:
            cp.wait()
        x = jnp.broadcast_to(xbuf[0].astype(F32), (ROWS, D))
        x = attention(x, True)
        x = ffn(x, True)
        x = attention(x, False)
        x = ffn(x, False)
        o_ref[0] = x[0:1].astype(o_ref.dtype)

    any_spec = pl.BlockSpec(memory_space=pl.ANY)
    return pl.pallas_call(
        kernel,
        out_shape=jax.ShapeDtypeStruct((B, SQ, D), A_x.dtype),
        in_specs=[any_spec] * 9,
        out_specs=pl.BlockSpec(memory_space=pltpu.VMEM),
        scratch_shapes=[
            pltpu.VMEM((NP, NB, ROWS, W), U32),
            pltpu.VMEM((NP, NB, ROWS, W), U32),
            pltpu.VMEM((D // 2, H * DH), U32),
            pltpu.VMEM((NP, DH, D), U32),
            pltpu.VMEM((D // 2, FF), U32),
            pltpu.VMEM((FF // 2, D), U32),
            pltpu.VMEM((B, SQ, D), BF16),
            pltpu.VMEM((FF,), BF16),
            pltpu.VMEM((D,), BF16),
            pltpu.VMEM((ROWS, D), U32),
            pltpu.VMEM((ROWS, D), F32),
            pltpu.SemaphoreType.DMA((5 + W2C + NRING,)),
        ] + [pltpu.VMEM(*pingpong[n]) for n in names for _ in range(2)],
        compiler_params=pltpu.CompilerParams(vmem_limit_bytes=124 * 1024 * 1024),
    )(A_x, kt, vt, A_wq, wo3, B_w1, B_b1, B_w2, B_b2)
```

```python
import math

import jax
import jax.numpy as jnp
from jax import lax
import jax.experimental.pallas as pl
import jax.experimental.pallas.tpu as pltpu

F32 = jnp.float32
BF16 = jnp.bfloat16
U32 = jnp.uint32

LANES = 128
ROWS = 8
PROWS = 16
NT_DIMS = (((1,), (1,)), ((), ()))


def _ln_stats(x, eps=1e-5):
    m = jnp.mean(x, axis=-1, keepdims=True)
    c = x - m
    v = jnp.mean(c * c, axis=-1, keepdims=True)
    return m, 1.0 / jnp.sqrt(v + eps)


def _centered_dot(x, m, w):
    lhs = jnp.concatenate([x, jnp.ones_like(x)], axis=0).astype(BF16)
    y = jnp.dot(lhs, w, preferred_element_type=F32)
    return y[0:ROWS] - m * y[ROWS:PROWS]


def _round_bf16(x):
    return x.astype(BF16).astype(F32)


def _gelu_tanh(x):
    c = math.sqrt(2.0 / math.pi)
    return 0.5 * x * (1.0 + jnp.tanh(c * (x + 0.044715 * (x * x * x))))


def _pack(x, y=None):
    y = jnp.zeros_like(x) if y is None else y
    return pltpu.bitcast(jnp.concatenate([x, y], axis=0).astype(BF16), U32)


def _unpack(u):
    return pltpu.bitcast(u, BF16)


@jax.jit
def pallas_interleave_layers__sliding_block_cached__dense_activation_gelu__decode_kernel(
    A_x: jax.Array,
    A_k_cache: jax.Array,
    A_v_cache: jax.Array,
    A_wq: jax.Array,
    A_wo: jax.Array,
    B_x: jax.Array,
    B_w1: jax.Array,
    B_b1: jax.Array,
    B_w2: jax.Array,
    B_b2: jax.Array,
):
    B, SQ, D = A_x.shape
    _, H, SK, DH = A_k_cache.shape
    FF = B_w1.shape[1]
    assert B == 1 and SQ == 1 and A_wq.shape[1] == H * DH and H % 4 == 0
    W = min(4096, max(256, SK // 4))
    NP = H // 2
    PD = 2 * DH
    HW = DH // 2
    NT = W // LANES
    KQ = D // LANES
    KP = PD // LANES
    W2B = [0, 512, 1024, FF - LANES, FF]
    W2C = len(W2B) - 1
    XT = 4
    XT2 = 16
    XN = 2
    ND = (NP - 4) // 2
    G = 2 * ROWS
    DB = 2
    NRING = 3
    exp2_scale = float(DH) ** -0.5 * math.log2(math.e)

    NB = PD // PROWS
    kt = jnp.transpose(A_k_cache, (0, 1, 3, 2)).reshape(NP, NB, 2, ROWS, SK)
    vt = jnp.transpose(A_v_cache, (0, 1, 3, 2)).reshape(NP, NB, 2, ROWS, SK)
    wo3 = A_wo.reshape(NP, PD, D)

    pingpong = dict(
        qp=((KQ * ROWS, PD), F32),
        qpk=((ROWS, PD), U32),
        sp=((KP * ROWS, W), F32),
        p=((ROWS, W), F32),
        st=((ROWS, 3 * LANES), F32),
        gpk=((ROWS, LANES), U32),
        gl=((PROWS, LANES), F32),
        den=((PROWS, LANES), F32),
        acca=((DH, LANES), U32),
        accb=((DH, LANES), U32),
        ppk=((ROWS, max(XN, 1) * LANES), U32),
        oraw=(((1 + XN) * PROWS, PD), F32),
        op=((ND * KP * ROWS, D), F32),
    )
    names = list(pingpong)

    def kernel(x_hbm, k_hbm, v_hbm, wq_hbm, wo_hbm, w1_hbm, b1_hbm, w2_hbm, b2_hbm,
               o_ref,
               kbuf, vbuf, wqbuf, wobuf, w1buf, w2buf, xbuf, b1buf, b2buf, xnpk, att, opk, scale, vlo, vlo2, sems, *pp):
        bufs = {n: (pp[2 * k], pp[2 * k + 1]) for k, n in enumerate(names)}
        qp, qpk, sp, p, st, gpk, gl, den, acca, accb, ppk, oraw, op = (bufs[n] for n in names)
        kb = kbuf.bitcast(BF16)
        vb = vbuf.bitcast(BF16)
        wqb = wqbuf.bitcast(BF16)
        wob = wobuf.bitcast(BF16)
        w1b = w1buf.bitcast(BF16)
        w2b = w2buf.bitcast(BF16)

        S_SMALL, S_WQ, S_K0, S_WO, S_W1, S_W2 = 0, 1, 2, 3, 4, 5
        S_RING = S_W2 + W2C

        def window_copies(hbm, buf, start, n, sem):
            return [pltpu.make_async_copy(
                hbm.at[pl.ds(start, n), :, h, :, pl.ds(SK - W, W)],
                buf.at[pl.ds(start, n), :, pl.ds(h * ROWS, ROWS), :], sem) for h in range(2)]

        def group_copies(j, with_k):
            sem = sems.at[S_RING + j % NRING]
            return ((window_copies(k_hbm, kb, j + 2, 1, sem) if with_k else [])
                    + window_copies(v_hbm, vb, j, 1, sem))

        small = [pltpu.make_async_copy(x_hbm, xbuf, sems.at[S_SMALL]),
                 pltpu.make_async_copy(b1_hbm, b1buf, sems.at[S_SMALL]),
                 pltpu.make_async_copy(b2_hbm, b2buf, sems.at[S_SMALL])]
        wq_cps = [pltpu.make_async_copy(wq_hbm.at[:, i * PD:(i + 1) * PD], wqb.at[i], sems.at[S_WQ])
                  for i in range(NP)]
        k0_cps = window_copies(k_hbm, kb, 0, 2, sems.at[S_K0])
        wo_cp = pltpu.make_async_copy(wo_hbm, wob, sems.at[S_WO])
        w1_cp = pltpu.make_async_copy(w1_hbm, w1b, sems.at[S_W1])
        w2_cps = [pltpu.make_async_copy(w2_hbm.at[W2B[c]:W2B[c + 1]], w2b.at[W2B[c]:W2B[c + 1]],
                                        sems.at[S_W2 + c]) for c in range(W2C)]

        for cp in wq_cps:
            cp.start()
        for cp in small:
            cp.start()
        for cp in k0_cps:
            cp.start()
        wo_cp.start()
        for j in range(NRING):
            for cp in group_copies(j, True):
                cp.start()

        row_id = lax.broadcasted_iota(jnp.int32, (ROWS, PD), 0)
        col = lax.broadcasted_iota(jnp.int32, (ROWS, PD), 1)
        first_head = col < DH
        diag = jnp.where(first_head, 0, 1) == row_id

        def tile(t):
            return slice(t * LANES, (t + 1) * LANES)

        def rows(t):
            return slice(t * ROWS, (t + 1) * ROWS)

        def mm(a, b_):
            return jnp.dot(a, b_, preferred_element_type=F32)[0:ROWS]

        def q_proj(i, b):
            for c in range(KQ):
                qp[b][rows(c)] = mm(_unpack(xnpk[:, tile(c)]), wqb[i, tile(c), :])

        def qk(i, b, cs=range(KP)):
            for c in cs:
                sp[b][rows(c)] = mm(_unpack(qpk[b][:, tile(c)]), kb[i, rows(c)].reshape(LANES, W))

        def nt(a, b_):
            return lax.dot_general(a, b_, NT_DIMS, preferred_element_type=F32)

        def combine_parts(i, b, acc_ref, xn=XN):
            parts = [nt(_unpack(gpk[b][...]), _unpack(acc_ref[...]))]
            for t in range(xn):
                parts.append(nt(_unpack(ppk[b][:, tile(t)]), vb[i, :, :, tile(t)].reshape(PD, LANES)))
            return parts

        def combine(i, b):
            for k, part in enumerate(combine_parts(i, b, accb[b])):
                oraw[b][k * PROWS:(k + 1) * PROWS] = part

        def o_proj(i0, b):
            for k in range(ND):
                for c in range(KP):
                    op[b][rows(k * KP + c)] = mm(_unpack(opk[i0 + k, :, tile(c)]), wob[i0 + k, tile(c), :])

        def row_max(b):
            st[b][:, tile(2)] = jnp.broadcast_to(
                jnp.max(st[b][:, tile(0)], axis=1, keepdims=True), (ROWS, LANES))

        def row_sum(b):
            return jnp.broadcast_to(jnp.sum(gl[b][...], axis=1, keepdims=True), (PROWS, LANES))

        def sum_rows(ref, n, cols=slice(None), off=0):
            s = ref[rows(off), cols]
            for c in range(1, n):
                s = s + ref[rows(off + c), cols]
            return s

        def q_pack(b):
            qpk[b][...] = _pack(jnp.where(diag, sum_rows(qp[b], KQ), 0.0))

        def row(ref, r, cols=slice(None)):
            v = ref[r:r + 1, cols]
            return jnp.broadcast_to(v, (ROWS, v.shape[1]))

        def lane_weights(b, xn=XN):
            g = []
            for r in range(2):
                g.append(_round_bf16(jnp.exp2((row(st[b], r, tile(0)) - row(st[b], r, tile(2))) * scale[...])))
                gl[b][rows(r)] = g[r] * row(st[b], r, tile(1))
            gpk[b][...] = _pack(g[0], g[1])
            for t in range(xn):
                ppk[b][:, tile(t)] = _pack(g[0] * row(p[b], 0, tile(t)), g[1] * row(p[b], 1, tile(t)))

        def normalise(parts, dn):
            o = parts[0]
            for part in parts[1:]:
                o = o + part
            o = o * jnp.concatenate([1.0 / dn] * KP, axis=1)
            return _pack(jnp.where(first_head, o[0:ROWS], o[ROWS:PROWS]))

        def stored_parts(b):
            return [oraw[b][k * PROWS:(k + 1) * PROWS] for k in range(1 + XN)]

        def o_pack(i, b):
            opk[i] = normalise(stored_parts(b), den[b][...])

        def softmax_steps(b):
            NC = 4

            def tree(f, xs):
                while len(xs) > 1:
                    xs = [f(xs[k], xs[k + 1]) for k in range(0, len(xs), 2)]
                return xs[0]

            mc = [None] * NC
            for t in range(NT):
                s = sum_rows(sp[b], KP, tile(t))
                sp[b][rows(0), tile(t)] = s
                mc[t % NC] = s if t < NC else jnp.maximum(mc[t % NC], s)
                yield
            mm_ = tree(jnp.maximum, mc)
            st[b][:, tile(0)] = mm_
            lc = [None] * NC
            sc = scale[...]
            for t in range(NT):
                e = jnp.exp2((sp[b][rows(0), tile(t)] - mm_) * sc)
                p[b][:, tile(t)] = e
                lc[t % NC] = e if t < NC else lc[t % NC] + e
                if t == NT - 1:
                    st[b][:, tile(1)] = tree(jnp.add, lc)
                yield

        def pv_steps(i, b, first, xn, xt, lo_ref):
            HB = HW // DB
            order = sorted(range(xn, NT), key=lambda t: ((t - xn + 0.5) / (NT - xt - xn) if t < NT - xt
                                                         else (t - (NT - xt) + 0.5) / xt))
            for j in range(2):
                for db in range(DB):
                    ng = HB // G
                    lo_acc = [None] * ng
                    hi_acc = [None] * ng
                    for pos, t in enumerate(order):
                        pb = p[b][j:j + 1, tile(t)]
                        for g in range(ng):
                            r0 = j * HW + db * HB + g * G
                            bands = slice(r0 // ROWS, (r0 + G) // ROWS)
                            u = vbuf[i, bands, :, tile(t)]
                            if t < NT - xt or first:
                                lo = u << 16
                                hi = u & U32(0xFFFF0000)
                                if t >= NT - xt:
                                    vbuf[i, bands, :, tile(t)] = hi
                                    lo_ref[bands, :, tile(t - (NT - xt))] = lo
                            else:
                                lo = lo_ref[bands, :, tile(t - (NT - xt))]
                                hi = u
                            lo = pltpu.bitcast(lo.reshape(G, LANES), F32) * pb
                            lo_acc[g] = lo if pos == 0 else lo_acc[g] + lo
                            hi = pltpu.bitcast(hi.reshape(G, LANES), F32) * pb
                            hi_acc[g] = hi if pos == 0 else hi_acc[g] + hi
                            if pos == len(order) - 1:
                                acca[b][r0:r0 + G, :] = pltpu.pack_elementwise(
                                    [lo_acc[g], hi_acc[g]], packed_dtype=BF16)
                        yield

        def step(j, b, first, left):
            nb = 1 - b
            xn = XN if left is None else 0
            extra = [lambda: lane_weights(nb, 0 if left == 1 else XN),
                     lambda: o_pack(jnp.maximum(j - 3, 0), nb)]

            def copy_acc():
                accb[nb][...] = acca[nb][...]
            extra.append(copy_acc)
            if left is None:
                extra.append(lambda: q_pack(nb))
            if left == 1:
                for k in range(ND):
                    def acc_op(k=k):
                        s_ = sum_rows(op[nb], KP, off=k * KP)
                        att[...] = s_ if k == 0 else att[...] + s_
                    extra.append(acc_op)
            if left != 1:
                sm = softmax_steps(nb)
                extra += [lambda: next(sm)] * (2 * NT)
            steps = list(range(2 * DB * (NT - xn)))
            done = 0
            for k, _ in enumerate(pv_steps(j, b, first, xn, *(
                    (XT, vlo.at[j]) if left is None else (XT2, vlo2.at[2 - left])))):
                upto = (k + 1) * len(extra) // len(steps)
                for f in extra[done:upto]:
                    f()
                done = upto
            if left is None:
                qk(j + 2, b)
            combine(jnp.maximum(j - 2, 0), b)
            if left is None:
                q_proj(jnp.minimum(j + 4, NP - 1), b)
            else:
                o_proj((2 - left) * ND, b)
            row_max(b)
            den[b][...] = row_sum(b)

        def attention(x, first):
            mean, rstd = _ln_stats(x)
            xnpk[...] = _pack(x - mean)
            scale[...] = jnp.broadcast_to(rstd * exp2_scale, (ROWS, LANES))
            for ref in (p[1].at[:, 0:max(XN, 1) * LANES], gpk[0], ppk[0], accb[0], acca[1], oraw[1]):
                ref[...] = jnp.zeros(ref.shape, ref.dtype)
            for ref in (st[1], gl[0], den[1]):
                ref[...] = jnp.ones(ref.shape, ref.dtype)
            if first:
                for cp in wq_cps:
                    cp.wait()
            qpk[0][...] = _pack(jnp.where(diag, _centered_dot(x, mean, wqb[0]), 0.0))
            if first:
                for cp in k0_cps:
                    cp.wait()
            qk(0, 0, (0,))
            q_proj(1, 1)
            q_pack(1)
            qk(0, 0, range(1, KP))
            qk(1, 1)
            q_proj(2, 0)
            q_pack(0)
            q_proj(3, 1)
            for _ in softmax_steps(0):
                pass
            if first:
                wo_cp.wait()

            def body(j, carry):
                if first:
                    @pl.when(j < NP - 2)
                    def _():
                        for cp in group_copies(j, True):
                            cp.wait()

                    @pl.when(j >= NP - 2)
                    def _():
                        for cp in group_copies(j, False):
                            cp.wait()

                    @pl.when(j + NRING < NP - 2)
                    def _():
                        for cp in group_copies(j + NRING, True):
                            cp.start()

                    @pl.when(jnp.logical_and(j + NRING >= NP - 2, j + NRING < NP))
                    def _():
                        for cp in group_copies(j + NRING, False):
                            cp.start()

                    @pl.when(j + NRING == NP - 1)
                    def _():
                        w1_cp.start()
                        for cp in w2_cps:
                            cp.start()

                for b in range(2):
                    @pl.when(jnp.logical_and(j % 2 == b, j < NP - 2))
                    def _():
                        step(j, b, first, None)

                for left in (2, 1):
                    @pl.when(j == NP - left)
                    def _():
                        step(NP - left, (NP - left) % 2, first, left)
                return carry

            lax.fori_loop(0, NP, body, 0)

            lane_weights(1, 0)
            o2 = combine_parts(NP - 2, 0, accb[0], 0)
            o1 = combine_parts(NP - 1, 1, acca[1], 0)
            a = att[...] + sum_rows(op[1], ND * KP)
            a = a + mm(_unpack(opk[NP - 4]), wob[NP - 4])
            a = a + mm(_unpack(normalise(stored_parts(1), den[1][...])), wob[NP - 3])
            a = a + mm(_unpack(normalise(o2, row_sum(0))), wob[NP - 2])
            a = a + mm(_unpack(normalise(o1, row_sum(1))), wob[NP - 1])
            return _round_bf16(x + _round_bf16(a))

        def ffn(x, first):
            mean, rstd = _ln_stats(x)
            if first:
                w1_cp.wait()
            b1 = b1buf[...].reshape(1, FF).astype(F32)
            b2 = b2buf[...].reshape(1, D).astype(F32)
            h = _centered_dot(x, mean, w1b[...]) * rstd
            h = _round_bf16(_round_bf16(h) + b1)
            h = _gelu_tanh(h).astype(BF16)
            y = None
            for c in range(W2C):
                if first:
                    w2_cps[c].wait()
                yc = jnp.dot(h[:, W2B[c]:W2B[c + 1]], w2b[W2B[c]:W2B[c + 1], :],
                             preferred_element_type=F32)
                y = yc if y is None else y + yc
            y = _round_bf16(_round_bf16(y) + b2)
            return _round_bf16(x + y)

        for cp in small:
            cp.wait()
        x = jnp.broadcast_to(xbuf[0].astype(F32), (ROWS, D))
        x = attention(x, True)
        x = ffn(x, True)
        x = attention(x, False)
        x = ffn(x, False)
        o_ref[0] = x[0:1].astype(o_ref.dtype)

    any_spec = pl.BlockSpec(memory_space=pl.ANY)
    return pl.pallas_call(
        kernel,
        out_shape=jax.ShapeDtypeStruct((B, SQ, D), A_x.dtype),
        in_specs=[any_spec] * 9,
        out_specs=pl.BlockSpec(memory_space=pltpu.VMEM),
        scratch_shapes=[
            pltpu.VMEM((NP, NB, ROWS, W), U32),
            pltpu.VMEM((NP, NB, ROWS, W), U32),
            pltpu.VMEM((NP, D // 2, PD), U32),
            pltpu.VMEM((NP, DH, D), U32),
            pltpu.VMEM((D // 2, FF), U32),
            pltpu.VMEM((FF // 2, D), U32),
            pltpu.VMEM((B, SQ, D), BF16),
            pltpu.VMEM((FF,), BF16),
            pltpu.VMEM((D,), BF16),
            pltpu.VMEM((ROWS, D), U32),
            pltpu.VMEM((ROWS, D), F32),
            pltpu.VMEM((NP, ROWS, PD), U32),
            pltpu.VMEM((ROWS, LANES), F32),
            pltpu.VMEM((NP - 2, NB, ROWS, max(XT, 1) * LANES), U32),
            pltpu.VMEM((2, NB, ROWS, max(XT2, 1) * LANES), U32),
            pltpu.SemaphoreType.DMA((5 + W2C + NRING,)),
        ] + [pltpu.VMEM(*pingpong[n]) for n in names for _ in range(2)],
        compiler_params=pltpu.CompilerParams(vmem_limit_bytes=511 * 256 * 1024),
    )(A_x, kt, vt, A_wq, wo3, B_w1, B_b1, B_w2, B_b2)
```

```python
import math

import jax
import jax.numpy as jnp
from jax import lax
import jax.experimental.pallas as pl
import jax.experimental.pallas.tpu as pltpu

F32 = jnp.float32
BF16 = jnp.bfloat16
U32 = jnp.uint32

LANES = 128
ROWS = 8
PROWS = 16
NT_DIMS = (((1,), (1,)), ((), ()))


def _ln_stats(x, eps=1e-5):
    m = jnp.mean(x, axis=-1, keepdims=True)
    c = x - m
    v = jnp.mean(c * c, axis=-1, keepdims=True)
    return m, 1.0 / jnp.sqrt(v + eps)


def _centered_dot(x, m, w):
    lhs = jnp.concatenate([x, jnp.ones_like(x)], axis=0).astype(BF16)
    y = jnp.dot(lhs, w, preferred_element_type=F32)
    return y[0:ROWS] - m * y[ROWS:PROWS]


def _round_bf16(x):
    return x.astype(BF16).astype(F32)


def _gelu_tanh(x):
    c = math.sqrt(2.0 / math.pi)
    return 0.5 * x * (1.0 + jnp.tanh(c * (x + 0.044715 * (x * x * x))))


def _pack(x, y=None):
    y = jnp.zeros_like(x) if y is None else y
    return pltpu.bitcast(jnp.concatenate([x, y], axis=0).astype(BF16), U32)


def _unpack(u):
    return pltpu.bitcast(u, BF16)


def _split(u):
    return u << 16, u & U32(0xFFFF0000)


def _deinterleave(u):
    rows16 = pltpu.bitcast(jnp.concatenate(_split(u), axis=0), F32)
    return pltpu.bitcast(rows16.astype(BF16), U32)


@jax.jit
def pallas_interleave_layers__sliding_block_cached__dense_activation_gelu__decode_kernel(
    A_x: jax.Array,
    A_k_cache: jax.Array,
    A_v_cache: jax.Array,
    A_wq: jax.Array,
    A_wo: jax.Array,
    B_x: jax.Array,
    B_w1: jax.Array,
    B_b1: jax.Array,
    B_w2: jax.Array,
    B_b2: jax.Array,
):
    B, SQ, D = A_x.shape
    _, H, SK, DH = A_k_cache.shape
    FF = B_w1.shape[1]
    assert B == 1 and SQ == 1 and A_wq.shape[1] == H * DH and H % 4 == 0
    W = min(4096, max(256, SK // 4))
    NP = H // 2
    PD = 2 * DH
    HW = DH // 2
    NT = W // LANES
    KQ = D // LANES
    KP = PD // LANES
    W2B = [0, 512, 1024, FF - LANES, FF]
    W2C = len(W2B) - 1
    XT = 3
    XT2 = 16
    XU = 9
    XN = -(-XU // KP)
    CB = LANES // PROWS
    ND = (NP - 4) // 2
    G = 2 * ROWS
    DB = 3
    NRING = 3
    exp2_scale = float(DH) ** -0.5 * math.log2(math.e)

    NB = PD // PROWS
    kt = jnp.transpose(A_k_cache, (0, 1, 3, 2)).reshape(NP, NB, 2, ROWS, SK)
    vt = jnp.transpose(A_v_cache, (0, 1, 3, 2)).reshape(NP, NB, 2, ROWS, SK)
    wo3 = A_wo.reshape(NP, PD, D)

    pingpong = dict(
        qp=((KQ * ROWS, PD), F32),
        qpk=((ROWS, PD), U32),
        sp=((KP * ROWS, W), F32),
        p=((ROWS, W), F32),
        st=((ROWS, 3 * LANES), F32),
        gl=((PROWS, LANES), F32),
        den=((PROWS, LANES), F32),
        acca=((ROWS, NB * LANES), U32),
        accb=((ROWS, NB * LANES), U32),
        gpk=((ROWS, (1 + max(XN, 1)) * LANES), U32),
        oraw=(((1 + XN) * PROWS, PD), F32),
        op=((ND * KP * ROWS, D), F32),
    )
    names = list(pingpong)

    def kernel(x_hbm, k_hbm, v_hbm, wq_hbm, wo_hbm, w1_hbm, b1_hbm, w2_hbm, b2_hbm,
               o_ref,
               kbuf, vbuf, wqbuf, wobuf, w1buf, w2buf, xbuf, b1buf, b2buf, xnpk, att, opk, scale, vlo, vlo2, sems, *pp):
        bufs = {n: (pp[2 * k], pp[2 * k + 1]) for k, n in enumerate(names)}
        qp, qpk, sp, p, st, gl, den, acca, accb, gpk, oraw, op = (bufs[n] for n in names)
        kb = kbuf.bitcast(BF16)
        vb = vbuf.bitcast(BF16)
        wqb = wqbuf.bitcast(BF16)
        wob = wobuf.bitcast(BF16)
        w1b = w1buf.bitcast(BF16)
        w2b = w2buf.bitcast(BF16)

        S_SMALL, S_WQ, S_K0, S_WO, S_W1, S_W2 = 0, 1, 2, 3, 4, 5
        S_RING = S_W2 + W2C

        def window_copies(hbm, buf, start, n, sem):
            return [pltpu.make_async_copy(
                hbm.at[pl.ds(start, n), :, h, :, pl.ds(SK - W, W)],
                buf.at[pl.ds(start, n), :, pl.ds(h * ROWS, ROWS), :], sem) for h in range(2)]

        def group_copies(j, with_k):
            sem = sems.at[S_RING + j % NRING]
            return ((window_copies(k_hbm, kb, j + 2, 1, sem) if with_k else [])
                    + window_copies(v_hbm, vb, j, 1, sem))

        small = [pltpu.make_async_copy(x_hbm, xbuf, sems.at[S_SMALL]),
                 pltpu.make_async_copy(b1_hbm, b1buf, sems.at[S_SMALL]),
                 pltpu.make_async_copy(b2_hbm, b2buf, sems.at[S_SMALL])]
        wq_cps = [pltpu.make_async_copy(wq_hbm.at[:, i * PD:(i + 1) * PD], wqb.at[i], sems.at[S_WQ])
                  for i in range(NP)]
        k0_cps = window_copies(k_hbm, kb, 0, 2, sems.at[S_K0])
        wo_cp = pltpu.make_async_copy(wo_hbm, wob, sems.at[S_WO])
        w1_cp = pltpu.make_async_copy(w1_hbm, w1b, sems.at[S_W1])
        w2_cps = [pltpu.make_async_copy(w2_hbm.at[W2B[c]:W2B[c + 1]], w2b.at[W2B[c]:W2B[c + 1]],
                                        sems.at[S_W2 + c]) for c in range(W2C)]

        for cp in wq_cps:
            cp.start()
        for cp in small:
            cp.start()
        for cp in k0_cps:
            cp.start()
        wo_cp.start()
        for j in range(NRING):
            for cp in group_copies(j, True):
                cp.start()

        row_id = lax.broadcasted_iota(jnp.int32, (ROWS, PD), 0)
        col = lax.broadcasted_iota(jnp.int32, (ROWS, PD), 1)
        first_head = col < DH
        diag = jnp.where(first_head, 0, 1) == row_id

        def tile(t):
            return slice(t * LANES, (t + 1) * LANES)

        def rows(t):
            return slice(t * ROWS, (t + 1) * ROWS)

        def mm(a, b_):
            return jnp.dot(a, b_, preferred_element_type=F32)[0:ROWS]

        def q_proj(i, b):
            for c in range(KQ):
                qp[b][rows(c)] = mm(_unpack(xnpk[:, tile(c)]), wqb[i, tile(c), :])

        def qk(i, b, cs=range(KP)):
            for c in cs:
                sp[b][rows(c)] = mm(_unpack(qpk[b][:, tile(c)]), kb[i, rows(c)].reshape(LANES, W))

        def nt(a, b_):
            return lax.dot_general(a, b_, NT_DIMS, preferred_element_type=F32)

        def combine_parts(i, b, acc_ref, xn=XN):
            acc = jnp.concatenate([acc_ref[:, tile(k)] for k in range(NB)], axis=0)
            parts = [nt(_unpack(gpk[b][:, tile(0)]), _unpack(acc))]
            for t in range(xn):
                w = jnp.concatenate([vbuf[i, c * CB:(c + 1) * CB, :, tile(t)].reshape(LANES // 2, LANES)
                                     for c in range(min(KP, XU - t * KP))], axis=1)
                parts.append(jnp.dot(_unpack(gpk[b][:, tile(1 + t)]), _unpack(w),
                                     preferred_element_type=F32))
            return parts

        def combine(i, b):
            for k, part in enumerate(combine_parts(i, b, accb[b])):
                oraw[b][k * PROWS:(k + 1) * PROWS, 0:part.shape[1]] = part

        def o_proj(i0, b):
            for k in range(ND):
                for c in range(KP):
                    op[b][rows(k * KP + c)] = mm(_unpack(opk[i0 + k, :, tile(c)]), wob[i0 + k, tile(c), :])

        def row_max(b):
            st[b][:, tile(2)] = jnp.broadcast_to(
                jnp.max(st[b][:, tile(0)], axis=1, keepdims=True), (ROWS, LANES))

        def row_sum(b):
            return jnp.broadcast_to(jnp.sum(gl[b][...], axis=1, keepdims=True), (PROWS, LANES))

        def sum_rows(ref, n, cols=slice(None), off=0):
            s = ref[rows(off), cols]
            for c in range(1, n):
                s = s + ref[rows(off + c), cols]
            return s

        def q_pack(b):
            qpk[b][...] = _pack(jnp.where(diag, sum_rows(qp[b], KQ), 0.0))

        def row(ref, r, cols=slice(None)):
            v = ref[r:r + 1, cols]
            return jnp.broadcast_to(v, (ROWS, v.shape[1]))

        def lane_weights(b, xn=XN):
            g = []
            for r in range(2):
                g.append(_round_bf16(jnp.exp2((row(st[b], r, tile(0)) - row(st[b], r, tile(2))) * scale[...])))
                gl[b][rows(r)] = g[r] * row(st[b], r, tile(1))
            gpk[b][:, tile(0)] = _pack(g[0], g[1])
            for t in range(xn):
                gpk[b][:, tile(1 + t)] = _pack(g[0] * row(p[b], 0, tile(t)), g[1] * row(p[b], 1, tile(t)))

        def normalise(parts, dn):
            o = parts[0]
            for part in parts[1:]:
                n = part.shape[1]
                o = o + part if n == PD else jnp.concatenate([o[:, :n] + part, o[:, n:]], axis=1)
            o = o * jnp.concatenate([1.0 / dn] * KP, axis=1)
            return _pack(jnp.where(first_head, o[0:ROWS], o[ROWS:PROWS]))

        def stored_parts(b):
            return [oraw[b][k * PROWS:(k + 1) * PROWS, 0:min(KP, XU - (k - 1) * KP) * LANES]
                    for k in range(1 + XN)]

        def o_pack(i, b):
            opk[i] = normalise(stored_parts(b), den[b][...])

        def softmax_steps(b):
            NC = 4

            def tree(f, xs):
                while len(xs) > 1:
                    xs = [f(xs[k], xs[k + 1]) for k in range(0, len(xs), 2)]
                return xs[0]

            mc = [None] * NC
            for t in range(NT):
                s = sum_rows(sp[b], KP, tile(t))
                sp[b][rows(0), tile(t)] = s
                mc[t % NC] = s if t < NC else jnp.maximum(mc[t % NC], s)
                yield
            mm_ = tree(jnp.maximum, mc)
            st[b][:, tile(0)] = mm_
            lc = [None] * NC
            sc = scale[...]
            for t in range(NT):
                e = jnp.exp2((sp[b][rows(0), tile(t)] - mm_) * sc)
                p[b][:, tile(t)] = e
                lc[t % NC] = e if t < NC else lc[t % NC] + e
                if t == NT - 1:
                    st[b][:, tile(1)] = tree(jnp.add, lc)
                yield

        def pv_steps(i, b, first, xn, xt, lo_ref):
            HB = HW // DB
            for j in range(2):
                for db in range(DB):
                    ng = HB // G
                    col = (j * HW + db * HB) // ROWS // CB
                    assert col == ((j * HW + (db + 1) * HB) // ROWS - 1) // CB
                    t0 = len(range(col, XU, KP)) if xn else 0
                    order = sorted(range(t0, NT),
                                   key=lambda t: ((t - t0 + 0.5) / (NT - xt - t0) if t < NT - xt
                                                  else (t - (NT - xt) + 0.5) / xt))
                    acc = [None] * ng
                    for pos, t in enumerate(order):
                        pb = p[b][j:j + 1, tile(t)]
                        for g in range(ng):
                            b0 = (j * HW + db * HB + g * G) // ROWS
                            bands = slice(b0, b0 + G // ROWS)
                            u = vbuf[i, bands, :, tile(t)]
                            if t < NT - xt or first:
                                lo, hi = _split(u)
                                if t >= NT - xt:
                                    vbuf[i, bands, :, tile(t)] = hi
                                    lo_ref[bands, :, tile(t - (NT - xt))] = lo
                            else:
                                lo = lo_ref[bands, :, tile(t - (NT - xt))]
                                hi = u
                            term = pltpu.bitcast(jnp.concatenate([lo, hi], axis=1), F32) * pb
                            acc[g] = term if pos == 0 else acc[g] + term
                            if pos == len(order) - 1:
                                for k in range(G // ROWS):
                                    acca[b][:, tile(b0 + k)] = pltpu.bitcast(
                                        acc[g][k].astype(BF16), U32)
                        yield

        def step(j, b, first, left):
            nb = 1 - b
            xn = XN if left is None else 0
            extra = [lambda: lane_weights(nb, 0 if left == 1 else XN),
                     lambda: o_pack(jnp.maximum(j - 3, 0), nb)]

            def copy_acc():
                accb[nb][...] = acca[nb][...]
            extra.append(copy_acc)
            if left is None:
                extra.append(lambda: q_pack(nb))
            if first and xn:
                def transpose_v():
                    for u_ in range(XU):
                        blk = (j, slice(u_ % KP * CB, (u_ % KP + 1) * CB), slice(None), tile(u_ // KP))
                        v32 = jnp.concatenate(_split(vbuf[blk]), axis=1)
                        v32 = pltpu.bitcast(v32, F32).reshape(LANES, LANES)
                        w = pltpu.bitcast(v32.T.astype(BF16), U32)
                        vbuf[blk] = w.reshape(CB, ROWS, LANES)
                extra.append(transpose_v)
            if left == 1:
                for k in range(ND):
                    def acc_op(k=k):
                        s_ = sum_rows(op[nb], KP, off=k * KP)
                        att[...] = s_ if k == 0 else att[...] + s_
                    extra.append(acc_op)
            if left != 1:
                sm = softmax_steps(nb)
                extra += [lambda: next(sm)] * (2 * NT)
            nsteps = 2 * DB * NT - (XU * 2 * DB // KP if xn else 0)
            done = 0
            for k, _ in enumerate(pv_steps(j, b, first, xn, *(
                    (XT, vlo.at[j]) if left is None else (XT2, vlo2.at[2 - left])))):
                upto = (k + 1) * len(extra) // nsteps
                for f in extra[done:upto]:
                    f()
                done = upto
            assert done == len(extra)
            if left is None:
                qk(j + 2, b)
            combine(jnp.maximum(j - 2, 0), b)
            if left is None:
                q_proj(jnp.minimum(j + 4, NP - 1), b)
            else:
                o_proj((2 - left) * ND, b)
            row_max(b)
            den[b][...] = row_sum(b)

        def attention(x, first):
            mean, rstd = _ln_stats(x)
            xnpk[...] = _pack(x - mean)
            scale[...] = jnp.broadcast_to(rstd * exp2_scale, (ROWS, LANES))
            for ref in (p[1].at[:, 0:max(XN, 1) * LANES], gpk[0], accb[0], acca[1], oraw[1]):
                ref[...] = jnp.zeros(ref.shape, ref.dtype)
            for ref in (st[1], gl[0], den[1]):
                ref[...] = jnp.ones(ref.shape, ref.dtype)
            if first:
                for cp in wq_cps:
                    cp.wait()
            qpk[0][...] = _pack(jnp.where(diag, _centered_dot(x, mean, wqb[0]), 0.0))
            if first:
                for cp in k0_cps:
                    cp.wait()
            qk(0, 0, (0,))
            q_proj(1, 1)
            q_pack(1)
            qk(0, 0, range(1, KP))
            qk(1, 1)
            q_proj(2, 0)
            q_pack(0)
            q_proj(3, 1)
            for _ in softmax_steps(0):
                pass
            if first:
                wo_cp.wait()

                def reorder_wo(i, carry):
                    for band in range(NB):
                        wobuf[i, rows(band)] = _deinterleave(wobuf[i, rows(band)])
                    return carry
                lax.fori_loop(0, NP, reorder_wo, 0)

            def body(j, carry):
                if first:
                    @pl.when(j < NP - 2)
                    def _():
                        for cp in group_copies(j, True):
                            cp.wait()

                    @pl.when(j >= NP - 2)
                    def _():
                        for cp in group_copies(j, False):
                            cp.wait()

                    @pl.when(j + NRING < NP - 2)
                    def _():
                        for cp in group_copies(j + NRING, True):
                            cp.start()

                    @pl.when(jnp.logical_and(j + NRING >= NP - 2, j + NRING < NP))
                    def _():
                        for cp in group_copies(j + NRING, False):
                            cp.start()

                    @pl.when(j + NRING == NP - 1)
                    def _():
                        w1_cp.start()
                        for cp in w2_cps:
                            cp.start()

                for b in range(2):
                    @pl.when(jnp.logical_and((j & 1) == b, j < NP - 2))
                    def _():
                        step(j, b, first, None)

                for left in (2, 1):
                    @pl.when(j == NP - left)
                    def _():
                        step(NP - left, (NP - left) % 2, first, left)
                return carry

            lax.fori_loop(0, NP, body, 0)

            lane_weights(1, 0)
            o2 = combine_parts(NP - 2, 0, accb[0], 0)
            o1 = combine_parts(NP - 1, 1, acca[1], 0)
            a = att[...] + sum_rows(op[1], ND * KP)
            a = a + mm(_unpack(opk[NP - 4]), wob[NP - 4])
            a = a + mm(_unpack(normalise(stored_parts(1), den[1][...])), wob[NP - 3])
            a = a + mm(_unpack(normalise(o2, row_sum(0))), wob[NP - 2])
            a = a + mm(_unpack(normalise(o1, row_sum(1))), wob[NP - 1])
            return _round_bf16(x + _round_bf16(a))

        def ffn(x, first):
            mean, rstd = _ln_stats(x)
            if first:
                w1_cp.wait()
            b1 = b1buf[...].reshape(1, FF).astype(F32)
            b2 = b2buf[...].reshape(1, D).astype(F32)
            h = _centered_dot(x, mean, w1b[...]) * rstd
            h = _round_bf16(_round_bf16(h) + b1)
            h = _gelu_tanh(h).astype(BF16)
            y = None
            for c in range(W2C):
                if first:
                    w2_cps[c].wait()
                yc = jnp.dot(h[:, W2B[c]:W2B[c + 1]], w2b[W2B[c]:W2B[c + 1], :],
                             preferred_element_type=F32)
                y = yc if y is None else y + yc
            y = _round_bf16(_round_bf16(y) + b2)
            return _round_bf16(x + y)

        for cp in small:
            cp.wait()
        x = jnp.broadcast_to(xbuf[0].astype(F32), (ROWS, D))
        x = attention(x, True)
        x = ffn(x, True)
        x = attention(x, False)
        x = ffn(x, False)
        o_ref[0] = x[0:1].astype(o_ref.dtype)

    any_spec = pl.BlockSpec(memory_space=pl.ANY)
    return pl.pallas_call(
        kernel,
        out_shape=jax.ShapeDtypeStruct((B, SQ, D), A_x.dtype),
        in_specs=[any_spec] * 9,
        out_specs=pl.BlockSpec(memory_space=pltpu.VMEM),
        scratch_shapes=[
            pltpu.VMEM((NP, NB, ROWS, W), U32),
            pltpu.VMEM((NP, NB, ROWS, W), U32),
            pltpu.VMEM((NP, D // 2, PD), U32),
            pltpu.VMEM((NP, DH, D), U32),
            pltpu.VMEM((D // 2, FF), U32),
            pltpu.VMEM((FF // 2, D), U32),
            pltpu.VMEM((B, SQ, D), BF16),
            pltpu.VMEM((FF,), BF16),
            pltpu.VMEM((D,), BF16),
            pltpu.VMEM((ROWS, D), U32),
            pltpu.VMEM((ROWS, D), F32),
            pltpu.VMEM((NP, ROWS, PD), U32),
            pltpu.VMEM((ROWS, LANES), F32),
            pltpu.VMEM((NP - 2, NB, ROWS, max(XT, 1) * LANES), U32),
            pltpu.VMEM((2, NB, ROWS, max(XT2, 1) * LANES), U32),
            pltpu.SemaphoreType.DMA((5 + W2C + NRING,)),
        ] + [pltpu.VMEM(*pingpong[n]) for n in names for _ in range(2)],
        compiler_params=pltpu.CompilerParams(vmem_limit_bytes=511 * 256 * 1024),
    )(A_x, kt, vt, A_wq, wo3, B_w1, B_b1, B_w2, B_b2)
```

```python
import math

import jax
import jax.numpy as jnp
from jax import lax
import jax.experimental.pallas as pl
import jax.experimental.pallas.tpu as pltpu

F32 = jnp.float32
BF16 = jnp.bfloat16
U32 = jnp.uint32

LANES = 128
ROWS = 8
PROWS = 16
NT_DIMS = (((1,), (1,)), ((), ()))


def _ln_stats(x, eps=1e-5):
    m = jnp.mean(x, axis=-1, keepdims=True)
    c = x - m
    v = jnp.mean(c * c, axis=-1, keepdims=True)
    return m, 1.0 / jnp.sqrt(v + eps)


def _centered_dot(x, m, w):
    lhs = jnp.concatenate([x, jnp.ones_like(x)], axis=0).astype(BF16)
    y = jnp.dot(lhs, w, preferred_element_type=F32)
    return y[0:ROWS] - m * y[ROWS:PROWS]


def _round_bf16(x):
    return x.astype(BF16).astype(F32)


def _gelu_tanh(x):
    c = math.sqrt(2.0 / math.pi)
    return 0.5 * x * (1.0 + jnp.tanh(c * (x + 0.044715 * (x * x * x))))


def _pack(x, y=None):
    y = jnp.zeros_like(x) if y is None else y
    return pltpu.bitcast(jnp.concatenate([x, y], axis=0).astype(BF16), U32)


def _unpack(u):
    return pltpu.bitcast(u, BF16)


def _split(u):
    return u << 16, u & U32(0xFFFF0000)


def _deinterleave(u):
    rows16 = pltpu.bitcast(jnp.concatenate(_split(u), axis=0), F32)
    return pltpu.bitcast(rows16.astype(BF16), U32)


@jax.jit
def pallas_interleave_layers__sliding_block_cached__dense_activation_gelu__decode_kernel(
    A_x: jax.Array,
    A_k_cache: jax.Array,
    A_v_cache: jax.Array,
    A_wq: jax.Array,
    A_wo: jax.Array,
    B_x: jax.Array,
    B_w1: jax.Array,
    B_b1: jax.Array,
    B_w2: jax.Array,
    B_b2: jax.Array,
):
    B, SQ, D = A_x.shape
    _, H, SK, DH = A_k_cache.shape
    FF = B_w1.shape[1]
    assert B == 1 and SQ == 1 and A_wq.shape[1] == H * DH and H % 4 == 0
    W = min(4096, max(256, SK // 4))
    NP = H // 2
    PD = 2 * DH
    HW = DH // 2
    NT = W // LANES
    KQ = D // LANES
    KP = PD // LANES
    W2B = [0, FF - 4 * LANES, FF - LANES, FF]
    W2C = len(W2B) - 1
    XT = 3
    XT2 = 16
    XU = 9
    XN = -(-XU // KP)
    CB = LANES // PROWS
    ND = (NP - 4) // 2
    G = 2 * ROWS
    DB = 3
    NRING = 3
    exp2_scale = float(DH) ** -0.5 * math.log2(math.e)

    NB = PD // PROWS
    kt = jnp.transpose(A_k_cache, (0, 1, 3, 2)).reshape(NP, NB, 2, ROWS, SK)
    vt = jnp.transpose(A_v_cache, (0, 1, 3, 2)).reshape(NP, NB, 2, ROWS, SK)
    wo3 = A_wo.reshape(NP, PD, D)

    pingpong = dict(
        qp=((KQ * ROWS, PD), F32),
        qpk=((ROWS, PD), U32),
        sp=((KP * ROWS, W), F32),
        p=((ROWS, W), F32),
        st=((ROWS, 3 * LANES), F32),
        gl=((PROWS, LANES), F32),
        den=((PROWS, LANES), F32),
        acca=((ROWS, NB * LANES), U32),
        accb=((LANES // 2, PD), U32),
        gpk=((ROWS, (1 + max(XN, 1)) * LANES), U32),
        oraw=(((1 + XN) * PROWS, PD), F32),
        op=((ND * KP * ROWS, D), F32),
    )
    names = list(pingpong)

    def kernel(x_hbm, k_hbm, v_hbm, wq_hbm, wo_hbm, w1_hbm, b1_hbm, w2_hbm, b2_hbm,
               o_ref,
               kbuf, vbuf, wqbuf, wobuf, w1buf, w2buf, xnpk, att, opk, scale, vlo, vlo2, sems, *pp):
        xbuf, b1buf, b2buf = pp[-3:]
        bufs = {n: (pp[2 * k], pp[2 * k + 1]) for k, n in enumerate(names)}
        qp, qpk, sp, p, st, gl, den, acca, accb, gpk, oraw, op = (bufs[n] for n in names)
        kb = kbuf.bitcast(BF16)
        vb = vbuf.bitcast(BF16)
        wqb = wqbuf.bitcast(BF16)
        wob = wobuf.bitcast(BF16)
        w1b = w1buf.bitcast(BF16)
        w2b = w2buf.bitcast(BF16)

        S_SMALL, S_WQ, S_K0, S_WO, S_RING = 0, 1, 2, 3, 4
        S_W1, S_W2 = 0, 1
        assert S_W2 + W2C <= S_RING

        def window_copies(hbm, buf, start, n, sem):
            return [pltpu.make_async_copy(
                hbm.at[pl.ds(start, n), :, h, :, pl.ds(SK - W, W)],
                buf.at[pl.ds(start, n), :, pl.ds(h * ROWS, ROWS), :], sem) for h in range(2)]

        def group_copies(j, with_k):
            sem = sems.at[S_RING + j % NRING]
            return ((window_copies(k_hbm, kb, j + 2, 1, sem) if with_k else [])
                    + window_copies(v_hbm, vb, j, 1, sem))

        small = [pltpu.make_async_copy(x_hbm, xbuf, sems.at[S_SMALL]),
                 pltpu.make_async_copy(b1_hbm, b1buf, sems.at[S_SMALL]),
                 pltpu.make_async_copy(b2_hbm, b2buf, sems.at[S_SMALL])]
        wq_cps = [pltpu.make_async_copy(wq_hbm.at[:, i * PD:(i + 1) * PD], wqb.at[i], sems.at[S_WQ])
                  for i in range(NP)]
        k0_cps = window_copies(k_hbm, kb, 0, 2, sems.at[S_K0])
        wo_cp = pltpu.make_async_copy(wo_hbm, wob, sems.at[S_WO])
        w1_cp = pltpu.make_async_copy(w1_hbm, w1b, sems.at[S_W1])
        w2_cps = [pltpu.make_async_copy(w2_hbm.at[W2B[c]:W2B[c + 1]], w2b.at[W2B[c]:W2B[c + 1]],
                                        sems.at[S_W2 + c]) for c in range(W2C)]

        for cp in wq_cps:
            cp.start()
        for cp in small:
            cp.start()
        for cp in k0_cps:
            cp.start()
        wo_cp.start()
        for j in range(NRING):
            for cp in group_copies(j, True):
                cp.start()

        row_id = lax.broadcasted_iota(jnp.int32, (ROWS, PD), 0)
        col = lax.broadcasted_iota(jnp.int32, (ROWS, PD), 1)
        first_head = col < DH
        diag = jnp.where(first_head, 0, 1) == row_id

        def tile(t):
            return slice(t * LANES, (t + 1) * LANES)

        def rows(t):
            return slice(t * ROWS, (t + 1) * ROWS)

        def mm(a, b_):
            return jnp.dot(a, b_, preferred_element_type=F32)[0:ROWS]

        def q_proj(i, b):
            for c in range(KQ):
                qp[b][rows(c)] = mm(_unpack(xnpk[:, tile(c)]), wqb[i, tile(c), :])

        def qk(i, b, cs=range(KP)):
            for c in cs:
                sp[b][rows(c)] = mm(_unpack(qpk[b][:, tile(c)]), kb[i, rows(c)].reshape(LANES, W))

        def nt(a, b_):
            return lax.dot_general(a, b_, NT_DIMS, preferred_element_type=F32)

        def packed_acc(b):
            return _unpack(jnp.concatenate([acca[b][:, tile(k)] for k in range(NB)], axis=0))

        def combine_parts(i, b, xn=XN, transposed=True):
            g = _unpack(gpk[b][:, tile(0)])
            parts = [jnp.dot(g, _unpack(accb[b][...]), preferred_element_type=F32) if transposed
                     else nt(g, packed_acc(b))]
            for t in range(xn):
                w = jnp.concatenate([vbuf[i, c * CB:(c + 1) * CB, :, tile(t)].reshape(LANES // 2, LANES)
                                     for c in range(min(KP, XU - t * KP))], axis=1)
                parts.append(jnp.dot(_unpack(gpk[b][:, tile(1 + t)]), _unpack(w),
                                     preferred_element_type=F32))
            return parts

        def combine(i, b):
            for k, part in enumerate(combine_parts(i, b)):
                oraw[b][k * PROWS:(k + 1) * PROWS, 0:part.shape[1]] = part

        def o_proj(i0, b):
            for k in range(ND):
                for c in range(KP):
                    op[b][rows(k * KP + c)] = mm(_unpack(opk[i0 + k, :, tile(c)]), wob[i0 + k, tile(c), :])

        def row_max(b):
            st[b][:, tile(2)] = jnp.broadcast_to(
                jnp.max(st[b][:, tile(0)], axis=1, keepdims=True), (ROWS, LANES))

        def row_sum(b):
            return jnp.broadcast_to(jnp.sum(gl[b][...], axis=1, keepdims=True), (PROWS, LANES))

        def sum_rows(ref, n, cols=slice(None), off=0):
            s = ref[rows(off), cols]
            for c in range(1, n):
                s = s + ref[rows(off + c), cols]
            return s

        def q_pack(b):
            qpk[b][...] = _pack(jnp.where(diag, sum_rows(qp[b], KQ), 0.0))

        def row(ref, r, cols=slice(None)):
            v = ref[r:r + 1, cols]
            return jnp.broadcast_to(v, (ROWS, v.shape[1]))

        def lane_weights(b, xn=XN):
            g = []
            for r in range(2):
                g.append(_round_bf16(jnp.exp2((row(st[b], r, tile(0)) - row(st[b], r, tile(2))) * scale[...])))
                gl[b][rows(r)] = g[r] * row(st[b], r, tile(1))
            gpk[b][:, tile(0)] = _pack(g[0], g[1])
            for t in range(xn):
                gpk[b][:, tile(1 + t)] = _pack(g[0] * row(p[b], 0, tile(t)), g[1] * row(p[b], 1, tile(t)))

        def normalise(parts, dn):
            o = parts[0]
            for part in parts[1:]:
                n = part.shape[1]
                o = o + part if n == PD else jnp.concatenate([o[:, :n] + part, o[:, n:]], axis=1)
            o = o * jnp.concatenate([1.0 / dn] * KP, axis=1)
            return _pack(jnp.where(first_head, o[0:ROWS], o[ROWS:PROWS]))

        def stored_parts(b):
            return [oraw[b][k * PROWS:(k + 1) * PROWS, 0:min(KP, XU - (k - 1) * KP) * LANES]
                    for k in range(1 + XN)]

        def o_pack(i, b):
            opk[i] = normalise(stored_parts(b), den[b][...])

        def softmax_steps(b):
            NC = 4

            def tree(f, xs):
                while len(xs) > 1:
                    xs = [f(xs[k], xs[k + 1]) for k in range(0, len(xs), 2)]
                return xs[0]

            mc = [None] * NC
            for t in range(NT):
                s = sum_rows(sp[b], KP, tile(t))
                sp[b][rows(0), tile(t)] = s
                mc[t % NC] = s if t < NC else jnp.maximum(mc[t % NC], s)
                yield
            mm_ = tree(jnp.maximum, mc)
            st[b][:, tile(0)] = mm_
            lc = [None] * NC
            sc = scale[...]
            for t in range(NT):
                e = jnp.exp2((sp[b][rows(0), tile(t)] - mm_) * sc)
                p[b][:, tile(t)] = e
                lc[t % NC] = e if t < NC else lc[t % NC] + e
                if t == NT - 1:
                    st[b][:, tile(1)] = tree(jnp.add, lc)
                yield

        def pv_steps(i, b, first, xn, xt, lo_ref):
            HB = HW // DB
            for j in range(2):
                for db in range(DB):
                    ng = HB // G
                    col = (j * HW + db * HB) // ROWS // CB
                    assert XU % KP == 0 or col == ((j * HW + (db + 1) * HB) // ROWS - 1) // CB
                    t0 = len(range(col, XU, KP)) if xn else 0
                    order = sorted(range(t0, NT),
                                   key=lambda t: ((t - t0 + 0.5) / (NT - xt - t0) if t < NT - xt
                                                  else (t - (NT - xt) + 0.5) / xt))
                    acc = [None] * ng
                    for pos, t in enumerate(order):
                        pb = p[b][j:j + 1, tile(t)]
                        for g in range(ng):
                            b0 = (j * HW + db * HB + g * G) // ROWS
                            bands = slice(b0, b0 + G // ROWS)
                            u = vbuf[i, bands, :, tile(t)]
                            if t < NT - xt or first:
                                lo, hi = _split(u)
                                if t >= NT - xt:
                                    vbuf[i, bands, :, tile(t)] = hi
                                    lo_ref[bands, :, tile(t - (NT - xt))] = lo
                            else:
                                lo = lo_ref[bands, :, tile(t - (NT - xt))]
                                hi = u
                            term = pltpu.bitcast(jnp.concatenate([lo, hi], axis=1), F32) * pb
                            acc[g] = term if pos == 0 else acc[g] + term
                            if pos == len(order) - 1:
                                for k in range(G // ROWS):
                                    acca[b][:, tile(b0 + k)] = pltpu.bitcast(
                                        acc[g][k].astype(BF16), U32)
                        yield

        def step(j, b, first, left):
            nb = 1 - b
            xn = XN if left is None else 0
            extra = [lambda: lane_weights(nb, 0 if left == 1 else XN),
                     lambda: o_pack(jnp.maximum(j - 3, 0), nb)]

            if left is None:
                extra.append(lambda: q_pack(nb))
            if first and xn:
                def transpose_v():
                    for u_ in range(XU):
                        blk = (j, slice(u_ % KP * CB, (u_ % KP + 1) * CB), slice(None), tile(u_ // KP))
                        v32 = pltpu.bitcast(jnp.concatenate(_split(vbuf[blk]), axis=1), F32)
                        w = pltpu.bitcast(v32.reshape(LANES, LANES).astype(BF16).T, U32)
                        vbuf[blk] = w.reshape(CB, ROWS, LANES)
                extra.append(transpose_v)
            if left == 1:
                for k in range(ND):
                    def acc_op(k=k):
                        s_ = sum_rows(op[nb], KP, off=k * KP)
                        att[...] = s_ if k == 0 else att[...] + s_
                    extra.append(acc_op)
            if left != 1:
                sm = softmax_steps(nb)
                extra += [lambda: next(sm)] * (2 * NT)
            nsteps = 2 * DB * NT - (XU * 2 * DB // KP if xn else 0)
            done = 0
            for k, _ in enumerate(pv_steps(j, b, first, xn, *(
                    (XT, vlo.at[j]) if left is None else (XT2, vlo2.at[2 - left])))):
                upto = (k + 1) * len(extra) // nsteps
                for f in extra[done:upto]:
                    f()
                done = upto
            assert done == len(extra)
            if left is None:
                qk(j + 2, b)
            combine(jnp.maximum(j - 2, 0), b)
            if left is None:
                q_proj(jnp.minimum(j + 4, NP - 1), b)
            else:
                o_proj((2 - left) * ND, b)
            accb[nb][...] = pltpu.bitcast(packed_acc(nb).T, U32)
            row_max(b)
            den[b][...] = row_sum(b)

        def attention(x, first):
            mean, rstd = _ln_stats(x)
            xnpk[...] = _pack(x - mean)
            scale[...] = jnp.broadcast_to(rstd * exp2_scale, (ROWS, LANES))
            for ref in (p[1].at[:, 0:max(XN, 1) * LANES], gpk[0], accb[0], acca[1], oraw[1]):
                ref[...] = jnp.zeros(ref.shape, ref.dtype)
            for ref in (st[1], gl[0], den[1]):
                ref[...] = jnp.ones(ref.shape, ref.dtype)
            if first:
                for cp in wq_cps:
                    cp.wait()
            qpk[0][...] = _pack(jnp.where(diag, _centered_dot(x, mean, wqb[0]), 0.0))
            if first:
                for cp in k0_cps:
                    cp.wait()
            qk(0, 0, (0,))
            q_proj(1, 1)
            q_pack(1)
            qk(0, 0, range(1, KP))
            qk(1, 1)
            q_proj(2, 0)
            q_pack(0)
            q_proj(3, 1)
            for _ in softmax_steps(0):
                pass
            if first:
                wo_cp.wait()

                def reorder_wo(i, carry):
                    for band in range(NB):
                        wobuf[i, rows(band)] = _deinterleave(wobuf[i, rows(band)])
                    return carry
                lax.fori_loop(0, NP, reorder_wo, 0)

            def stream(j):
                if not first:
                    return
                if isinstance(j, int):
                    for cp in group_copies(j, False):
                        cp.wait()
                    return
                for cp in group_copies(j, True):
                    cp.wait()

                @pl.when(j + NRING < NP - 2)
                def _():
                    for cp in group_copies(j + NRING, True):
                        cp.start()

                @pl.when(jnp.logical_and(j + NRING >= NP - 2, j + NRING < NP))
                def _():
                    for cp in group_copies(j + NRING, False):
                        cp.start()

                @pl.when(j + NRING == NP - 1)
                def _():
                    w1_cp.start()
                    for cp in w2_cps:
                        cp.start()

            def body(_, j):
                for b in range(2):
                    stream(j + b)

                    @pl.when(((j + b) & 1) == b)
                    def _():
                        step(j + b, b, first, None)
                return j + 2

            j_end = lax.fori_loop(0, NP // 2 - 1, body, 0)
            for left in (2, 1):
                stream(NP - left)

                @pl.when(j_end + (2 - left) == NP - left)
                def _():
                    step(NP - left, (NP - left) % 2, first, left)

            lane_weights(1, 0)
            o2 = combine_parts(NP - 2, 0, 0)
            o1 = combine_parts(NP - 1, 1, 0, transposed=False)
            a = att[...] + sum_rows(op[1], ND * KP)
            a = a + mm(_unpack(opk[NP - 4]), wob[NP - 4])
            a = a + mm(_unpack(normalise(stored_parts(1), den[1][...])), wob[NP - 3])
            a = a + mm(_unpack(normalise(o2, row_sum(0))), wob[NP - 2])
            a = a + mm(_unpack(normalise(o1, row_sum(1))), wob[NP - 1])
            return _round_bf16(x + _round_bf16(a))

        def ffn(x, first):
            mean, rstd = _ln_stats(x)
            if first:
                w1_cp.wait()
            b1 = b1buf[...].reshape(1, FF).astype(F32)
            b2 = b2buf[...].reshape(1, D).astype(F32)
            h = _centered_dot(x, mean, w1b[...]) * rstd
            h = _round_bf16(_round_bf16(h) + b1)
            h = _gelu_tanh(h).astype(BF16)
            y = None
            for c in range(W2C):
                if first:
                    w2_cps[c].wait()
                yc = jnp.dot(h[:, W2B[c]:W2B[c + 1]], w2b[W2B[c]:W2B[c + 1], :],
                             preferred_element_type=F32)
                y = yc if y is None else y + yc
            y = _round_bf16(_round_bf16(y) + b2)
            return _round_bf16(x + y)

        for cp in small:
            cp.wait()
        x = jnp.broadcast_to(xbuf[0].astype(F32), (ROWS, D))
        x = attention(x, True)
        x = ffn(x, True)
        x = attention(x, False)
        x = ffn(x, False)
        o_ref[0] = x[0:1].astype(o_ref.dtype)

    any_spec = pl.BlockSpec(memory_space=pl.ANY)
    return pl.pallas_call(
        kernel,
        out_shape=jax.ShapeDtypeStruct((B, SQ, D), A_x.dtype),
        in_specs=[any_spec] * 9,
        out_specs=pl.BlockSpec(memory_space=pltpu.VMEM),
        scratch_shapes=[
            pltpu.VMEM((NP, NB, ROWS, W), U32),
            pltpu.VMEM((NP, NB, ROWS, W), U32),
            pltpu.VMEM((NP, D // 2, PD), U32),
            pltpu.VMEM((NP, DH, D), U32),
            pltpu.VMEM((D // 2, FF), U32),
            pltpu.VMEM((FF // 2, D), U32),
            pltpu.VMEM((ROWS, D), U32),
            pltpu.VMEM((ROWS, D), F32),
            pltpu.VMEM((NP, ROWS, PD), U32),
            pltpu.VMEM((ROWS, LANES), F32),
            pltpu.VMEM((NP - 2, NB, ROWS, max(XT, 1) * LANES), U32),
            pltpu.VMEM((2, NB, ROWS, max(XT2, 1) * LANES), U32),
            pltpu.SemaphoreType.DMA((4 + NRING,)),
        ] + [pltpu.VMEM(*pingpong[n]) for n in names for _ in range(2)] + [
            pltpu.VMEM((B, SQ, D), BF16),
            pltpu.VMEM((FF,), BF16),
            pltpu.VMEM((D,), BF16),
        ],
        compiler_params=pltpu.CompilerParams(vmem_limit_bytes=511 * 256 * 1024),
    )(A_x, kt, vt, A_wq, wo3, B_w1, B_b1, B_w2, B_b2)
```

```python
import math

import jax
import jax.numpy as jnp
from jax import lax
import jax.experimental.pallas as pl
import jax.experimental.pallas.tpu as pltpu

F32 = jnp.float32
BF16 = jnp.bfloat16
U32 = jnp.uint32

LANES = 128
ROWS = 8
PROWS = 16
NT_DIMS = (((1,), (1,)), ((), ()))


def _ln_stats(x, eps=1e-5):
    m = jnp.mean(x, axis=-1, keepdims=True)
    c = x - m
    v = jnp.mean(c * c, axis=-1, keepdims=True)
    return m, 1.0 / jnp.sqrt(v + eps)


def _centered_dot(x, m, w):
    lhs = jnp.concatenate([x, jnp.ones_like(x)], axis=0).astype(BF16)
    y = jnp.dot(lhs, w, preferred_element_type=F32)
    return y[0:ROWS] - m * y[ROWS:PROWS]


def _round_bf16(x):
    return x.astype(BF16).astype(F32)


def _gelu_tanh(x):
    c = math.sqrt(2.0 / math.pi)
    return 0.5 * x * (1.0 + jnp.tanh(c * (x + 0.044715 * (x * x * x))))


def _pack(x, y=None):
    y = jnp.zeros_like(x) if y is None else y
    return pltpu.bitcast(jnp.concatenate([x, y], axis=0).astype(BF16), U32)


def _unpack(u):
    return pltpu.bitcast(u, BF16)


def _split(u):
    return u << 16, u & U32(0xFFFF0000)


def _deinterleave(u):
    rows16 = pltpu.bitcast(jnp.concatenate(_split(u), axis=0), F32)
    return pltpu.bitcast(rows16.astype(BF16), U32)


@jax.jit
def pallas_interleave_layers__sliding_block_cached__dense_activation_gelu__decode_kernel(
    A_x: jax.Array,
    A_k_cache: jax.Array,
    A_v_cache: jax.Array,
    A_wq: jax.Array,
    A_wo: jax.Array,
    B_x: jax.Array,
    B_w1: jax.Array,
    B_b1: jax.Array,
    B_w2: jax.Array,
    B_b2: jax.Array,
):
    B, SQ, D = A_x.shape
    _, H, SK, DH = A_k_cache.shape
    FF = B_w1.shape[1]
    assert B == 1 and SQ == 1 and A_wq.shape[1] == H * DH and H % 4 == 0
    W = min(4096, max(256, SK // 4))
    NP = H // 2
    PD = 2 * DH
    HW = DH // 2
    NT = W // LANES
    KQ = D // LANES
    KP = PD // LANES
    W2B = [0, FF - 8 * LANES, FF - 4 * LANES, FF - LANES, FF]
    W2C = len(W2B) - 1
    XT = 3
    XT2 = 16
    XU = 9
    XN = -(-XU // KP)
    CB = LANES // PROWS
    ND = (NP - 4) // 2
    G = 2 * ROWS
    DB = 3
    NRING = 3
    exp2_scale = float(DH) ** -0.5 * math.log2(math.e)

    NB = PD // PROWS
    kt = jnp.transpose(A_k_cache, (0, 1, 3, 2)).reshape(NP, NB, 2, ROWS, SK)
    vt = jnp.transpose(A_v_cache, (0, 1, 3, 2)).reshape(NP, NB, 2, ROWS, SK)
    wo3 = A_wo.reshape(NP, PD, D)

    pingpong = dict(
        qp=((KQ * ROWS, PD), F32),
        qpk=((ROWS, PD), U32),
        sp=((KP * ROWS, W), F32),
        p=((ROWS, W), F32),
        st=((ROWS, 3 * LANES), F32),
        gl=((PROWS, LANES), F32),
        den=((PROWS, LANES), F32),
        acca=((ROWS, NB * LANES), U32),
        accb=((LANES // 2, PD), U32),
        gpk=((ROWS, (1 + max(XN, 1)) * LANES), U32),
        oraw=(((1 + XN) * PROWS, PD), F32),
        op=((ND * KP * ROWS, D), F32),
    )
    names = list(pingpong)

    def kernel(x_hbm, k_hbm, v_hbm, wq_hbm, wo_hbm, w1_hbm, b1_hbm, w2_hbm, b2_hbm,
               o_ref,
               kbuf, vbuf, wqbuf, wobuf, w1buf, w2buf, xnpk, att, opk, scale, vlo, vlo2, sems, *pp):
        xbuf, b1buf, b2buf = pp[-3:]
        bufs = {n: (pp[2 * k], pp[2 * k + 1]) for k, n in enumerate(names)}
        qp, qpk, sp, p, st, gl, den, acca, accb, gpk, oraw, op = (bufs[n] for n in names)
        kb = kbuf.bitcast(BF16)
        vb = vbuf.bitcast(BF16)
        wqb = wqbuf.bitcast(BF16)
        wob = wobuf.bitcast(BF16)
        w1b = w1buf.bitcast(BF16)
        w2b = w2buf.bitcast(BF16)

        S_SMALL, S_WQ, S_K0, S_WO, S_RING = 0, 1, 2, 3, 1 + W2C
        S_W1, S_W2 = 0, 1
        assert S_RING > S_WO

        def window_copies(hbm, buf, start, n, sem):
            return [pltpu.make_async_copy(
                hbm.at[pl.ds(start, n), :, h, :, pl.ds(SK - W, W)],
                buf.at[pl.ds(start, n), :, pl.ds(h * ROWS, ROWS), :], sem) for h in range(2)]

        def group_copies(j, with_k):
            sem = sems.at[S_RING + j % NRING]
            return ((window_copies(k_hbm, kb, j + 2, 1, sem) if with_k else [])
                    + window_copies(v_hbm, vb, j, 1, sem))

        small = [pltpu.make_async_copy(x_hbm, xbuf, sems.at[S_SMALL]),
                 pltpu.make_async_copy(b1_hbm, b1buf, sems.at[S_SMALL]),
                 pltpu.make_async_copy(b2_hbm, b2buf, sems.at[S_SMALL])]
        wq_cps = [pltpu.make_async_copy(wq_hbm.at[:, i * PD:(i + 1) * PD], wqb.at[i], sems.at[S_WQ])
                  for i in range(NP)]
        k0_cps = window_copies(k_hbm, kb, 0, 2, sems.at[S_K0])
        wo_cp = pltpu.make_async_copy(wo_hbm, wob, sems.at[S_WO])
        w1_cp = pltpu.make_async_copy(w1_hbm, w1b, sems.at[S_W1])
        w2_cps = [pltpu.make_async_copy(w2_hbm.at[W2B[c]:W2B[c + 1]], w2b.at[W2B[c]:W2B[c + 1]],
                                        sems.at[S_W2 + c]) for c in range(W2C)]

        for cp in wq_cps:
            cp.start()
        for cp in small:
            cp.start()
        for cp in k0_cps:
            cp.start()
        wo_cp.start()
        for j in range(NRING):
            for cp in group_copies(j, True):
                cp.start()

        row_id = lax.broadcasted_iota(jnp.int32, (ROWS, PD), 0)
        col = lax.broadcasted_iota(jnp.int32, (ROWS, PD), 1)
        first_head = col < DH
        diag = jnp.where(first_head, 0, 1) == row_id

        def tile(t):
            return slice(t * LANES, (t + 1) * LANES)

        def rows(t):
            return slice(t * ROWS, (t + 1) * ROWS)

        def mm(a, b_):
            return jnp.dot(a, b_, preferred_element_type=F32)[0:ROWS]

        def q_proj(i, b):
            for c in range(KQ):
                qp[b][rows(c)] = mm(_unpack(xnpk[:, tile(c)]), wqb[i, tile(c), :])

        def qk(i, b, cs=range(KP)):
            for c in cs:
                sp[b][rows(c)] = mm(_unpack(qpk[b][:, tile(c)]), kb[i, rows(c)].reshape(LANES, W))

        def nt(a, b_):
            return lax.dot_general(a, b_, NT_DIMS, preferred_element_type=F32)

        def packed_acc(b):
            return _unpack(jnp.concatenate([acca[b][:, tile(k)] for k in range(NB)], axis=0))

        def combine_parts(i, b, xn=XN, transposed=True):
            g = _unpack(gpk[b][:, tile(0)])
            parts = [jnp.dot(g, _unpack(accb[b][...]), preferred_element_type=F32) if transposed
                     else nt(g, packed_acc(b))]
            for t in range(xn):
                w = jnp.concatenate([vbuf[i, c * CB:(c + 1) * CB, :, tile(t)].reshape(LANES // 2, LANES)
                                     for c in range(min(KP, XU - t * KP))], axis=1)
                parts.append(jnp.dot(_unpack(gpk[b][:, tile(1 + t)]), _unpack(w),
                                     preferred_element_type=F32))
            return parts

        def combine(i, b):
            for k, part in enumerate(combine_parts(i, b)):
                oraw[b][k * PROWS:(k + 1) * PROWS, 0:part.shape[1]] = part

        def o_proj(i0, b):
            for k in range(ND):
                for c in range(KP):
                    op[b][rows(k * KP + c)] = mm(_unpack(opk[i0 + k, :, tile(c)]), wob[i0 + k, tile(c), :])

        def row_max(b):
            st[b][:, tile(2)] = jnp.broadcast_to(
                jnp.max(st[b][:, tile(0)], axis=1, keepdims=True), (ROWS, LANES))

        def row_sum(b):
            return jnp.broadcast_to(jnp.sum(gl[b][...], axis=1, keepdims=True), (PROWS, LANES))

        def sum_rows(ref, n, cols=slice(None), off=0):
            s = ref[rows(off), cols]
            for c in range(1, n):
                s = s + ref[rows(off + c), cols]
            return s

        def q_pack(b):
            qpk[b][...] = _pack(jnp.where(diag, sum_rows(qp[b], KQ), 0.0))

        def row(ref, r, cols=slice(None)):
            v = ref[r:r + 1, cols]
            return jnp.broadcast_to(v, (ROWS, v.shape[1]))

        def lane_weights(b, xn=XN):
            g = []
            for r in range(2):
                g.append(_round_bf16(jnp.exp2((row(st[b], r, tile(0)) - row(st[b], r, tile(2))) * scale[...])))
                gl[b][rows(r)] = g[r] * row(st[b], r, tile(1))
            gpk[b][:, tile(0)] = _pack(g[0], g[1])
            for t in range(xn):
                gpk[b][:, tile(1 + t)] = _pack(g[0] * row(p[b], 0, tile(t)), g[1] * row(p[b], 1, tile(t)))

        def normalise(parts, dn):
            o = parts[0]
            for part in parts[1:]:
                n = part.shape[1]
                o = o + part if n == PD else jnp.concatenate([o[:, :n] + part, o[:, n:]], axis=1)
            o = o * jnp.concatenate([1.0 / dn] * KP, axis=1)
            return _pack(jnp.where(first_head, o[0:ROWS], o[ROWS:PROWS]))

        def stored_parts(b):
            return [oraw[b][k * PROWS:(k + 1) * PROWS, 0:min(KP, XU - (k - 1) * KP) * LANES]
                    for k in range(1 + XN)]

        def o_pack(i, b):
            opk[i] = normalise(stored_parts(b), den[b][...])

        def softmax_steps(b):
            NC = 4

            def tree(f, xs):
                while len(xs) > 1:
                    xs = [f(xs[k], xs[k + 1]) for k in range(0, len(xs), 2)]
                return xs[0]

            mc = [None] * NC
            for t in range(NT):
                s = sum_rows(sp[b], KP, tile(t))
                sp[b][rows(0), tile(t)] = s
                mc[t % NC] = s if t < NC else jnp.maximum(mc[t % NC], s)
                yield
            mm_ = tree(jnp.maximum, mc)
            st[b][:, tile(0)] = mm_
            lc = [None] * NC
            sc = scale[...]
            for t in range(NT):
                e = jnp.exp2((sp[b][rows(0), tile(t)] - mm_) * sc)
                p[b][:, tile(t)] = e
                lc[t % NC] = e if t < NC else lc[t % NC] + e
                if t == NT - 1:
                    st[b][:, tile(1)] = tree(jnp.add, lc)
                yield

        def pv_steps(i, b, first, xn, xt, lo_ref):
            HB = HW // DB
            for j in range(2):
                for db in range(DB):
                    ng = HB // G
                    col = (j * HW + db * HB) // ROWS // CB
                    assert XU % KP == 0 or col == ((j * HW + (db + 1) * HB) // ROWS - 1) // CB
                    t0 = len(range(col, XU, KP)) if xn else 0
                    order = sorted(range(t0, NT),
                                   key=lambda t: ((t - t0 + 0.5) / (NT - xt - t0) if t < NT - xt
                                                  else (t - (NT - xt) + 0.5) / xt))
                    acc = [None] * ng
                    for pos, t in enumerate(order):
                        pb = p[b][j:j + 1, tile(t)]
                        for g in range(ng):
                            b0 = (j * HW + db * HB + g * G) // ROWS
                            bands = slice(b0, b0 + G // ROWS)
                            u = vbuf[i, bands, :, tile(t)]
                            if t < NT - xt or first:
                                lo, hi = _split(u)
                                if t >= NT - xt:
                                    vbuf[i, bands, :, tile(t)] = hi
                                    lo_ref[bands, :, tile(t - (NT - xt))] = lo
                            else:
                                lo = lo_ref[bands, :, tile(t - (NT - xt))]
                                hi = u
                            term = pltpu.bitcast(jnp.concatenate([lo, hi], axis=1), F32) * pb
                            acc[g] = term if pos == 0 else acc[g] + term
                            if pos == len(order) - 1:
                                for k in range(G // ROWS):
                                    acca[b][:, tile(b0 + k)] = pltpu.bitcast(
                                        acc[g][k].astype(BF16), U32)
                        yield

        def step(j, b, first, left):
            nb = 1 - b
            xn = XN if left is None else 0
            extra = [lambda: lane_weights(nb, 0 if left == 1 else XN),
                     lambda: o_pack(jnp.maximum(j - 3, 0), nb)]

            if left is None:
                extra.append(lambda: q_pack(nb))
            if first and xn:
                def transpose_v():
                    for u_ in range(XU):
                        blk = (j, slice(u_ % KP * CB, (u_ % KP + 1) * CB), slice(None), tile(u_ // KP))
                        v32 = pltpu.bitcast(jnp.concatenate(_split(vbuf[blk]), axis=1), F32)
                        w = pltpu.bitcast(v32.reshape(LANES, LANES).astype(BF16).T, U32)
                        vbuf[blk] = w.reshape(CB, ROWS, LANES)
                extra.append(transpose_v)
            if left == 1:
                for k in range(ND):
                    def acc_op(k=k):
                        s_ = sum_rows(op[nb], KP, off=k * KP)
                        att[...] = s_ if k == 0 else att[...] + s_
                    extra.append(acc_op)
            if left != 1:
                sm = softmax_steps(nb)
                extra += [lambda: next(sm)] * (2 * NT)
            nsteps = 2 * DB * NT - (XU * 2 * DB // KP if xn else 0)
            done = 0
            for k, _ in enumerate(pv_steps(j, b, first, xn, *(
                    (XT, vlo.at[j]) if left is None else (XT2, vlo2.at[2 - left])))):
                upto = (k + 1) * len(extra) // nsteps
                for f in extra[done:upto]:
                    f()
                done = upto
            assert done == len(extra)
            if left is None:
                qk(j + 2, b)
            combine(jnp.maximum(j - 2, 0), b)
            if left is None:
                q_proj(jnp.minimum(j + 4, NP - 1), b)
            else:
                o_proj((2 - left) * ND, b)
            accb[nb][...] = pltpu.bitcast(packed_acc(nb).T, U32)
            row_max(b)
            den[b][...] = row_sum(b)

        def attention(x, first):
            mean, rstd = _ln_stats(x)
            xnpk[...] = _pack(x - mean)
            scale[...] = jnp.broadcast_to(rstd * exp2_scale, (ROWS, LANES))
            for ref in (p[1].at[:, 0:max(XN, 1) * LANES], gpk[0], accb[0], acca[1], oraw[1]):
                ref[...] = jnp.zeros(ref.shape, ref.dtype)
            for ref in (st[1], gl[0], den[1]):
                ref[...] = jnp.ones(ref.shape, ref.dtype)
            if first:
                for cp in wq_cps:
                    cp.wait()
            qpk[0][...] = _pack(jnp.where(diag, _centered_dot(x, mean, wqb[0]), 0.0))
            if first:
                for cp in k0_cps:
                    cp.wait()
            qk(0, 0, (0,))
            q_proj(1, 1)
            q_pack(1)
            qk(0, 0, range(1, KP))
            qk(1, 1)
            q_proj(2, 0)
            q_pack(0)
            q_proj(3, 1)
            for _ in softmax_steps(0):
                pass
            if first:
                wo_cp.wait()

                def reorder_wo(i, carry):
                    for band in range(NB):
                        wobuf[i, rows(band)] = _deinterleave(wobuf[i, rows(band)])
                    return carry
                lax.fori_loop(0, NP, reorder_wo, 0)

            def stream(j):
                if not first:
                    return
                if isinstance(j, int):
                    for cp in group_copies(j, False):
                        cp.wait()
                    return
                for cp in group_copies(j, True):
                    cp.wait()

                @pl.when(j + NRING < NP - 2)
                def _():
                    for cp in group_copies(j + NRING, True):
                        cp.start()

                @pl.when(jnp.logical_and(j + NRING >= NP - 2, j + NRING < NP))
                def _():
                    for cp in group_copies(j + NRING, False):
                        cp.start()

                @pl.when(j + NRING == NP - 1)
                def _():
                    w1_cp.start()
                    for cp in w2_cps:
                        cp.start()

            def body(_, j):
                for b in range(2):
                    stream(j + b)

                    @pl.when(((j + b) & 1) == b)
                    def _():
                        step(j + b, b, first, None)
                return j + 2

            j_end = lax.fori_loop(0, NP // 2 - 1, body, 0)
            for left in (2, 1):
                stream(NP - left)

                @pl.when(j_end + (2 - left) == NP - left)
                def _():
                    step(NP - left, (NP - left) % 2, first, left)

            lane_weights(1, 0)
            o2 = combine_parts(NP - 2, 0, 0)
            o1 = combine_parts(NP - 1, 1, 0, transposed=False)
            a = x + att[...] + sum_rows(op[1], ND * KP)
            a = a + mm(_unpack(opk[NP - 4]), wob[NP - 4])
            a = a + mm(_unpack(normalise(stored_parts(1), den[1][...])), wob[NP - 3])
            a = a + mm(_unpack(normalise(o2, row_sum(0))), wob[NP - 2])
            a = a + mm(_unpack(normalise(o1, row_sum(1))), wob[NP - 1])
            return _round_bf16(a)

        def ffn(x, first):
            mean, rstd = _ln_stats(x)
            if first:
                w1_cp.wait()
            b1 = b1buf[...].reshape(1, FF).astype(F32)
            b2 = b2buf[...].reshape(1, D).astype(F32)
            h = _centered_dot(x, mean, w1b[...]) * rstd
            h = _gelu_tanh(h + b1).astype(BF16)
            y = x + b2
            bounds = W2B if first else list(range(0, FF + 1, 128))
            for c in range(len(bounds) - 1):
                if first:
                    w2_cps[c].wait()
                yc = jnp.dot(h[:, bounds[c]:bounds[c + 1]], w2b[bounds[c]:bounds[c + 1], :],
                             preferred_element_type=F32)
                y = y + yc
            return _round_bf16(y)

        for cp in small:
            cp.wait()
        x = jnp.broadcast_to(xbuf[0].astype(F32), (ROWS, D))
        x = attention(x, True)
        x = ffn(x, True)
        x = attention(x, False)
        x = ffn(x, False)
        o_ref[0] = x[0:1].astype(o_ref.dtype)

    any_spec = pl.BlockSpec(memory_space=pl.ANY)
    return pl.pallas_call(
        kernel,
        out_shape=jax.ShapeDtypeStruct((B, SQ, D), A_x.dtype),
        in_specs=[any_spec] * 9,
        out_specs=pl.BlockSpec(memory_space=pltpu.VMEM),
        scratch_shapes=[
            pltpu.VMEM((NP, NB, ROWS, W), U32),
            pltpu.VMEM((NP, NB, ROWS, W), U32),
            pltpu.VMEM((NP, D // 2, PD), U32),
            pltpu.VMEM((NP, DH, D), U32),
            pltpu.VMEM((D // 2, FF), U32),
            pltpu.VMEM((FF // 2, D), U32),
            pltpu.VMEM((ROWS, D), U32),
            pltpu.VMEM((ROWS, D), F32),
            pltpu.VMEM((NP, ROWS, PD), U32),
            pltpu.VMEM((ROWS, LANES), F32),
            pltpu.VMEM((NP - 2, NB, ROWS, max(XT, 1) * LANES), U32),
            pltpu.VMEM((2, NB, ROWS, max(XT2, 1) * LANES), U32),
            pltpu.SemaphoreType.DMA((1 + W2C + NRING,)),
        ] + [pltpu.VMEM(*pingpong[n]) for n in names for _ in range(2)] + [
            pltpu.VMEM((B, SQ, D), BF16),
            pltpu.VMEM((FF,), BF16),
            pltpu.VMEM((D,), BF16),
        ],
        compiler_params=pltpu.CompilerParams(vmem_limit_bytes=511 * 256 * 1024),
    )(A_x, kt, vt, A_wq, wo3, B_w1, B_b1, B_w2, B_b2)
```

```python
import math

import jax
import jax.numpy as jnp
from jax import lax
import jax.experimental.pallas as pl
import jax.experimental.pallas.tpu as pltpu

F32 = jnp.float32
BF16 = jnp.bfloat16
U32 = jnp.uint32

LANES = 128
ROWS = 8
PROWS = 16
NT_DIMS = (((1,), (1,)), ((), ()))


def _ln_stats(x, eps=1e-5):
    m = jnp.mean(x, axis=-1, keepdims=True)
    c = x - m
    v = jnp.mean(c * c, axis=-1, keepdims=True)
    return m, 1.0 / jnp.sqrt(v + eps)


def _centered_dot(x, m, w):
    lhs = jnp.concatenate([x, jnp.ones_like(x)], axis=0).astype(BF16)
    y = jnp.dot(lhs, w, preferred_element_type=F32)
    return y[0:ROWS] - m * y[ROWS:PROWS]


def _round_bf16(x):
    return x.astype(BF16).astype(F32)


def _gelu_tanh(x):
    c = math.sqrt(2.0 / math.pi)
    return 0.5 * x * (1.0 + jnp.tanh(c * (x + 0.044715 * (x * x * x))))


def _pack(x, y=None):
    y = jnp.zeros_like(x) if y is None else y
    return pltpu.bitcast(jnp.concatenate([x, y], axis=0).astype(BF16), U32)


def _unpack(u):
    return pltpu.bitcast(u, BF16)


def _split(u):
    return u << 16, u & U32(0xFFFF0000)


def _deinterleave(u):
    rows16 = pltpu.bitcast(jnp.concatenate(_split(u), axis=0), F32)
    return pltpu.bitcast(rows16.astype(BF16), U32)


@jax.jit
def pallas_interleave_layers__sliding_block_cached__dense_activation_gelu__decode_kernel(
    A_x: jax.Array,
    A_k_cache: jax.Array,
    A_v_cache: jax.Array,
    A_wq: jax.Array,
    A_wo: jax.Array,
    B_x: jax.Array,
    B_w1: jax.Array,
    B_b1: jax.Array,
    B_w2: jax.Array,
    B_b2: jax.Array,
):
    B, SQ, D = A_x.shape
    _, H, SK, DH = A_k_cache.shape
    FF = B_w1.shape[1]
    assert B == 1 and SQ == 1 and A_wq.shape[1] == H * DH and H % 4 == 0
    W = min(4096, max(256, SK // 4))
    NP = H // 2
    PD = 2 * DH
    NT = W // LANES
    KQ = D // LANES
    KP = PD // LANES
    W2B = [0, FF - 8 * LANES, FF - 4 * LANES, FF - LANES, FF]
    W2C = len(W2B) - 1
    XU = [10, 10, 10, 10, 10, 10, 10, 10, 2, 2, 13, 13, 23, 19, 0, 0]
    XT = [8, 9, 3, 3, 3, 3, 3, 3, 12, 12, 6, 6, 0, 2, 16, 16]
    OPN = [0, 0, 6, 6]
    assert len(XU) == len(XT) == NP and XU[-1] == XU[-2] == 0 and sum(OPN) == NP - 4
    XO = [sum(XT[:i]) for i in range(NP)]
    XN = -(-max(XU) // KP)
    CB = LANES // PROWS
    ND = max(OPN + [(NP - 4) // 2])
    G = 2 * ROWS
    DB = 3
    NRING = 3
    exp2_scale = float(DH) ** -0.5 * math.log2(math.e)

    NB = PD // PROWS
    kt = jnp.transpose(A_k_cache, (0, 1, 3, 2)).reshape(NP, NB, 2, ROWS, SK)
    vt = jnp.transpose(A_v_cache, (0, 1, 3, 2)).reshape(NP, NB, 2, ROWS, SK)
    wo3 = A_wo.reshape(NP, PD, D)

    pingpong = dict(
        qp=((KQ * ROWS, PD), F32),
        qpk=((ROWS, PD), U32),
        sp=((KP * ROWS, W), F32),
        p=((ROWS, W), F32),
        st=((ROWS, 3 * LANES), F32),
        gl=((PROWS, LANES), F32),
        den=((PROWS, LANES), F32),
        acca=((ROWS, NB * LANES), U32),
        accb=((LANES // 2, PD), U32),
        gpk=((ROWS, (1 + XN) * LANES), U32),
        oraw=(((1 + XN) * PROWS, PD), F32),
        op=((ND * KP * ROWS, D), F32),
    )
    names = list(pingpong)

    def kernel(x_hbm, k_hbm, v_hbm, wq_hbm, wo_hbm, w1_hbm, b1_hbm, w2_hbm, b2_hbm,
               o_ref,
               kbuf, vbuf, wqbuf, wobuf, w1buf, w2buf, xnpk, att, opk, scale, vlo, tbl, sems, *pp):
        xbuf, b1buf, b2buf = pp[-3:]
        bufs = {n: (pp[2 * k], pp[2 * k + 1]) for k, n in enumerate(names)}
        qp, qpk, sp, p, st, gl, den, acca, accb, gpk, oraw, op = (bufs[n] for n in names)
        kb = kbuf.bitcast(BF16)
        vb = vbuf.bitcast(BF16)
        wqb = wqbuf.bitcast(BF16)
        wob = wobuf.bitcast(BF16)
        w1b = w1buf.bitcast(BF16)
        w2b = w2buf.bitcast(BF16)

        S_SMALL, S_WQ, S_K0, S_WO, S_RING = 0, 1, 2, 3, 1 + W2C
        S_W1, S_W2 = 0, 1
        assert S_RING > S_WO

        def window_copies(hbm, buf, start, n, sem):
            return [pltpu.make_async_copy(
                hbm.at[pl.ds(start, n), :, h, :, pl.ds(SK - W, W)],
                buf.at[pl.ds(start, n), :, pl.ds(h * ROWS, ROWS), :], sem) for h in range(2)]

        def group_copies(j, with_k):
            sem = sems.at[S_RING + j % NRING]
            return ((window_copies(k_hbm, kb, j + 2, 1, sem) if with_k else [])
                    + window_copies(v_hbm, vb, j, 1, sem))

        small = [pltpu.make_async_copy(x_hbm, xbuf, sems.at[S_SMALL]),
                 pltpu.make_async_copy(b1_hbm, b1buf, sems.at[S_SMALL]),
                 pltpu.make_async_copy(b2_hbm, b2buf, sems.at[S_SMALL])]
        wq_cps = [pltpu.make_async_copy(wq_hbm.at[:, i * PD:(i + 1) * PD], wqb.at[i], sems.at[S_WQ])
                  for i in range(NP)]
        k0_cps = window_copies(k_hbm, kb, 0, 2, sems.at[S_K0])
        wo_cp = pltpu.make_async_copy(wo_hbm, wob, sems.at[S_WO])
        w1_cp = pltpu.make_async_copy(w1_hbm, w1b, sems.at[S_W1])
        w2_cps = [pltpu.make_async_copy(w2_hbm.at[W2B[c]:W2B[c + 1]], w2b.at[W2B[c]:W2B[c + 1]],
                                        sems.at[S_W2 + c]) for c in range(W2C)]

        for cp in wq_cps:
            cp.start()
        for cp in small:
            cp.start()
        for cp in k0_cps:
            cp.start()
        wo_cp.start()
        for j in range(NRING):
            for cp in group_copies(j, True):
                cp.start()

        row_id = lax.broadcasted_iota(jnp.int32, (ROWS, PD), 0)
        col = lax.broadcasted_iota(jnp.int32, (ROWS, PD), 1)
        first_head = col < DH
        diag = jnp.where(first_head, 0, 1) == row_id

        def tile(t):
            return slice(t * LANES, (t + 1) * LANES)

        def rows(t):
            return slice(t * ROWS, (t + 1) * ROWS)

        def mm(a, b_):
            return jnp.dot(a, b_, preferred_element_type=F32)[0:ROWS]

        def q_proj(i, b):
            for c in range(KQ):
                qp[b][rows(c)] = mm(_unpack(xnpk[:, tile(c)]), wqb[i, tile(c), :])

        def qk(i, b, cs=range(KP)):
            for c in cs:
                sp[b][rows(c)] = mm(_unpack(qpk[b][:, tile(c)]), kb[i, rows(c)].reshape(LANES, W))

        def nt(a, b_):
            return lax.dot_general(a, b_, NT_DIMS, preferred_element_type=F32)

        def packed_acc(b):
            return _unpack(jnp.concatenate([acca[b][:, tile(k)] for k in range(NB)], axis=0))

        def combine_parts(i, b, xu, transposed=True):
            g = _unpack(gpk[b][:, tile(0)])
            parts = [jnp.dot(g, _unpack(accb[b][...]), preferred_element_type=F32) if transposed
                     else nt(g, packed_acc(b))]
            for t in range(-(-xu // KP)):
                w = jnp.concatenate([vbuf[i, c * CB:(c + 1) * CB, :, tile(t)].reshape(LANES // 2, LANES)
                                     for c in range(min(KP, xu - t * KP))], axis=1)
                parts.append(jnp.dot(_unpack(gpk[b][:, tile(1 + t)]), _unpack(w),
                                     preferred_element_type=F32))
            return parts

        def combine(i, b, xu):
            for k, part in enumerate(combine_parts(i, b, xu)):
                oraw[b][k * PROWS:(k + 1) * PROWS, 0:part.shape[1]] = part

        def o_proj(i0, n, b):
            for k in range(n):
                for c in range(KP):
                    op[b][rows(k * KP + c)] = mm(_unpack(opk[i0 + k, :, tile(c)]), wob[i0 + k, tile(c), :])

        def row_max(b):
            st[b][:, tile(2)] = jnp.broadcast_to(
                jnp.max(st[b][:, tile(0)], axis=1, keepdims=True), (ROWS, LANES))

        def row_sum(b):
            return jnp.broadcast_to(jnp.sum(gl[b][...], axis=1, keepdims=True), (PROWS, LANES))

        def sum_rows(ref, n, cols=slice(None), off=0):
            s = ref[rows(off), cols]
            for c in range(1, n):
                s = s + ref[rows(off + c), cols]
            return s

        def q_pack(b):
            qpk[b][...] = _pack(jnp.where(diag, sum_rows(qp[b], KQ), 0.0))

        def row(ref, r, cols=slice(None)):
            v = ref[r:r + 1, cols]
            return jnp.broadcast_to(v, (ROWS, v.shape[1]))

        def lane_weights(b, xu):
            g = []
            for r in range(2):
                g.append(_round_bf16(jnp.exp2((row(st[b], r, tile(0)) - row(st[b], r, tile(2))) * scale[...])))
                gl[b][rows(r)] = g[r] * row(st[b], r, tile(1))
            gpk[b][:, tile(0)] = _pack(g[0], g[1])
            for t in range(-(-xu // KP)):
                gpk[b][:, tile(1 + t)] = _pack(g[0] * row(p[b], 0, tile(t)), g[1] * row(p[b], 1, tile(t)))

        def normalise(parts, dn):
            o = parts[0]
            for part in parts[1:]:
                n = part.shape[1]
                o = o + part if n == PD else jnp.concatenate([o[:, :n] + part, o[:, n:]], axis=1)
            o = o * jnp.concatenate([1.0 / dn] * KP, axis=1)
            return _pack(jnp.where(first_head, o[0:ROWS], o[ROWS:PROWS]))

        def stored_parts(b, xu):
            return [oraw[b][k * PROWS:(k + 1) * PROWS, 0:min(KP, xu - (k - 1) * KP) * LANES]
                    for k in range(1 - (-xu // KP))]

        def o_pack(i, b, xu):
            opk[i] = normalise(stored_parts(b, xu), den[b][...])

        def softmax_steps(b):
            NC = 4

            def tree(f, xs):
                while len(xs) > 1:
                    xs = [f(xs[k], xs[k + 1]) for k in range(0, len(xs), 2)]
                return xs[0]

            mc = [None] * NC
            for t in range(NT):
                s = sum_rows(sp[b], KP, tile(t))
                sp[b][rows(0), tile(t)] = s
                mc[t % NC] = s if t < NC else jnp.maximum(mc[t % NC], s)
                yield
            mm_ = tree(jnp.maximum, mc)
            st[b][:, tile(0)] = mm_
            lc = [None] * NC
            sc = scale[...]
            for t in range(NT):
                e = jnp.exp2((sp[b][rows(0), tile(t)] - mm_) * sc)
                p[b][:, tile(t)] = e
                lc[t % NC] = e if t < NC else lc[t % NC] + e
                if t == NT - 1:
                    st[b][:, tile(1)] = tree(jnp.add, lc)
                yield

        def pv_tiles(xu):
            nbands = NB // 2 // DB
            return [(h, b0, range(len(range(b0 // CB, xu, KP)), NT))
                    for h in range(2) for b0 in range(h * NB // 2, (h + 1) * NB // 2, nbands)]

        def pv_steps(i, b, xu, xt, xo):
            gb = G // ROWS
            for h, b0, tiles in pv_tiles(xu):
                npk = len(tiles) - xt
                order = sorted(tiles, key=lambda t: ((t - tiles[0] + 0.5) / npk if t < NT - xt
                                                     else (t - (NT - xt) + 0.5) / xt))
                groups = range(b0, b0 + NB // 2 // DB, gb)
                acc = {}
                for pos, t in enumerate(order):
                    pb = p[b][h:h + 1, tile(t)]
                    for g0 in groups:
                        u = vbuf[i, g0:g0 + gb, :, tile(t)]
                        if t < NT - xt:
                            lo, hi = _split(u)
                        else:
                            lo, hi = vlo[xo + NT - 1 - t, g0:g0 + gb], u
                        term = pltpu.bitcast(jnp.concatenate([lo, hi], axis=1), F32) * pb
                        acc[g0] = term if pos == 0 else acc[g0] + term
                        if pos == len(order) - 1:
                            for k in range(gb):
                                acca[b][:, tile(g0 + k)] = pltpu.bitcast(acc[g0][k].astype(BF16), U32)
                    yield

        def rewrite_v(i):
            def transpose(u_, carry):
                blk = (i, pl.ds(pl.multiple_of(u_ % KP * CB, CB), CB), slice(None),
                       pl.ds(pl.multiple_of(u_ // KP * LANES, LANES), LANES))
                v32 = pltpu.bitcast(jnp.concatenate(_split(vbuf[blk]), axis=1), F32)
                w = pltpu.bitcast(v32.reshape(LANES, LANES).astype(BF16).T, U32)
                vbuf[blk] = w.reshape(CB, ROWS, LANES)
                return carry

            def unpack(k, carry):
                blk = (i, slice(None), slice(None),
                       pl.ds(pl.multiple_of((NT - 1 - k) * LANES, LANES), LANES))
                lo, hi = _split(vbuf[blk])
                vbuf[blk] = hi
                vlo[tbl[2 * NP + i] + k] = lo
                return carry

            lax.fori_loop(0, tbl[i], transpose, 0)
            lax.fori_loop(0, tbl[NP + i], unpack, 0)

        def step(j, b, first):
            nb = 1 - b
            static = isinstance(j, int)

            def live(i):
                return not static or 0 <= i < NP

            def at(i):
                return i if static else jnp.clip(i, 0, NP - 1)

            def xu(i):
                return 0 if first or not live(i) else XU[i]

            opn = [0, 0, (NP - 4) // 2, (NP - 4) // 2] if first else OPN
            ops = {NP - 4 + k: (sum(opn[:k]), n) for k, n in enumerate(opn) if n}
            extra = []
            if live(j - 1):
                extra.append(lambda: lane_weights(nb, xu(j - 1)))
            if live(j - 3):
                extra.append(lambda: o_pack(at(j - 3), nb, xu(j - 3)))
            if live(j + 3):
                extra.append(lambda: q_pack(nb))
            if static and j - 1 in ops:
                i0, n = ops[j - 1]
                for k in range(n):
                    def acc_op(k=k):
                        s_ = sum_rows(op[nb], KP, off=k * KP)
                        att[...] = s_ if i0 + k == 0 else att[...] + s_
                    extra.append(acc_op)
            if live(j + 1):
                sm = softmax_steps(nb)
                extra += [lambda: next(sm)] * (2 * NT)
            nsteps = sum(len(tiles) for _, _, tiles in pv_tiles(xu(j)))
            done = 0
            for k, _ in enumerate(pv_steps(j, b, xu(j), *((0, 0) if first else (XT[j], XO[j])))):
                upto = (k + 1) * len(extra) // nsteps
                for f in extra[done:upto]:
                    f()
                done = upto
            if live(j + 2):
                qk(j + 2, b)
            if live(j - 2):
                combine(at(j - 2), b, xu(j - 2))
            if live(j + 4):
                q_proj(at(j + 4), b)
            if static and j in ops:
                o_proj(*ops[j], b)
            if live(j - 1):
                accb[nb][...] = pltpu.bitcast(packed_acc(nb).T, U32)
            row_max(b)
            if live(j - 2):
                den[b][...] = row_sum(b)

        state = {}

        def attention(x, first):
            mean, rstd = _ln_stats(x)
            xnpk[...] = _pack(x - mean)
            scale[...] = jnp.broadcast_to(rstd * exp2_scale, (ROWS, LANES))
            if first:
                for ref in (gpk[0].at[:, tile(0)], accb[0], acca[1], oraw[1].at[0:PROWS]):
                    ref[...] = jnp.zeros(ref.shape, ref.dtype)
                for ref in (st[1], gl[0], den[1]):
                    ref[...] = jnp.ones(ref.shape, ref.dtype)
                for cp in wq_cps:
                    cp.wait()
            qpk[0][...] = _pack(jnp.where(diag, _centered_dot(x, mean, wqb[0]), 0.0))
            if first:
                for cp in k0_cps:
                    cp.wait()
            qk(0, 0, (0,))
            q_proj(1, 1)
            q_pack(1)
            qk(0, 0, range(1, KP))
            qk(1, 1)
            q_proj(2, 0)
            q_pack(0)
            q_proj(3, 1)
            for _ in softmax_steps(0):
                pass
            if first:
                wo_cp.wait()

                def reorder_wo(i, carry):
                    for band in range(NB):
                        wobuf[i, rows(band)] = _deinterleave(wobuf[i, rows(band)])
                    return carry
                lax.fori_loop(0, NP, reorder_wo, 0)

            def stream(j):
                if not first:
                    return
                if isinstance(j, int):
                    for cp in group_copies(j, False):
                        cp.wait()
                    return
                for cp in group_copies(j, True):
                    cp.wait()

                @pl.when(j + NRING < NP - 2)
                def _():
                    for cp in group_copies(j + NRING, True):
                        cp.start()

                @pl.when(jnp.logical_and(j + NRING >= NP - 2, j + NRING < NP))
                def _():
                    for cp in group_copies(j + NRING, False):
                        cp.start()

                @pl.when(j + NRING == NP - 1)
                def _():
                    w1_cp.start()
                    for cp in w2_cps:
                        cp.start()

            def run(j, b, cond):
                stream(j)

                @pl.when(cond)
                def _():
                    step(j, b, first)
                if first:
                    rewrite_v(j)

            if first:
                def body(_, j):
                    for b in range(2):
                        run(j + b, b, ((j + b) & 1) == b)
                    return j + 2
                state['zero'] = lax.fori_loop(0, NP // 2 - 1, body, 0) - (NP - 2)
            for j in range(NP - 2 if first else 0, NP):
                run(j, j % 2, state['zero'] + j == j)

            lane_weights(1, 0)
            o2 = combine_parts(NP - 2, 0, 0)
            o1 = combine_parts(NP - 1, 1, 0, transposed=False)
            n_last = (NP - 4) // 2 if first else OPN[-1]
            a = x + att[...] + sum_rows(op[1], n_last * KP)
            a = a + mm(_unpack(opk[NP - 4]), wob[NP - 4])
            a = a + mm(_unpack(normalise(stored_parts(1, 0 if first else XU[NP - 3]), den[1][...])), wob[NP - 3])
            a = a + mm(_unpack(normalise(o2, row_sum(0))), wob[NP - 2])
            a = a + mm(_unpack(normalise(o1, row_sum(1))), wob[NP - 1])
            return _round_bf16(a)

        def ffn(x, first):
            mean, rstd = _ln_stats(x)
            if first:
                w1_cp.wait()
            b1 = b1buf[...].reshape(1, FF).astype(F32)
            b2 = b2buf[...].reshape(1, D).astype(F32)
            h = _centered_dot(x, mean, w1b[...]) * rstd
            h = _gelu_tanh(h + b1).astype(BF16)
            y = x + b2
            bounds = W2B if first else list(range(0, FF + 1, 128))
            for c in range(len(bounds) - 1):
                if first:
                    w2_cps[c].wait()
                yc = jnp.dot(h[:, bounds[c]:bounds[c + 1]], w2b[bounds[c]:bounds[c + 1], :],
                             preferred_element_type=F32)
                y = y + yc
            return _round_bf16(y)

        for k, v in enumerate(XU + XT + XO):
            tbl[k] = v
        for cp in small:
            cp.wait()
        x = jnp.broadcast_to(xbuf[0].astype(F32), (ROWS, D))
        for first in (True, False):
            x = attention(x, first)
            x = ffn(x, first)
        o_ref[0] = x[0:1].astype(o_ref.dtype)

    any_spec = pl.BlockSpec(memory_space=pl.ANY)
    return pl.pallas_call(
        kernel,
        out_shape=jax.ShapeDtypeStruct((B, SQ, D), A_x.dtype),
        in_specs=[any_spec] * 9,
        out_specs=pl.BlockSpec(memory_space=pltpu.VMEM),
        scratch_shapes=[
            pltpu.VMEM((NP, NB, ROWS, W), U32),
            pltpu.VMEM((NP, NB, ROWS, W), U32),
            pltpu.VMEM((NP, D // 2, PD), U32),
            pltpu.VMEM((NP, DH, D), U32),
            pltpu.VMEM((D // 2, FF), U32),
            pltpu.VMEM((FF // 2, D), U32),
            pltpu.VMEM((ROWS, D), U32),
            pltpu.VMEM((ROWS, D), F32),
            pltpu.VMEM((NP, ROWS, PD), U32),
            pltpu.VMEM((ROWS, LANES), F32),
            pltpu.VMEM((sum(XT), NB, ROWS, LANES), U32),
            pltpu.SMEM((3 * NP,), jnp.int32),
            pltpu.SemaphoreType.DMA((1 + W2C + NRING,)),
        ] + [pltpu.VMEM(*pingpong[n]) for n in names for _ in range(2)] + [
            pltpu.VMEM((B, SQ, D), BF16),
            pltpu.VMEM((FF,), BF16),
            pltpu.VMEM((D,), BF16),
        ],
        compiler_params=pltpu.CompilerParams(vmem_limit_bytes=511 * 256 * 1024),
    )(A_x, kt, vt, A_wq, wo3, B_w1, B_b1, B_w2, B_b2)
```

```python
import math

import jax
import jax.numpy as jnp
from jax import lax
import jax.experimental.pallas as pl
import jax.experimental.pallas.tpu as pltpu

F32 = jnp.float32
BF16 = jnp.bfloat16
U32 = jnp.uint32

LANES = 128
ROWS = 8
PROWS = 16
NT_DIMS = (((1,), (1,)), ((), ()))


def _ln_stats(x, eps=1e-5):
    m = jnp.mean(x, axis=-1, keepdims=True)
    c = x - m
    v = jnp.mean(c * c, axis=-1, keepdims=True)
    return m, 1.0 / jnp.sqrt(v + eps)


def _centered_dot(x, m, w):
    lhs = jnp.concatenate([x, jnp.ones_like(x)], axis=0).astype(BF16)
    y = jnp.dot(lhs, w, preferred_element_type=F32)
    return y[0:ROWS] - m * y[ROWS:PROWS]


def _round_bf16(x):
    return x.astype(BF16).astype(F32)


def _gelu_tanh(x):
    c = math.sqrt(2.0 / math.pi)
    return 0.5 * x * (1.0 + jnp.tanh(c * (x + 0.044715 * (x * x * x))))


def _pack(x, y=None):
    y = jnp.zeros_like(x) if y is None else y
    return pltpu.bitcast(jnp.concatenate([x, y], axis=0).astype(BF16), U32)


def _unpack(u):
    return pltpu.bitcast(u, BF16)


def _split(u):
    return u << 16, u & U32(0xFFFF0000)


def _deinterleave(u):
    rows16 = pltpu.bitcast(jnp.concatenate(_split(u), axis=0), F32)
    return pltpu.bitcast(rows16.astype(BF16), U32)


@jax.jit
def pallas_interleave_layers__sliding_block_cached__dense_activation_gelu__decode_kernel(
    A_x: jax.Array,
    A_k_cache: jax.Array,
    A_v_cache: jax.Array,
    A_wq: jax.Array,
    A_wo: jax.Array,
    B_x: jax.Array,
    B_w1: jax.Array,
    B_b1: jax.Array,
    B_w2: jax.Array,
    B_b2: jax.Array,
):
    B, SQ, D = A_x.shape
    _, H, SK, DH = A_k_cache.shape
    FF = B_w1.shape[1]
    assert B == 1 and SQ == 1 and A_wq.shape[1] == H * DH and H % 4 == 0
    W = min(4096, max(256, SK // 4))
    NP = H // 2
    PD = 2 * DH
    NT = W // LANES
    KQ = D // LANES
    KP = PD // LANES
    W2B = [0, FF - 8 * LANES, FF - 4 * LANES, FF - LANES, FF]
    W2C = len(W2B) - 1
    XU = [10, 10, 10, 10, 10, 10, 10, 10, 2, 2, 13, 13, 23, 19, 0, 0]
    XT = [8, 9, 3, 3, 3, 3, 3, 3, 12, 12, 6, 6, 0, 2, 16, 16]
    OPN = [0, 0, 6, 6]
    assert len(XU) == len(XT) == NP and XU[-1] == XU[-2] == 0 and sum(OPN) == NP - 4
    XO = [sum(XT[:i]) for i in range(NP)]
    XN = -(-max(XU) // KP)
    CB = LANES // PROWS
    ND = max(OPN + [(NP - 4) // 2])
    PV_BANDS = (4, 2)
    NRING = 3
    exp2_scale = float(DH) ** -0.5 * math.log2(math.e)

    NB = PD // PROWS
    kt = jnp.transpose(A_k_cache, (0, 1, 3, 2)).reshape(NP, NB, 2, ROWS, SK)
    vt = jnp.transpose(A_v_cache, (0, 1, 3, 2)).reshape(NP, NB, 2, ROWS, SK)
    wo3 = A_wo.reshape(NP, PD, D)

    pingpong = dict(
        qp=((KQ * ROWS, PD), F32),
        qpk=((ROWS, PD), U32),
        sp=((KP * ROWS, W), F32),
        p=((ROWS, W), F32),
        st=((ROWS, 3 * LANES), F32),
        gl=((PROWS, LANES), F32),
        den=((PROWS, LANES), F32),
        acca=((ROWS, NB * LANES), U32),
        accb=((LANES // 2, PD), U32),
        gpk=((ROWS, (1 + XN) * LANES), U32),
        oraw=(((1 + XN) * PROWS, PD), F32),
        op=((ND * KP * ROWS, D), F32),
    )
    names = list(pingpong)

    def kernel(x_hbm, k_hbm, v_hbm, wq_hbm, wo_hbm, w1_hbm, b1_hbm, w2_hbm, b2_hbm,
               o_ref,
               kbuf, vbuf, wqbuf, wobuf, w1buf, w2buf, xnpk, att, opk, scale, vlo, tbl, sems, *pp):
        xbuf, b1buf, b2buf = pp[-3:]
        bufs = {n: (pp[2 * k], pp[2 * k + 1]) for k, n in enumerate(names)}
        qp, qpk, sp, p, st, gl, den, acca, accb, gpk, oraw, op = (bufs[n] for n in names)
        kb = kbuf.bitcast(BF16)
        vb = vbuf.bitcast(BF16)
        wqb = wqbuf.bitcast(BF16)
        wob = wobuf.bitcast(BF16)
        w1b = w1buf.bitcast(BF16)
        w2b = w2buf.bitcast(BF16)

        S_SMALL, S_WQ, S_K0, S_WO, S_RING = 0, 1, 2, 3, 1 + W2C
        S_W1, S_W2 = 0, 1
        assert S_RING > S_WO

        def window_copies(hbm, buf, start, n, sem):
            return [pltpu.make_async_copy(
                hbm.at[pl.ds(start, n), :, h, :, pl.ds(SK - W, W)],
                buf.at[pl.ds(start, n), :, pl.ds(h * ROWS, ROWS), :], sem) for h in range(2)]

        def group_copies(j, with_k):
            sem = sems.at[S_RING + j % NRING]
            return ((window_copies(k_hbm, kb, j + 2, 1, sem) if with_k else [])
                    + window_copies(v_hbm, vb, j, 1, sem))

        small = [pltpu.make_async_copy(x_hbm, xbuf, sems.at[S_SMALL]),
                 pltpu.make_async_copy(b1_hbm, b1buf, sems.at[S_SMALL]),
                 pltpu.make_async_copy(b2_hbm, b2buf, sems.at[S_SMALL])]
        wq_cps = [pltpu.make_async_copy(wq_hbm.at[:, i * PD:(i + 1) * PD], wqb.at[i], sems.at[S_WQ])
                  for i in range(NP)]
        k0_cps = window_copies(k_hbm, kb, 0, 2, sems.at[S_K0])
        wo_cp = pltpu.make_async_copy(wo_hbm, wob, sems.at[S_WO])
        w1_cp = pltpu.make_async_copy(w1_hbm, w1b, sems.at[S_W1])
        w2_cps = [pltpu.make_async_copy(w2_hbm.at[W2B[c]:W2B[c + 1]], w2b.at[W2B[c]:W2B[c + 1]],
                                        sems.at[S_W2 + c]) for c in range(W2C)]

        for cp in wq_cps:
            cp.start()
        for cp in small:
            cp.start()
        for cp in k0_cps:
            cp.start()
        wo_cp.start()
        for j in range(NRING):
            for cp in group_copies(j, True):
                cp.start()

        row_id = lax.broadcasted_iota(jnp.int32, (ROWS, PD), 0)
        col = lax.broadcasted_iota(jnp.int32, (ROWS, PD), 1)
        first_head = col < DH
        diag = jnp.where(first_head, 0, 1) == row_id

        def tile(t):
            return slice(t * LANES, (t + 1) * LANES)

        def rows(t):
            return slice(t * ROWS, (t + 1) * ROWS)

        def mm(a, b_):
            return jnp.dot(a, b_, preferred_element_type=F32)[0:ROWS]

        def q_proj(i, b):
            for c in range(KQ):
                qp[b][rows(c)] = mm(_unpack(xnpk[:, tile(c)]), wqb[i, tile(c), :])

        def qk(i, b, cs=range(KP)):
            for c in cs:
                sp[b][rows(c)] = mm(_unpack(qpk[b][:, tile(c)]), kb[i, rows(c)].reshape(LANES, W))

        def nt(a, b_):
            return lax.dot_general(a, b_, NT_DIMS, preferred_element_type=F32)

        def packed_acc(b):
            return _unpack(jnp.concatenate([acca[b][:, tile(k)] for k in range(NB)], axis=0))

        def combine_parts(i, b, xu, transposed=True):
            g = _unpack(gpk[b][:, tile(0)])
            parts = [jnp.dot(g, _unpack(accb[b][...]), preferred_element_type=F32) if transposed
                     else nt(g, packed_acc(b))]
            for t in range(-(-xu // KP)):
                w = jnp.concatenate([vbuf[i, c * CB:(c + 1) * CB, :, tile(t)].reshape(LANES // 2, LANES)
                                     for c in range(min(KP, xu - t * KP))], axis=1)
                parts.append(jnp.dot(_unpack(gpk[b][:, tile(1 + t)]), _unpack(w),
                                     preferred_element_type=F32))
            return parts

        def combine(i, b, xu):
            for k, part in enumerate(combine_parts(i, b, xu)):
                oraw[b][k * PROWS:(k + 1) * PROWS, 0:part.shape[1]] = part

        def o_proj(i0, n, b):
            for k in range(n):
                for c in range(KP):
                    op[b][rows(k * KP + c)] = mm(_unpack(opk[i0 + k, :, tile(c)]), wob[i0 + k, tile(c), :])

        def row_max(b):
            st[b][:, tile(2)] = jnp.broadcast_to(
                jnp.max(st[b][:, tile(0)], axis=1, keepdims=True), (ROWS, LANES))

        def row_sum(b):
            return jnp.broadcast_to(jnp.sum(gl[b][...], axis=1, keepdims=True), (PROWS, LANES))

        def sum_rows(ref, n, cols=slice(None), off=0):
            s = ref[rows(off), cols]
            for c in range(1, n):
                s = s + ref[rows(off + c), cols]
            return s

        def q_pack(b):
            qpk[b][...] = _pack(jnp.where(diag, sum_rows(qp[b], KQ), 0.0))

        def row(ref, r, cols=slice(None)):
            v = ref[r:r + 1, cols]
            return jnp.broadcast_to(v, (ROWS, v.shape[1]))

        def lane_weights(b, xu):
            g = []
            for r in range(2):
                g.append(_round_bf16(jnp.exp2((row(st[b], r, tile(0)) - row(st[b], r, tile(2))) * scale[...])))
                gl[b][rows(r)] = g[r] * row(st[b], r, tile(1))
            gpk[b][:, tile(0)] = _pack(g[0], g[1])
            for t in range(-(-xu // KP)):
                gpk[b][:, tile(1 + t)] = _pack(g[0] * row(p[b], 0, tile(t)), g[1] * row(p[b], 1, tile(t)))

        def normalise(parts, dn):
            o = parts[0]
            for part in parts[1:]:
                n = part.shape[1]
                o = o + part if n == PD else jnp.concatenate([o[:, :n] + part, o[:, n:]], axis=1)
            o = o * jnp.concatenate([1.0 / dn] * KP, axis=1)
            return _pack(jnp.where(first_head, o[0:ROWS], o[ROWS:PROWS]))

        def stored_parts(b, xu):
            return [oraw[b][k * PROWS:(k + 1) * PROWS, 0:min(KP, xu - (k - 1) * KP) * LANES]
                    for k in range(1 - (-xu // KP))]

        def o_pack(i, b, xu):
            opk[i] = normalise(stored_parts(b, xu), den[b][...])

        def softmax_steps(b):
            NC = 4

            def tree(f, xs):
                while len(xs) > 1:
                    xs = [f(xs[k], xs[k + 1]) for k in range(0, len(xs), 2)]
                return xs[0]

            mc = [None] * NC
            for t in range(NT):
                s = sum_rows(sp[b], KP, tile(t))
                sp[b][rows(0), tile(t)] = s
                mc[t % NC] = s if t < NC else jnp.maximum(mc[t % NC], s)
                yield
            mm_ = tree(jnp.maximum, mc)
            st[b][:, tile(0)] = mm_
            lc = [None] * NC
            sc = scale[...]
            for t in range(NT):
                e = jnp.exp2((sp[b][rows(0), tile(t)] - mm_) * sc)
                p[b][:, tile(t)] = e
                lc[t % NC] = e if t < NC else lc[t % NC] + e
                if t == NT - 1:
                    st[b][:, tile(1)] = tree(jnp.add, lc)
                yield

        def pv_tiles(xu, nbands):
            return [(h, b0, range(len(range(b0 // CB, xu, KP)), NT))
                    for h in range(2) for b0 in range(h * NB // 2, (h + 1) * NB // 2, nbands)]

        def pv_steps(i, b, xu, xt, xo, nbands, gb):
            for h, b0, tiles in pv_tiles(xu, nbands):
                npk = len(tiles) - xt
                order = sorted(tiles, key=lambda t: ((t - tiles[0] + 0.5) / npk if t < NT - xt
                                                     else (t - (NT - xt) + 0.5) / xt))
                groups = range(b0, b0 + nbands, gb)
                acc = {}
                for pos, t in enumerate(order):
                    pb = p[b][h:h + 1, tile(t)]
                    for g0 in groups:
                        u = vbuf[i, g0:g0 + gb, :, tile(t)]
                        if t < NT - xt:
                            lo, hi = _split(u)
                        else:
                            lo, hi = vlo[xo + NT - 1 - t, g0:g0 + gb], u
                        term = pltpu.bitcast(jnp.concatenate([lo, hi], axis=1), F32) * pb
                        acc[g0] = term if pos == 0 else acc[g0] + term
                        if pos == len(order) - 1:
                            for k in range(gb):
                                acca[b][:, tile(g0 + k)] = pltpu.bitcast(acc[g0][k].astype(BF16), U32)
                    yield

        def rewrite_v(i):
            def transpose(u_, carry):
                blk = (i, pl.ds(pl.multiple_of(u_ % KP * CB, CB), CB), slice(None),
                       pl.ds(pl.multiple_of(u_ // KP * LANES, LANES), LANES))
                v32 = pltpu.bitcast(jnp.concatenate(_split(vbuf[blk]), axis=1), F32)
                w = pltpu.bitcast(v32.reshape(LANES, LANES).astype(BF16).T, U32)
                vbuf[blk] = w.reshape(CB, ROWS, LANES)
                return carry

            def unpack(k, carry):
                blk = (i, slice(None), slice(None),
                       pl.ds(pl.multiple_of((NT - 1 - k) * LANES, LANES), LANES))
                lo, hi = _split(vbuf[blk])
                vbuf[blk] = hi
                vlo[tbl[2 * NP + i] + k] = lo
                return carry

            lax.fori_loop(0, tbl[i], transpose, 0)
            lax.fori_loop(0, tbl[NP + i], unpack, 0)

        def step(j, b, first):
            nb = 1 - b
            static = isinstance(j, int)

            def live(i):
                return not static or 0 <= i < NP

            def at(i):
                return i if static else jnp.clip(i, 0, NP - 1)

            def xu(i):
                return 0 if first or not live(i) else XU[i]

            opn = [0, 0, (NP - 4) // 2, (NP - 4) // 2] if first else OPN
            ops = {NP - 4 + k: (sum(opn[:k]), n) for k, n in enumerate(opn) if n}
            extra = []
            if live(j - 1):
                extra.append(lambda: lane_weights(nb, xu(j - 1)))
            if live(j - 3):
                extra.append(lambda: o_pack(at(j - 3), nb, xu(j - 3)))
            if live(j + 3):
                extra.append(lambda: q_pack(nb))
            if static and j - 1 in ops:
                i0, n = ops[j - 1]
                for k in range(n):
                    def acc_op(k=k):
                        s_ = sum_rows(op[nb], KP, off=k * KP)
                        att[...] = s_ if i0 + k == 0 else att[...] + s_
                    extra.append(acc_op)
            if live(j + 1):
                sm = softmax_steps(nb)
                extra += [lambda: next(sm)] * (2 * NT)
            xt, xo, nbands, gb = (0, 0, NB // 2, NB // 4) if first else (XT[j], XO[j], *PV_BANDS)
            nsteps = sum(len(tiles) for _, _, tiles in pv_tiles(xu(j), nbands))
            done = 0
            for k, _ in enumerate(pv_steps(j, b, xu(j), xt, xo, nbands, gb)):
                upto = (k + 1) * len(extra) // nsteps
                for f in extra[done:upto]:
                    f()
                done = upto
            if live(j + 2):
                qk(j + 2, b)
            if live(j - 2):
                combine(at(j - 2), b, xu(j - 2))
            if live(j + 4):
                q_proj(at(j + 4), b)
            if static and j in ops:
                o_proj(*ops[j], b)
            if live(j - 1):
                accb[nb][...] = pltpu.bitcast(packed_acc(nb).T, U32)
            row_max(b)
            if live(j - 2):
                den[b][...] = row_sum(b)

        state = {}

        def attention(x, first):
            mean, rstd = _ln_stats(x)
            xnpk[...] = _pack(x - mean)
            scale[...] = jnp.broadcast_to(rstd * exp2_scale, (ROWS, LANES))
            if first:
                for ref in (gpk[0].at[:, tile(0)], accb[0], acca[1], oraw[1].at[0:PROWS]):
                    ref[...] = jnp.zeros(ref.shape, ref.dtype)
                for ref in (st[1], gl[0], den[1]):
                    ref[...] = jnp.ones(ref.shape, ref.dtype)
                for cp in wq_cps:
                    cp.wait()
            qpk[0][...] = _pack(jnp.where(diag, _centered_dot(x, mean, wqb[0]), 0.0))
            if first:
                for cp in k0_cps:
                    cp.wait()
            qk(0, 0, (0,))
            q_proj(1, 1)
            q_pack(1)
            qk(0, 0, range(1, KP))
            qk(1, 1)
            q_proj(2, 0)
            q_pack(0)
            q_proj(3, 1)
            for _ in softmax_steps(0):
                pass
            if first:
                wo_cp.wait()

                def reorder_wo(i, carry):
                    for band in range(NB):
                        wobuf[i, rows(band)] = _deinterleave(wobuf[i, rows(band)])
                    return carry
                lax.fori_loop(0, NP, reorder_wo, 0)

            def stream(j):
                if not first:
                    return
                if isinstance(j, int):
                    for cp in group_copies(j, False):
                        cp.wait()
                    return
                for cp in group_copies(j, True):
                    cp.wait()

                @pl.when(j + NRING < NP - 2)
                def _():
                    for cp in group_copies(j + NRING, True):
                        cp.start()

                @pl.when(jnp.logical_and(j + NRING >= NP - 2, j + NRING < NP))
                def _():
                    for cp in group_copies(j + NRING, False):
                        cp.start()

                @pl.when(j + NRING == NP - 1)
                def _():
                    w1_cp.start()
                    for cp in w2_cps:
                        cp.start()

            def run(j, b, cond):
                stream(j)

                @pl.when(cond)
                def _():
                    step(j, b, first)
                if first:
                    rewrite_v(j)

            if first:
                def body(_, j):
                    for b in range(2):
                        run(j + b, b, ((j + b) & 1) == b)
                    return j + 2
                state['zero'] = lax.fori_loop(0, NP // 2 - 1, body, 0) - (NP - 2)
            for j in range(NP - 2 if first else 0, NP):
                run(j, j % 2, state['zero'] + j == j)

            lane_weights(1, 0)
            o2 = combine_parts(NP - 2, 0, 0)
            o1 = combine_parts(NP - 1, 1, 0, transposed=False)
            n_last = (NP - 4) // 2 if first else OPN[-1]
            a = x + att[...] + sum_rows(op[1], n_last * KP)
            a = a + mm(_unpack(opk[NP - 4]), wob[NP - 4])
            a = a + mm(_unpack(normalise(stored_parts(1, 0 if first else XU[NP - 3]), den[1][...])), wob[NP - 3])
            a = a + mm(_unpack(normalise(o2, row_sum(0))), wob[NP - 2])
            a = a + mm(_unpack(normalise(o1, row_sum(1))), wob[NP - 1])
            return _round_bf16(a)

        def ffn(x, first):
            mean, rstd = _ln_stats(x)
            if first:
                w1_cp.wait()
            b1 = b1buf[...].reshape(1, FF).astype(F32)
            b2 = b2buf[...].reshape(1, D).astype(F32)
            h = _centered_dot(x, mean, w1b[...]) * rstd
            h = _gelu_tanh(h + b1).astype(BF16)
            y = x + b2
            bounds = W2B if first else list(range(0, FF + 1, 128))
            for c in range(len(bounds) - 1):
                if first:
                    w2_cps[c].wait()
                yc = jnp.dot(h[:, bounds[c]:bounds[c + 1]], w2b[bounds[c]:bounds[c + 1], :],
                             preferred_element_type=F32)
                y = y + yc
            return _round_bf16(y)

        for k, v in enumerate(XU + XT + XO):
            tbl[k] = v
        for cp in small:
            cp.wait()
        x = jnp.broadcast_to(xbuf[0].astype(F32), (ROWS, D))
        for first in (True, False):
            x = attention(x, first)
            x = ffn(x, first)
        o_ref[0] = x[0:1].astype(o_ref.dtype)

    any_spec = pl.BlockSpec(memory_space=pl.ANY)
    return pl.pallas_call(
        kernel,
        out_shape=jax.ShapeDtypeStruct((B, SQ, D), A_x.dtype),
        in_specs=[any_spec] * 9,
        out_specs=pl.BlockSpec(memory_space=pltpu.VMEM),
        scratch_shapes=[
            pltpu.VMEM((NP, NB, ROWS, W), U32),
            pltpu.VMEM((NP, NB, ROWS, W), U32),
            pltpu.VMEM((NP, D // 2, PD), U32),
            pltpu.VMEM((NP, DH, D), U32),
            pltpu.VMEM((D // 2, FF), U32),
            pltpu.VMEM((FF // 2, D), U32),
            pltpu.VMEM((ROWS, D), U32),
            pltpu.VMEM((ROWS, D), F32),
            pltpu.VMEM((NP, ROWS, PD), U32),
            pltpu.VMEM((ROWS, LANES), F32),
            pltpu.VMEM((sum(XT), NB, ROWS, LANES), U32),
            pltpu.SMEM((3 * NP,), jnp.int32),
            pltpu.SemaphoreType.DMA((1 + W2C + NRING,)),
        ] + [pltpu.VMEM(*pingpong[n]) for n in names for _ in range(2)] + [
            pltpu.VMEM((B, SQ, D), BF16),
            pltpu.VMEM((FF,), BF16),
            pltpu.VMEM((D,), BF16),
        ],
        compiler_params=pltpu.CompilerParams(vmem_limit_bytes=511 * 256 * 1024),
    )(A_x, kt, vt, A_wq, wo3, B_w1, B_b1, B_w2, B_b2)
```

```python
import math

import jax
import jax.numpy as jnp
from jax import lax
import jax.experimental.pallas as pl
import jax.experimental.pallas.tpu as pltpu

F32 = jnp.float32
BF16 = jnp.bfloat16
U32 = jnp.uint32

LANES = 128
ROWS = 8
PROWS = 16
NT_DIMS = (((1,), (1,)), ((), ()))


def _ln_stats(x, eps=1e-5):
    m = jnp.mean(x, axis=-1, keepdims=True)
    c = x - m
    v = jnp.mean(c * c, axis=-1, keepdims=True)
    return m, 1.0 / jnp.sqrt(v + eps)


def _centered_dot(x, m, w):
    lhs = jnp.concatenate([x, jnp.ones_like(x)], axis=0).astype(BF16)
    y = jnp.dot(lhs, w, preferred_element_type=F32)
    return y[0:ROWS] - m * y[ROWS:PROWS]


def _round_bf16(x):
    return x.astype(BF16).astype(F32)


def _gelu_tanh(x):
    c = math.sqrt(2.0 / math.pi)
    return 0.5 * x * (1.0 + jnp.tanh(c * (x + 0.044715 * (x * x * x))))


def _pack(x, y=None):
    y = jnp.zeros_like(x) if y is None else y
    return pltpu.bitcast(jnp.concatenate([x, y], axis=0).astype(BF16), U32)


def _unpack(u):
    return pltpu.bitcast(u, BF16)


def _split(u):
    return u << 16, u & U32(0xFFFF0000)


def _deinterleave(u):
    rows16 = pltpu.bitcast(jnp.concatenate(_split(u), axis=0), F32)
    return pltpu.bitcast(rows16.astype(BF16), U32)


@jax.jit
def pallas_interleave_layers__sliding_block_cached__dense_activation_gelu__decode_kernel(
    A_x: jax.Array,
    A_k_cache: jax.Array,
    A_v_cache: jax.Array,
    A_wq: jax.Array,
    A_wo: jax.Array,
    B_x: jax.Array,
    B_w1: jax.Array,
    B_b1: jax.Array,
    B_w2: jax.Array,
    B_b2: jax.Array,
):
    B, SQ, D = A_x.shape
    _, H, SK, DH = A_k_cache.shape
    FF = B_w1.shape[1]
    assert B == 1 and SQ == 1 and A_wq.shape[1] == H * DH and H % 4 == 0
    W = min(4096, max(256, SK // 4))
    NP = H // 2
    PD = 2 * DH
    NT = W // LANES
    KQ = D // LANES
    KP = PD // LANES
    W2B = [0, FF - 8 * LANES, FF - 4 * LANES, FF - LANES, FF]
    W2C = len(W2B) - 1
    XU = [10, 10, 10, 10, 10, 10, 10, 10, 2, 2, 13, 13, 23, 19, 0, 0]
    XT = [8, 9, 3, 3, 3, 3, 3, 3, 12, 12, 6, 6, 0, 2, 16, 16]
    OPN = [0, 0, 6, 6]
    assert len(XU) == len(XT) == NP and XU[-1] == XU[-2] == 0 and sum(OPN) == NP - 4
    XO = [sum(XT[:i]) for i in range(NP)]
    XN = -(-max(XU) // KP)
    CB = LANES // PROWS
    ND = max(OPN + [(NP - 4) // 2])
    PV_BANDS = (4, 2)
    NRING = 3
    exp2_scale = float(DH) ** -0.5 * math.log2(math.e)

    NB = PD // PROWS
    kt = jnp.transpose(A_k_cache, (0, 1, 3, 2)).reshape(NP, NB, 2, ROWS, SK)
    vt = jnp.transpose(A_v_cache, (0, 1, 3, 2)).reshape(NP, NB, 2, ROWS, SK)
    wo3 = A_wo.reshape(NP, PD, D)

    pingpong = dict(
        qp=((KQ * ROWS, PD), F32),
        qpk=((ROWS, PD), U32),
        sp=((KP * ROWS, W), F32),
        p=((ROWS, W), F32),
        st=((ROWS, 3 * LANES), F32),
        gl=((PROWS, LANES), F32),
        den=((PROWS, LANES), F32),
        acca=((ROWS, NB * LANES), U32),
        accb=((LANES // 2, PD), U32),
        gpk=((ROWS, (1 + XN) * LANES), U32),
        oraw=(((1 + XN) * PROWS, PD), F32),
        op=((ND * KP * ROWS, D), F32),
    )
    names = list(pingpong)

    def kernel(x_hbm, k_hbm, v_hbm, wq_hbm, wo_hbm, w1_hbm, b1_hbm, w2_hbm, b2_hbm,
               o_ref,
               kbuf, vbuf, wqbuf, wobuf, w1buf, w2buf, xnpk, att, opk, scale, vlo, sems, *pp):
        xbuf, b1buf, b2buf = pp[-3:]
        bufs = {n: (pp[2 * k], pp[2 * k + 1]) for k, n in enumerate(names)}
        qp, qpk, sp, p, st, gl, den, acca, accb, gpk, oraw, op = (bufs[n] for n in names)
        kb = kbuf.bitcast(BF16)
        vb = vbuf.bitcast(BF16)
        wqb = wqbuf.bitcast(BF16)
        wob = wobuf.bitcast(BF16)
        w1b = w1buf.bitcast(BF16)
        w2b = w2buf.bitcast(BF16)

        S_SMALL, S_WQ, S_K0, S_WO, S_RING = 0, 1, 2, 3, 1 + W2C
        S_W1, S_W2 = 0, 1
        assert S_RING > S_WO

        def window_copies(hbm, buf, start, n, sem):
            return [pltpu.make_async_copy(
                hbm.at[pl.ds(start, n), :, h, :, pl.ds(SK - W, W)],
                buf.at[pl.ds(start, n), :, pl.ds(h * ROWS, ROWS), :], sem) for h in range(2)]

        def group_copies(j, with_k):
            sem = sems.at[S_RING + j % NRING]
            return ((window_copies(k_hbm, kb, j + 2, 1, sem) if with_k else [])
                    + window_copies(v_hbm, vb, j, 1, sem))

        small = [pltpu.make_async_copy(x_hbm, xbuf, sems.at[S_SMALL]),
                 pltpu.make_async_copy(b1_hbm, b1buf, sems.at[S_SMALL]),
                 pltpu.make_async_copy(b2_hbm, b2buf, sems.at[S_SMALL])]
        wq_cps = [pltpu.make_async_copy(wq_hbm.at[:, i * PD:(i + 1) * PD], wqb.at[i], sems.at[S_WQ])
                  for i in range(NP)]
        k0_cps = window_copies(k_hbm, kb, 0, 2, sems.at[S_K0])
        wo_cp = pltpu.make_async_copy(wo_hbm, wob, sems.at[S_WO])
        w1_cp = pltpu.make_async_copy(w1_hbm, w1b, sems.at[S_W1])
        w2_cps = [pltpu.make_async_copy(w2_hbm.at[W2B[c]:W2B[c + 1]], w2b.at[W2B[c]:W2B[c + 1]],
                                        sems.at[S_W2 + c]) for c in range(W2C)]

        for cp in wq_cps:
            cp.start()
        for cp in small:
            cp.start()
        for cp in k0_cps:
            cp.start()
        wo_cp.start()
        for j in range(NRING):
            for cp in group_copies(j, True):
                cp.start()

        row_id = lax.broadcasted_iota(jnp.int32, (ROWS, PD), 0)
        col = lax.broadcasted_iota(jnp.int32, (ROWS, PD), 1)
        first_head = col < DH
        diag = jnp.where(first_head, 0, 1) == row_id

        def tile(t):
            return slice(t * LANES, (t + 1) * LANES)

        def rows(t):
            return slice(t * ROWS, (t + 1) * ROWS)

        def mm(a, b_):
            return jnp.dot(a, b_, preferred_element_type=F32)[0:ROWS]

        def q_proj(i, b):
            for c in range(KQ):
                qp[b][rows(c)] = mm(_unpack(xnpk[:, tile(c)]), wqb[i, tile(c), :])

        def qk(i, b, cs=range(KP)):
            for c in cs:
                sp[b][rows(c)] = mm(_unpack(qpk[b][:, tile(c)]), kb[i, rows(c)].reshape(LANES, W))

        def nt(a, b_):
            return lax.dot_general(a, b_, NT_DIMS, preferred_element_type=F32)

        def packed_acc(b):
            return _unpack(jnp.concatenate([acca[b][:, tile(k)] for k in range(NB)], axis=0))

        def combine_parts(i, b, xu, transposed=True):
            g = _unpack(gpk[b][:, tile(0)])
            parts = [jnp.dot(g, _unpack(accb[b][...]), preferred_element_type=F32) if transposed
                     else nt(g, packed_acc(b))]
            for t in range(-(-xu // KP)):
                w = jnp.concatenate([vbuf[i, c * CB:(c + 1) * CB, :, tile(t)].reshape(LANES // 2, LANES)
                                     for c in range(min(KP, xu - t * KP))], axis=1)
                parts.append(jnp.dot(_unpack(gpk[b][:, tile(1 + t)]), _unpack(w),
                                     preferred_element_type=F32))
            return parts

        def combine(i, b, xu):
            for k, part in enumerate(combine_parts(i, b, xu)):
                oraw[b][k * PROWS:(k + 1) * PROWS, 0:part.shape[1]] = part

        def o_proj(i0, n, b):
            for k in range(n):
                for c in range(KP):
                    op[b][rows(k * KP + c)] = mm(_unpack(opk[i0 + k, :, tile(c)]), wob[i0 + k, tile(c), :])

        def row_max(b):
            st[b][:, tile(2)] = jnp.broadcast_to(
                jnp.max(st[b][:, tile(0)], axis=1, keepdims=True), (ROWS, LANES))

        def row_sum(b):
            return jnp.broadcast_to(jnp.sum(gl[b][...], axis=1, keepdims=True), (PROWS, LANES))

        def sum_rows(ref, n, cols=slice(None), off=0):
            s = ref[rows(off), cols]
            for c in range(1, n):
                s = s + ref[rows(off + c), cols]
            return s

        def q_pack(b):
            qpk[b][...] = _pack(jnp.where(diag, sum_rows(qp[b], KQ), 0.0))

        def row(ref, r, cols=slice(None)):
            v = ref[r:r + 1, cols]
            return jnp.broadcast_to(v, (ROWS, v.shape[1]))

        def lane_weights(b, xu):
            g = []
            for r in range(2):
                g.append(_round_bf16(jnp.exp2((row(st[b], r, tile(0)) - row(st[b], r, tile(2))) * scale[...])))
                gl[b][rows(r)] = g[r] * row(st[b], r, tile(1))
            gpk[b][:, tile(0)] = _pack(g[0], g[1])
            for t in range(-(-xu // KP)):
                gpk[b][:, tile(1 + t)] = _pack(g[0] * row(p[b], 0, tile(t)), g[1] * row(p[b], 1, tile(t)))

        def normalise(parts, dn):
            o = parts[0]
            for part in parts[1:]:
                n = part.shape[1]
                o = o + part if n == PD else jnp.concatenate([o[:, :n] + part, o[:, n:]], axis=1)
            o = o * jnp.concatenate([1.0 / dn] * KP, axis=1)
            return _pack(jnp.where(first_head, o[0:ROWS], o[ROWS:PROWS]))

        def stored_parts(b, xu):
            return [oraw[b][k * PROWS:(k + 1) * PROWS, 0:min(KP, xu - (k - 1) * KP) * LANES]
                    for k in range(1 - (-xu // KP))]

        def o_pack(i, b, xu):
            opk[i] = normalise(stored_parts(b, xu), den[b][...])

        def softmax_steps(b):
            NC = 4

            def tree(f, xs):
                while len(xs) > 1:
                    xs = [f(xs[k], xs[k + 1]) for k in range(0, len(xs), 2)]
                return xs[0]

            mc = [None] * NC
            for t in range(NT):
                s = sum_rows(sp[b], KP, tile(t))
                sp[b][rows(0), tile(t)] = s
                mc[t % NC] = s if t < NC else jnp.maximum(mc[t % NC], s)
                yield
            mm_ = tree(jnp.maximum, mc)
            st[b][:, tile(0)] = mm_
            lc = [None] * NC
            sc = scale[...]
            for t in range(NT):
                e = jnp.exp2((sp[b][rows(0), tile(t)] - mm_) * sc)
                p[b][:, tile(t)] = e
                lc[t % NC] = e if t < NC else lc[t % NC] + e
                if t == NT - 1:
                    st[b][:, tile(1)] = tree(jnp.add, lc)
                yield

        def pv_tiles(xu, nbands):
            return [(h, b0, range(len(range(b0 // CB, xu, KP)), NT))
                    for h in range(2) for b0 in range(h * NB // 2, (h + 1) * NB // 2, nbands)]

        def pv_steps(i, b, xu, xt, xo, nbands, gb):
            for h, b0, tiles in pv_tiles(xu, nbands):
                npk = len(tiles) - xt
                order = sorted(tiles, key=lambda t: ((t - tiles[0] + 0.5) / npk if t < NT - xt
                                                     else (t - (NT - xt) + 0.5) / xt))
                groups = range(b0, b0 + nbands, gb)
                acc = {}
                for pos, t in enumerate(order):
                    pb = p[b][h:h + 1, tile(t)]
                    for g0 in groups:
                        u = vbuf[i, g0:g0 + gb, :, tile(t)]
                        if t < NT - xt:
                            lo, hi = _split(u)
                        else:
                            lo, hi = vlo[xo + NT - 1 - t, g0:g0 + gb], u
                        term = pltpu.bitcast(jnp.concatenate([lo, hi], axis=1), F32) * pb
                        acc[g0] = term if pos == 0 else acc[g0] + term
                        if pos == len(order) - 1:
                            for k in range(gb):
                                acca[b][:, tile(g0 + k)] = pltpu.bitcast(acc[g0][k].astype(BF16), U32)
                    yield

        def rewrite_v(i):
            def lookup(table):
                if isinstance(i, int):
                    return table[i]
                v = jnp.int32(table[0])
                for k in range(1, NP):
                    v = jnp.where(i == k, table[k], v)
                return v

            xo = lookup(XO)

            def transpose(u_, carry):
                blk = (i, pl.ds(pl.multiple_of(u_ % KP * CB, CB), CB), slice(None),
                       pl.ds(pl.multiple_of(u_ // KP * LANES, LANES), LANES))
                v32 = pltpu.bitcast(jnp.concatenate(_split(vbuf[blk]), axis=1), F32)
                w = pltpu.bitcast(v32.reshape(LANES, LANES).astype(BF16).T, U32)
                vbuf[blk] = w.reshape(CB, ROWS, LANES)
                return carry

            def unpack(k, carry):
                blk = (i, slice(None), slice(None),
                       pl.ds(pl.multiple_of((NT - 1 - k) * LANES, LANES), LANES))
                lo, hi = _split(vbuf[blk])
                vbuf[blk] = hi
                vlo[xo + k] = lo
                return carry

            lax.fori_loop(0, lookup(XU), transpose, 0)
            lax.fori_loop(0, lookup(XT), unpack, 0)

        def step(j, b, first):
            nb = 1 - b
            static = isinstance(j, int)

            def live(i):
                return not static or 0 <= i < NP

            def at(i):
                return i if static else jnp.clip(i, 0, NP - 1)

            def xu(i):
                return 0 if first or not live(i) else XU[i]

            opn = [0, 0, (NP - 4) // 2, (NP - 4) // 2] if first else OPN
            ops = {NP - 4 + k: (sum(opn[:k]), n) for k, n in enumerate(opn) if n}
            extra = []
            if live(j - 1):
                extra.append(lambda: lane_weights(nb, xu(j - 1)))
            if live(j - 3):
                extra.append(lambda: o_pack(at(j - 3), nb, xu(j - 3)))
            if live(j + 3):
                extra.append(lambda: q_pack(nb))
            if static and j - 1 in ops:
                i0, n = ops[j - 1]
                for k in range(n):
                    def acc_op(k=k):
                        s_ = sum_rows(op[nb], KP, off=k * KP)
                        att[...] = s_ if i0 + k == 0 else att[...] + s_
                    extra.append(acc_op)
            if live(j + 1):
                sm = softmax_steps(nb)
                extra += [lambda: next(sm)] * (2 * NT)
            xt, xo, nbands, gb = (0, 0, NB // 2, NB // 4) if first else (XT[j], XO[j], *PV_BANDS)
            nsteps = sum(len(tiles) for _, _, tiles in pv_tiles(xu(j), nbands))
            done = 0
            for k, _ in enumerate(pv_steps(j, b, xu(j), xt, xo, nbands, gb)):
                upto = (k + 1) * len(extra) // nsteps
                for f in extra[done:upto]:
                    f()
                done = upto
            if live(j + 2):
                qk(j + 2, b)
            if live(j - 2):
                combine(at(j - 2), b, xu(j - 2))
            if live(j + 4):
                q_proj(at(j + 4), b)
            if static and j in ops:
                o_proj(*ops[j], b)
            if live(j - 1):
                accb[nb][...] = pltpu.bitcast(packed_acc(nb).T, U32)
            row_max(b)
            if live(j - 2):
                den[b][...] = row_sum(b)

        state = {}

        def attention(x, first):
            mean, rstd = _ln_stats(x)
            xnpk[...] = _pack(x - mean)
            scale[...] = jnp.broadcast_to(rstd * exp2_scale, (ROWS, LANES))
            if first:
                for ref in (gpk[0].at[:, tile(0)], accb[0], acca[1], oraw[1].at[0:PROWS]):
                    ref[...] = jnp.zeros(ref.shape, ref.dtype)
                for ref in (st[1], gl[0], den[1]):
                    ref[...] = jnp.ones(ref.shape, ref.dtype)
                for cp in wq_cps:
                    cp.wait()
            qpk[0][...] = _pack(jnp.where(diag, _centered_dot(x, mean, wqb[0]), 0.0))
            if first:
                for cp in k0_cps:
                    cp.wait()
            qk(0, 0, (0,))
            q_proj(1, 1)
            q_pack(1)
            qk(0, 0, range(1, KP))
            qk(1, 1)
            q_proj(2, 0)
            q_pack(0)
            q_proj(3, 1)
            for _ in softmax_steps(0):
                pass
            if first:
                wo_cp.wait()

                def reorder_wo(i, carry):
                    for band in range(NB):
                        wobuf[i, rows(band)] = _deinterleave(wobuf[i, rows(band)])
                    return carry
                lax.fori_loop(0, NP, reorder_wo, 0)

            def stream(j):
                if not first:
                    return
                if isinstance(j, int):
                    for cp in group_copies(j, False):
                        cp.wait()
                    return
                for cp in group_copies(j, True):
                    cp.wait()

                @pl.when(j + NRING < NP - 2)
                def _():
                    for cp in group_copies(j + NRING, True):
                        cp.start()

                @pl.when(jnp.logical_and(j + NRING >= NP - 2, j + NRING < NP))
                def _():
                    for cp in group_copies(j + NRING, False):
                        cp.start()

                @pl.when(j + NRING == NP - 1)
                def _():
                    w1_cp.start()
                    for cp in w2_cps:
                        cp.start()

            def run(j, b, cond):
                stream(j)

                @pl.when(cond)
                def _():
                    step(j, b, first)
                if first:
                    rewrite_v(j)

            if first:
                def body(_, j):
                    for b in range(2):
                        run(j + b, b, ((j + b) & 1) == b)
                    return j + 2
                state['zero'] = lax.fori_loop(0, NP // 2 - 1, body, 0) - (NP - 2)
            for j in range(NP - 2 if first else 0, NP):
                run(j, j % 2, state['zero'] + j == j)

            lane_weights(1, 0)
            o2 = combine_parts(NP - 2, 0, 0)
            o1 = combine_parts(NP - 1, 1, 0, transposed=False)
            n_last = (NP - 4) // 2 if first else OPN[-1]
            a = x + att[...] + sum_rows(op[1], n_last * KP)
            a = a + mm(_unpack(opk[NP - 4]), wob[NP - 4])
            a = a + mm(_unpack(normalise(stored_parts(1, 0 if first else XU[NP - 3]), den[1][...])), wob[NP - 3])
            a = a + mm(_unpack(normalise(o2, row_sum(0))), wob[NP - 2])
            a = a + mm(_unpack(normalise(o1, row_sum(1))), wob[NP - 1])
            return _round_bf16(a)

        def ffn(x, first):
            mean, rstd = _ln_stats(x)
            if first:
                w1_cp.wait()
            b1 = b1buf[...].reshape(1, FF).astype(F32)
            b2 = b2buf[...].reshape(1, D).astype(F32)
            h = _centered_dot(x, mean, w1b[...]) * rstd
            h = _gelu_tanh(h + b1).astype(BF16)
            y = x + b2
            bounds = W2B if first else list(range(0, FF + 1, 128))
            for c in range(len(bounds) - 1):
                if first:
                    w2_cps[c].wait()
                yc = jnp.dot(h[:, bounds[c]:bounds[c + 1]], w2b[bounds[c]:bounds[c + 1], :],
                             preferred_element_type=F32)
                y = y + yc
            return _round_bf16(y)

        for cp in small:
            cp.wait()
        x = jnp.broadcast_to(xbuf[0].astype(F32), (ROWS, D))
        for first in (True, False):
            x = attention(x, first)
            x = ffn(x, first)
        o_ref[0] = x[0:1].astype(o_ref.dtype)

    any_spec = pl.BlockSpec(memory_space=pl.ANY)
    return pl.pallas_call(
        kernel,
        out_shape=jax.ShapeDtypeStruct((B, SQ, D), A_x.dtype),
        in_specs=[any_spec] * 9,
        out_specs=pl.BlockSpec(memory_space=pltpu.VMEM),
        scratch_shapes=[
            pltpu.VMEM((NP, NB, ROWS, W), U32),
            pltpu.VMEM((NP, NB, ROWS, W), U32),
            pltpu.VMEM((NP, D // 2, PD), U32),
            pltpu.VMEM((NP, DH, D), U32),
            pltpu.VMEM((D // 2, FF), U32),
            pltpu.VMEM((FF // 2, D), U32),
            pltpu.VMEM((ROWS, D), U32),
            pltpu.VMEM((ROWS, D), F32),
            pltpu.VMEM((NP, ROWS, PD), U32),
            pltpu.VMEM((ROWS, LANES), F32),
            pltpu.VMEM((sum(XT), NB, ROWS, LANES), U32),
            pltpu.SemaphoreType.DMA((1 + W2C + NRING,)),
        ] + [pltpu.VMEM(*pingpong[n]) for n in names for _ in range(2)] + [
            pltpu.VMEM((B, SQ, D), BF16),
            pltpu.VMEM((FF,), BF16),
            pltpu.VMEM((D,), BF16),
        ],
        compiler_params=pltpu.CompilerParams(vmem_limit_bytes=511 * 256 * 1024),
    )(A_x, kt, vt, A_wq, wo3, B_w1, B_b1, B_w2, B_b2)
```

```python
import math

import jax
import jax.numpy as jnp
from jax import lax
import jax.experimental.pallas as pl
import jax.experimental.pallas.tpu as pltpu

F32 = jnp.float32
BF16 = jnp.bfloat16
U32 = jnp.uint32

LANES = 128
ROWS = 8
PROWS = 16
NT_DIMS = (((1,), (1,)), ((), ()))


def _ln_stats(x, eps=1e-5):
    m = jnp.mean(x, axis=-1, keepdims=True)
    c = x - m
    v = jnp.mean(c * c, axis=-1, keepdims=True)
    return m, 1.0 / jnp.sqrt(v + eps)


def _centered_dot(x, m, w):
    lhs = jnp.concatenate([x, jnp.ones_like(x)], axis=0).astype(BF16)
    y = jnp.dot(lhs, w, preferred_element_type=F32)
    return y[0:ROWS] - m * y[ROWS:PROWS]


def _round_bf16(x):
    return x.astype(BF16).astype(F32)


def _gelu_tanh(x):
    c = math.sqrt(2.0 / math.pi)
    return 0.5 * x * (1.0 + jnp.tanh(c * (x + 0.044715 * (x * x * x))))


def _pack(x, y=None):
    y = jnp.zeros_like(x) if y is None else y
    return pltpu.bitcast(jnp.concatenate([x, y], axis=0).astype(BF16), U32)


def _unpack(u):
    return pltpu.bitcast(u, BF16)


def _split(u):
    return u << 16, u & U32(0xFFFF0000)


def _deinterleave(u):
    rows16 = pltpu.bitcast(jnp.concatenate(_split(u), axis=0), F32)
    return pltpu.bitcast(rows16.astype(BF16), U32)


@jax.jit
def pallas_interleave_layers__sliding_block_cached__dense_activation_gelu__decode_kernel(
    A_x: jax.Array,
    A_k_cache: jax.Array,
    A_v_cache: jax.Array,
    A_wq: jax.Array,
    A_wo: jax.Array,
    B_x: jax.Array,
    B_w1: jax.Array,
    B_b1: jax.Array,
    B_w2: jax.Array,
    B_b2: jax.Array,
):
    B, SQ, D = A_x.shape
    _, H, SK, DH = A_k_cache.shape
    FF = B_w1.shape[1]
    assert B == 1 and SQ == 1 and A_wq.shape[1] == H * DH and H % 4 == 0
    W = min(4096, max(256, SK // 4))
    NP = H // 2
    PD = 2 * DH
    NT = W // LANES
    KQ = D // LANES
    KP = PD // LANES
    W2B = [0, FF - 8 * LANES, FF - 4 * LANES, FF - LANES, FF]
    XU = [10, 10, 10, 10, 10, 10, 10, 10, 2, 2, 13, 13, 23, 19, 0, 0]
    XT = [8, 9, 3, 3, 3, 3, 3, 3, 12, 12, 6, 6, 0, 2, 16, 16]
    OPN = [0, 0, 6, 6]
    assert len(XU) == len(XT) == NP and XU[-1] == XU[-2] == 0 and sum(OPN) == NP - 4
    XO = [sum(XT[:i]) for i in range(NP)]
    XN = -(-max(XU) // KP)
    CB = LANES // PROWS
    ND = max(OPN + [(NP - 4) // 2])
    PV_BANDS = (4, 2)
    NRING = 2
    exp2_scale = float(DH) ** -0.5 * math.log2(math.e)

    NB = PD // PROWS
    kt = jnp.transpose(A_k_cache, (0, 1, 3, 2)).reshape(NP, NB, 2, ROWS, SK)
    vt = jnp.transpose(A_v_cache, (0, 1, 3, 2)).reshape(NP, NB, 2, ROWS, SK)
    wo3 = A_wo.reshape(NP, PD, D)

    pingpong = dict(
        qp=((KQ * ROWS, PD), F32),
        qpk=((ROWS, PD), U32),
        sp=((KP * ROWS, W), F32),
        p=((ROWS, W), F32),
        st=((ROWS, 3 * LANES), F32),
        gl=((PROWS, LANES), F32),
        den=((PROWS, LANES), F32),
        acca=((ROWS, NB * LANES), U32),
        accb=((LANES // 2, PD), U32),
        gpk=((ROWS, (1 + XN) * LANES), U32),
        oraw=(((1 + XN) * PROWS, PD), F32),
        op=((ND * KP * ROWS, D), F32),
    )
    names = list(pingpong)

    def kernel(x_hbm, k_hbm, v_hbm, wq_hbm, wo_hbm, w1_hbm, b1_hbm, w2_hbm, b2_hbm,
               o_ref,
               kbuf, vbuf, wqbuf, wobuf, w1buf, w2buf, xnpk, att, opk, scale, vlo, sems, *pp):
        xbuf, b1buf, b2buf = pp[-3:]
        bufs = {n: (pp[2 * k], pp[2 * k + 1]) for k, n in enumerate(names)}
        qp, qpk, sp, p, st, gl, den, acca, accb, gpk, oraw, op = (bufs[n] for n in names)
        kb = kbuf.bitcast(BF16)
        vb = vbuf.bitcast(BF16)
        wqb = wqbuf.bitcast(BF16)
        wob = wobuf.bitcast(BF16)
        w1b = w1buf.bitcast(BF16)
        w2b = w2buf.bitcast(BF16)

        S_A, S_B, S_RING = 0, 1, 2

        def window_copies(hbm, buf, start, n, sem):
            return [pltpu.make_async_copy(
                hbm.at[pl.ds(start, n), :, h, :, pl.ds(SK - W, W)],
                buf.at[pl.ds(start, n), :, pl.ds(h * ROWS, ROWS), :], sem) for h in range(2)]

        def group_copies(j, with_k):
            sem = sems.at[S_RING + j % NRING]
            return ((window_copies(k_hbm, kb, j + 2, 1, sem) if with_k else [])
                    + window_copies(v_hbm, vb, j, 1, sem))

        small = [pltpu.make_async_copy(x_hbm, xbuf, sems.at[S_A]),
                 pltpu.make_async_copy(b1_hbm, b1buf, sems.at[S_A]),
                 pltpu.make_async_copy(b2_hbm, b2buf, sems.at[S_A])]
        wq_cps = [pltpu.make_async_copy(wq_hbm.at[:, i * PD:(i + 1) * PD], wqb.at[i], sems.at[S_A])
                  for i in range(NP)]
        k0_cps = window_copies(k_hbm, kb, 0, 2, sems.at[S_B])
        wo_cp = pltpu.make_async_copy(wo_hbm, wob, sems.at[S_B])
        w1_cp = pltpu.make_async_copy(w1_hbm, w1b, sems.at[S_A])
        w2_cps = [pltpu.make_async_copy(w2_hbm.at[W2B[c]:W2B[c + 1]], w2b.at[W2B[c]:W2B[c + 1]],
                                        sems.at[sem])
                  for c, sem in enumerate((S_B, S_RING + NP % NRING, S_RING + (NP + 1) % NRING, S_A))]

        for cp in wq_cps:
            cp.start()
        for cp in small:
            cp.start()
        for cp in k0_cps:
            cp.start()
        wo_cp.start()
        for j in range(NRING):
            for cp in group_copies(j, True):
                cp.start()

        row_id = lax.broadcasted_iota(jnp.int32, (ROWS, PD), 0)
        col = lax.broadcasted_iota(jnp.int32, (ROWS, PD), 1)
        first_head = col < DH
        diag = jnp.where(first_head, 0, 1) == row_id

        def tile(t):
            return slice(t * LANES, (t + 1) * LANES)

        def rows(t):
            return slice(t * ROWS, (t + 1) * ROWS)

        def mm(a, b_):
            return jnp.dot(a, b_, preferred_element_type=F32)[0:ROWS]

        def q_proj(i, b):
            for c in range(KQ):
                qp[b][rows(c)] = mm(_unpack(xnpk[:, tile(c)]), wqb[i, tile(c), :])

        def qk(i, b, cs=range(KP)):
            for c in cs:
                sp[b][rows(c)] = mm(_unpack(qpk[b][:, tile(c)]), kb[i, rows(c)].reshape(LANES, W))

        def nt(a, b_):
            return lax.dot_general(a, b_, NT_DIMS, preferred_element_type=F32)

        def packed_acc(b):
            return _unpack(jnp.concatenate([acca[b][:, tile(k)] for k in range(NB)], axis=0))

        def combine_parts(i, b, xu, transposed=True):
            g = _unpack(gpk[b][:, tile(0)])
            parts = [jnp.dot(g, _unpack(accb[b][...]), preferred_element_type=F32) if transposed
                     else nt(g, packed_acc(b))]
            for t in range(-(-xu // KP)):
                w = jnp.concatenate([vbuf[i, c * CB:(c + 1) * CB, :, tile(t)].reshape(LANES // 2, LANES)
                                     for c in range(min(KP, xu - t * KP))], axis=1)
                parts.append(jnp.dot(_unpack(gpk[b][:, tile(1 + t)]), _unpack(w),
                                     preferred_element_type=F32))
            return parts

        def combine(i, b, xu):
            for k, part in enumerate(combine_parts(i, b, xu)):
                oraw[b][k * PROWS:(k + 1) * PROWS, 0:part.shape[1]] = part

        def o_proj(i0, n, b):
            for k in range(n):
                for c in range(KP):
                    op[b][rows(k * KP + c)] = mm(_unpack(opk[i0 + k, :, tile(c)]), wob[i0 + k, tile(c), :])

        def row_max(b):
            st[b][:, tile(2)] = jnp.broadcast_to(
                jnp.max(st[b][:, tile(0)], axis=1, keepdims=True), (ROWS, LANES))

        def row_sum(b):
            return jnp.broadcast_to(jnp.sum(gl[b][...], axis=1, keepdims=True), (PROWS, LANES))

        def sum_rows(ref, n, cols=slice(None), off=0):
            s = ref[rows(off), cols]
            for c in range(1, n):
                s = s + ref[rows(off + c), cols]
            return s

        def q_pack(b):
            qpk[b][...] = _pack(jnp.where(diag, sum_rows(qp[b], KQ), 0.0))

        def row(ref, r, cols=slice(None)):
            v = ref[r:r + 1, cols]
            return jnp.broadcast_to(v, (ROWS, v.shape[1]))

        def lane_weights(b, xu):
            g = []
            for r in range(2):
                g.append(_round_bf16(jnp.exp2((row(st[b], r, tile(0)) - row(st[b], r, tile(2))) * scale[...])))
                gl[b][rows(r)] = g[r] * row(st[b], r, tile(1))
            gpk[b][:, tile(0)] = _pack(g[0], g[1])
            for t in range(-(-xu // KP)):
                gpk[b][:, tile(1 + t)] = _pack(g[0] * row(p[b], 0, tile(t)), g[1] * row(p[b], 1, tile(t)))

        def normalise(parts, dn):
            o = parts[0]
            for part in parts[1:]:
                n = part.shape[1]
                o = o + part if n == PD else jnp.concatenate([o[:, :n] + part, o[:, n:]], axis=1)
            o = o * jnp.concatenate([1.0 / dn] * KP, axis=1)
            return _pack(jnp.where(first_head, o[0:ROWS], o[ROWS:PROWS]))

        def stored_parts(b, xu):
            return [oraw[b][k * PROWS:(k + 1) * PROWS, 0:min(KP, xu - (k - 1) * KP) * LANES]
                    for k in range(1 - (-xu // KP))]

        def o_pack(i, b, xu):
            opk[i] = normalise(stored_parts(b, xu), den[b][...])

        def softmax_steps(b):
            NC = 4

            def tree(f, xs):
                while len(xs) > 1:
                    xs = [f(xs[k], xs[k + 1]) for k in range(0, len(xs), 2)]
                return xs[0]

            mc = [None] * NC
            for t in range(NT):
                s = sum_rows(sp[b], KP, tile(t))
                sp[b][rows(0), tile(t)] = s
                mc[t % NC] = s if t < NC else jnp.maximum(mc[t % NC], s)
                yield
            mm_ = tree(jnp.maximum, mc)
            st[b][:, tile(0)] = mm_
            lc = [None] * NC
            sc = scale[...]
            for t in range(NT):
                e = jnp.exp2((sp[b][rows(0), tile(t)] - mm_) * sc)
                p[b][:, tile(t)] = e
                lc[t % NC] = e if t < NC else lc[t % NC] + e
                if t == NT - 1:
                    st[b][:, tile(1)] = tree(jnp.add, lc)
                yield

        def pv_tiles(xu, nbands):
            return [(h, b0, range(len(range(b0 // CB, xu, KP)), NT))
                    for h in range(2) for b0 in range(h * NB // 2, (h + 1) * NB // 2, nbands)]

        def pv_steps(i, b, xu, xt, xo, nbands, gb):
            for h, b0, tiles in pv_tiles(xu, nbands):
                npk = len(tiles) - xt
                order = sorted(tiles, key=lambda t: ((t - tiles[0] + 0.5) / npk if t < NT - xt
                                                     else (t - (NT - xt) + 0.5) / xt))
                groups = range(b0, b0 + nbands, gb)
                acc = {}
                for pos, t in enumerate(order):
                    pb = p[b][h:h + 1, tile(t)]
                    for g0 in groups:
                        u = vbuf[i, g0:g0 + gb, :, tile(t)]
                        if t < NT - xt:
                            lo, hi = _split(u)
                        else:
                            lo, hi = vlo[xo + NT - 1 - t, g0:g0 + gb], u
                        term = pltpu.bitcast(jnp.concatenate([lo, hi], axis=1), F32) * pb
                        acc[g0] = term if pos == 0 else acc[g0] + term
                        if pos == len(order) - 1:
                            for k in range(gb):
                                acca[b][:, tile(g0 + k)] = pltpu.bitcast(acc[g0][k].astype(BF16), U32)
                    yield

        def rewrite_v(i):
            def lookup(table):
                if isinstance(i, int):
                    return table[i]
                v = jnp.int32(table[0])
                for k in range(1, NP):
                    v = jnp.where(i == k, table[k], v)
                return v

            xo = lookup(XO)

            def transpose(u_, carry):
                blk = (i, pl.ds(pl.multiple_of(u_ % KP * CB, CB), CB), slice(None),
                       pl.ds(pl.multiple_of(u_ // KP * LANES, LANES), LANES))
                v32 = pltpu.bitcast(jnp.concatenate(_split(vbuf[blk]), axis=1), F32)
                w = pltpu.bitcast(v32.reshape(LANES, LANES).astype(BF16).T, U32)
                vbuf[blk] = w.reshape(CB, ROWS, LANES)
                return carry

            def unpack(k, carry):
                blk = (i, slice(None), slice(None),
                       pl.ds(pl.multiple_of((NT - 1 - k) * LANES, LANES), LANES))
                lo, hi = _split(vbuf[blk])
                vbuf[blk] = hi
                vlo[xo + k] = lo
                return carry

            lax.fori_loop(0, lookup(XU), transpose, 0)
            lax.fori_loop(0, lookup(XT), unpack, 0)

        def step(j, b, first):
            nb = 1 - b
            static = isinstance(j, int)

            def live(i):
                return not static or 0 <= i < NP

            def at(i):
                return i if static else jnp.clip(i, 0, NP - 1)

            def xu(i):
                return 0 if first or not live(i) else XU[i]

            opn = [0, 0, (NP - 4) // 2, (NP - 4) // 2] if first else OPN
            ops = {NP - 4 + k: (sum(opn[:k]), n) for k, n in enumerate(opn) if n}
            extra = []
            if live(j - 1):
                extra.append(lambda: lane_weights(nb, xu(j - 1)))
            if live(j - 3):
                extra.append(lambda: o_pack(at(j - 3), nb, xu(j - 3)))
            if live(j + 3):
                extra.append(lambda: q_pack(nb))
            if static and j - 1 in ops:
                i0, n = ops[j - 1]
                for k in range(n):
                    def acc_op(k=k):
                        s_ = sum_rows(op[nb], KP, off=k * KP)
                        att[...] = s_ if i0 + k == 0 else att[...] + s_
                    extra.append(acc_op)
            if live(j + 1):
                sm = softmax_steps(nb)
                extra += [lambda: next(sm)] * (2 * NT)
            xt, xo, nbands, gb = (0, 0, NB // 2, NB // 4) if first else (XT[j], XO[j], *PV_BANDS)
            nsteps = sum(len(tiles) for _, _, tiles in pv_tiles(xu(j), nbands))
            done = 0
            for k, _ in enumerate(pv_steps(j, b, xu(j), xt, xo, nbands, gb)):
                upto = (k + 1) * len(extra) // nsteps
                for f in extra[done:upto]:
                    f()
                done = upto
            if live(j + 2):
                qk(j + 2, b)
            if live(j - 2):
                combine(at(j - 2), b, xu(j - 2))
            if live(j + 4):
                q_proj(at(j + 4), b)
            if static and j in ops:
                o_proj(*ops[j], b)
            if live(j - 1):
                accb[nb][...] = pltpu.bitcast(packed_acc(nb).T, U32)
            row_max(b)
            if live(j - 2):
                den[b][...] = row_sum(b)

        state = {}

        def attention(x, first):
            mean, rstd = _ln_stats(x)
            xnpk[...] = _pack(x - mean)
            scale[...] = jnp.broadcast_to(rstd * exp2_scale, (ROWS, LANES))
            if first:
                for ref in (gpk[0].at[:, tile(0)], accb[0], acca[1], oraw[1].at[0:PROWS]):
                    ref[...] = jnp.zeros(ref.shape, ref.dtype)
                for ref in (st[1], gl[0], den[1]):
                    ref[...] = jnp.ones(ref.shape, ref.dtype)
            qpk[0][...] = _pack(jnp.where(diag, _centered_dot(x, mean, wqb[0]), 0.0))
            if first:
                for cp in k0_cps + [wo_cp]:
                    cp.wait()
            qk(0, 0, (0,))
            q_proj(1, 1)
            q_pack(1)
            qk(0, 0, range(1, KP))
            qk(1, 1)
            q_proj(2, 0)
            q_pack(0)
            q_proj(3, 1)
            for _ in softmax_steps(0):
                pass
            if first:
                def reorder_wo(i, carry):
                    for band in range(NB):
                        wobuf[i, rows(band)] = _deinterleave(wobuf[i, rows(band)])
                    return carry
                lax.fori_loop(0, NP, reorder_wo, 0)

            def stream(j):
                if not first:
                    return
                if isinstance(j, int):
                    for cp in group_copies(j, False):
                        cp.wait()
                    w2_cps[j - (NP - 3)].start()
                    return
                for cp in group_copies(j, True):
                    cp.wait()

                @pl.when(j + NRING < NP - 2)
                def _():
                    for cp in group_copies(j + NRING, True):
                        cp.start()

                @pl.when(jnp.logical_and(j + NRING >= NP - 2, j + NRING < NP))
                def _():
                    for cp in group_copies(j + NRING, False):
                        cp.start()

                @pl.when(j + NRING == NP - 1)
                def _():
                    w1_cp.start()
                    w2_cps[0].start()

            def run(j, b, cond):
                stream(j)

                @pl.when(cond)
                def _():
                    step(j, b, first)
                if first:
                    rewrite_v(j)

            if first:
                def body(_, j):
                    for b in range(2):
                        run(j + b, b, ((j + b) & 1) == b)
                    return j + 2
                state['zero'] = lax.fori_loop(0, NP // 2 - 1, body, 0) - (NP - 2)
            for j in range(NP - 2 if first else 0, NP):
                run(j, j % 2, state['zero'] + j == j)

            lane_weights(1, 0)
            o2 = combine_parts(NP - 2, 0, 0)
            o1 = combine_parts(NP - 1, 1, 0, transposed=False)
            n_last = (NP - 4) // 2 if first else OPN[-1]
            a = x + att[...] + sum_rows(op[1], n_last * KP)
            a = a + mm(_unpack(opk[NP - 4]), wob[NP - 4])
            a = a + mm(_unpack(normalise(stored_parts(1, 0 if first else XU[NP - 3]), den[1][...])), wob[NP - 3])
            a = a + mm(_unpack(normalise(o2, row_sum(0))), wob[NP - 2])
            a = a + mm(_unpack(normalise(o1, row_sum(1))), wob[NP - 1])
            return _round_bf16(a)

        def ffn(x, first):
            mean, rstd = _ln_stats(x)
            if first:
                w1_cp.wait()
                w2_cps[-1].start()
            b1 = b1buf[...].reshape(1, FF).astype(F32)
            b2 = b2buf[...].reshape(1, D).astype(F32)
            h = _centered_dot(x, mean, w1b[...]) * rstd
            h = _gelu_tanh(h + b1).astype(BF16)
            y = x + b2
            bounds = W2B if first else list(range(0, FF + 1, 128))
            for c in range(len(bounds) - 1):
                if first:
                    w2_cps[c].wait()
                yc = jnp.dot(h[:, bounds[c]:bounds[c + 1]], w2b[bounds[c]:bounds[c + 1], :],
                             preferred_element_type=F32)
                y = y + yc
            return _round_bf16(y)

        for cp in wq_cps + small:
            cp.wait()
        x = jnp.broadcast_to(xbuf[0].astype(F32), (ROWS, D))
        for first in (True, False):
            x = attention(x, first)
            x = ffn(x, first)
        o_ref[0] = x[0:1].astype(o_ref.dtype)

    any_spec = pl.BlockSpec(memory_space=pl.ANY)
    return pl.pallas_call(
        kernel,
        out_shape=jax.ShapeDtypeStruct((B, SQ, D), A_x.dtype),
        in_specs=[any_spec] * 9,
        out_specs=pl.BlockSpec(memory_space=pltpu.VMEM),
        scratch_shapes=[
            pltpu.VMEM((NP, NB, ROWS, W), U32),
            pltpu.VMEM((NP, NB, ROWS, W), U32),
            pltpu.VMEM((NP, D // 2, PD), U32),
            pltpu.VMEM((NP, DH, D), U32),
            pltpu.VMEM((D // 2, FF), U32),
            pltpu.VMEM((FF // 2, D), U32),
            pltpu.VMEM((ROWS, D), U32),
            pltpu.VMEM((ROWS, D), F32),
            pltpu.VMEM((NP, ROWS, PD), U32),
            pltpu.VMEM((ROWS, LANES), F32),
            pltpu.VMEM((sum(XT), NB, ROWS, LANES), U32),
            pltpu.SemaphoreType.DMA((2 + NRING,)),
        ] + [pltpu.VMEM(*pingpong[n]) for n in names for _ in range(2)] + [
            pltpu.VMEM((B, SQ, D), BF16),
            pltpu.VMEM((FF,), BF16),
            pltpu.VMEM((D,), BF16),
        ],
        compiler_params=pltpu.CompilerParams(vmem_limit_bytes=511 * 256 * 1024),
    )(A_x, kt, vt, A_wq, wo3, B_w1, B_b1, B_w2, B_b2)
```

```python
import math

import jax
import jax.numpy as jnp
from jax import lax
import jax.experimental.pallas as pl
import jax.experimental.pallas.tpu as pltpu

F32 = jnp.float32
BF16 = jnp.bfloat16
U32 = jnp.uint32

LANES = 128
ROWS = 8
PROWS = 16
NT_DIMS = (((1,), (1,)), ((), ()))


def _ln_stats(x, eps=1e-5):
    m = jnp.mean(x, axis=-1, keepdims=True)
    c = x - m
    v = jnp.mean(c * c, axis=-1, keepdims=True)
    return m, 1.0 / jnp.sqrt(v + eps)


def _centered_dot(x, m, w):
    lhs = jnp.concatenate([x, jnp.ones_like(x)], axis=0).astype(BF16)
    y = jnp.dot(lhs, w, preferred_element_type=F32)
    return y[0:ROWS] - m * y[ROWS:PROWS]


def _round_bf16(x):
    return x.astype(BF16).astype(F32)


def _gelu_tanh(x):
    c = math.sqrt(2.0 / math.pi)
    return 0.5 * x * (1.0 + jnp.tanh(c * (x + 0.044715 * (x * x * x))))


def _pack(x, y=None):
    y = jnp.zeros_like(x) if y is None else y
    return pltpu.bitcast(jnp.concatenate([x, y], axis=0).astype(BF16), U32)


def _unpack(u):
    return pltpu.bitcast(u, BF16)


def _split(u):
    return u << 16, u & U32(0xFFFF0000)


def _deinterleave(u):
    rows16 = pltpu.bitcast(jnp.concatenate(_split(u), axis=0), F32)
    return pltpu.bitcast(rows16.astype(BF16), U32)


@jax.jit
def pallas_interleave_layers__sliding_block_cached__dense_activation_gelu__decode_kernel(
    A_x: jax.Array,
    A_k_cache: jax.Array,
    A_v_cache: jax.Array,
    A_wq: jax.Array,
    A_wo: jax.Array,
    B_x: jax.Array,
    B_w1: jax.Array,
    B_b1: jax.Array,
    B_w2: jax.Array,
    B_b2: jax.Array,
):
    B, SQ, D = A_x.shape
    _, H, SK, DH = A_k_cache.shape
    FF = B_w1.shape[1]
    assert B == 1 and SQ == 1 and A_wq.shape[1] == H * DH and H % 4 == 0
    W = min(4096, max(256, SK // 4))
    NP = H // 2
    PD = 2 * DH
    NT = W // LANES
    KQ = D // LANES
    KP = PD // LANES
    W2B = [0, FF - 8 * LANES, FF - 4 * LANES, FF - LANES, FF]
    XU = [10, 10, 10, 10, 10, 10, 10, 10, 2, 2, 13, 13, 23, 19, 0, 0]
    XT = [8, 9, 4, 4, 4, 4, 4, 4, 10, 10, 5, 5, 0, 2, 16, 16]
    OPN = [0, 0, 6, 6]
    assert len(XU) == len(XT) == NP and XU[-1] == XU[-2] == 0 and sum(OPN) == NP - 4
    XO = [sum(XT[:i]) for i in range(NP)]
    XN = -(-max(XU) // KP)
    CB = LANES // PROWS
    ND = max(OPN + [(NP - 4) // 2])
    PV_BANDS = (4, 2)
    NRING = 2
    exp2_scale = float(DH) ** -0.5 * math.log2(math.e)

    NB = PD // PROWS
    kt = jnp.transpose(A_k_cache, (0, 1, 3, 2)).reshape(NP, NB, 2, ROWS, SK)
    vt = jnp.transpose(A_v_cache, (0, 1, 3, 2)).reshape(NP, NB, 2, ROWS, SK)
    wo3 = A_wo.reshape(NP, PD, D)

    pingpong = dict(
        qp=((KQ * ROWS, PD), F32),
        qpk=((ROWS, PD), U32),
        sp=((KP * ROWS, W), F32),
        p=((ROWS, W), F32),
        st=((ROWS, 3 * LANES), F32),
        gl=((PROWS, LANES), F32),
        den=((PROWS, LANES), F32),
        acca=((ROWS, NB * LANES), U32),
        accb=((LANES // 2, PD), U32),
        gpk=((ROWS, (1 + XN) * LANES), U32),
        oraw=(((1 + XN) * PROWS, PD), F32),
        op=((ND * KP * ROWS, D), F32),
    )
    names = list(pingpong)

    def kernel(x_hbm, k_hbm, v_hbm, wq_hbm, wo_hbm, w1_hbm, b1_hbm, w2_hbm, b2_hbm,
               o_ref,
               kbuf, vbuf, wqbuf, wobuf, w1buf, w2buf, xnpk, att, opk, scale, vlo, sems, *pp):
        xbuf, b1buf, b2buf = pp[-3:]
        bufs = {n: (pp[2 * k], pp[2 * k + 1]) for k, n in enumerate(names)}
        qp, qpk, sp, p, st, gl, den, acca, accb, gpk, oraw, op = (bufs[n] for n in names)
        kb = kbuf.bitcast(BF16)
        vb = vbuf.bitcast(BF16)
        wqb = wqbuf.bitcast(BF16)
        wob = wobuf.bitcast(BF16)
        w1b = w1buf.bitcast(BF16)
        w2b = w2buf.bitcast(BF16)

        S_A, S_B, S_RING = 0, 1, 2

        def window_copies(hbm, buf, start, n, sem):
            return [pltpu.make_async_copy(
                hbm.at[pl.ds(start, n), :, h, :, pl.ds(SK - W, W)],
                buf.at[pl.ds(start, n), :, pl.ds(h * ROWS, ROWS), :], sem) for h in range(2)]

        def group_copies(j, with_k):
            sem = sems.at[S_RING + j % NRING]
            return ((window_copies(k_hbm, kb, j + 2, 1, sem) if with_k else [])
                    + window_copies(v_hbm, vb, j, 1, sem))

        small = [pltpu.make_async_copy(x_hbm, xbuf, sems.at[S_A]),
                 pltpu.make_async_copy(b1_hbm, b1buf, sems.at[S_A]),
                 pltpu.make_async_copy(b2_hbm, b2buf, sems.at[S_A])]
        wq_cps = [pltpu.make_async_copy(wq_hbm.at[:, i * PD:(i + 1) * PD], wqb.at[i], sems.at[S_A])
                  for i in range(NP)]
        k0_cps = window_copies(k_hbm, kb, 0, 2, sems.at[S_B])
        wo_cp = pltpu.make_async_copy(wo_hbm, wob, sems.at[S_B])
        w1_cp = pltpu.make_async_copy(w1_hbm, w1b, sems.at[S_A])
        w2_cps = [pltpu.make_async_copy(w2_hbm.at[W2B[c]:W2B[c + 1]], w2b.at[W2B[c]:W2B[c + 1]],
                                        sems.at[sem])
                  for c, sem in enumerate((S_B, S_RING + NP % NRING, S_RING + (NP + 1) % NRING, S_A))]

        for cp in wq_cps:
            cp.start()
        for cp in small:
            cp.start()
        for cp in k0_cps:
            cp.start()
        wo_cp.start()
        for j in range(NRING):
            for cp in group_copies(j, True):
                cp.start()

        row_id = lax.broadcasted_iota(jnp.int32, (ROWS, PD), 0)
        col = lax.broadcasted_iota(jnp.int32, (ROWS, PD), 1)
        first_head = col < DH
        diag = jnp.where(first_head, 0, 1) == row_id

        def tile(t):
            return slice(t * LANES, (t + 1) * LANES)

        def rows(t):
            return slice(t * ROWS, (t + 1) * ROWS)

        def mm(a, b_):
            return jnp.dot(a, b_, preferred_element_type=F32)[0:ROWS]

        def q_proj(i, b):
            for c in range(KQ):
                qp[b][rows(c)] = mm(_unpack(xnpk[:, tile(c)]), wqb[i, tile(c), :])

        def qk(i, b, cs=range(KP)):
            for c in cs:
                sp[b][rows(c)] = mm(_unpack(qpk[b][:, tile(c)]), kb[i, rows(c)].reshape(LANES, W))

        def nt(a, b_):
            return lax.dot_general(a, b_, NT_DIMS, preferred_element_type=F32)

        def packed_acc(b):
            return _unpack(jnp.concatenate([acca[b][:, tile(k)] for k in range(NB)], axis=0))

        def combine_parts(i, b, xu, transposed=True):
            g = _unpack(gpk[b][:, tile(0)])
            parts = [jnp.dot(g, _unpack(accb[b][...]), preferred_element_type=F32) if transposed
                     else nt(g, packed_acc(b))]
            for t in range(-(-xu // KP)):
                w = jnp.concatenate([vbuf[i, c * CB:(c + 1) * CB, :, tile(t)].reshape(LANES // 2, LANES)
                                     for c in range(min(KP, xu - t * KP))], axis=1)
                parts.append(jnp.dot(_unpack(gpk[b][:, tile(1 + t)]), _unpack(w),
                                     preferred_element_type=F32))
            return parts

        def combine(i, b, xu):
            for k, part in enumerate(combine_parts(i, b, xu)):
                oraw[b][k * PROWS:(k + 1) * PROWS, 0:part.shape[1]] = part

        def o_proj(i0, n, b):
            for k in range(n):
                for c in range(KP):
                    op[b][rows(k * KP + c)] = mm(_unpack(opk[i0 + k, :, tile(c)]), wob[i0 + k, tile(c), :])

        def row_max(b):
            st[b][:, tile(2)] = jnp.broadcast_to(
                jnp.max(st[b][:, tile(0)], axis=1, keepdims=True), (ROWS, LANES))

        def row_sum(b):
            return jnp.broadcast_to(jnp.sum(gl[b][...], axis=1, keepdims=True), (PROWS, LANES))

        def sum_rows(ref, n, cols=slice(None), off=0):
            s = ref[rows(off), cols]
            for c in range(1, n):
                s = s + ref[rows(off + c), cols]
            return s

        def q_pack(b):
            qpk[b][...] = _pack(jnp.where(diag, sum_rows(qp[b], KQ), 0.0))

        def row(ref, r, cols=slice(None)):
            v = ref[r:r + 1, cols]
            return jnp.broadcast_to(v, (ROWS, v.shape[1]))

        def lane_weights(b, xu):
            g = []
            for r in range(2):
                g.append(_round_bf16(jnp.exp2((row(st[b], r, tile(0)) - row(st[b], r, tile(2))) * scale[...])))
                gl[b][rows(r)] = g[r] * row(st[b], r, tile(1))
            gpk[b][:, tile(0)] = _pack(g[0], g[1])
            for t in range(-(-xu // KP)):
                gpk[b][:, tile(1 + t)] = _pack(g[0] * row(p[b], 0, tile(t)), g[1] * row(p[b], 1, tile(t)))

        def normalise(parts, dn):
            o = parts[0]
            for part in parts[1:]:
                n = part.shape[1]
                o = o + part if n == PD else jnp.concatenate([o[:, :n] + part, o[:, n:]], axis=1)
            o = o * jnp.concatenate([1.0 / dn] * KP, axis=1)
            return _pack(jnp.where(first_head, o[0:ROWS], o[ROWS:PROWS]))

        def stored_parts(b, xu):
            return [oraw[b][k * PROWS:(k + 1) * PROWS, 0:min(KP, xu - (k - 1) * KP) * LANES]
                    for k in range(1 - (-xu // KP))]

        def o_pack(i, b, xu):
            opk[i] = normalise(stored_parts(b, xu), den[b][...])

        def softmax_steps(b):
            NC = 4

            def tree(f, xs):
                while len(xs) > 1:
                    xs = [f(xs[k], xs[k + 1]) for k in range(0, len(xs), 2)]
                return xs[0]

            mc = [None] * NC
            for t in range(NT):
                s = sum_rows(sp[b], KP, tile(t))
                sp[b][rows(0), tile(t)] = s
                mc[t % NC] = s if t < NC else jnp.maximum(mc[t % NC], s)
                yield
            mm_ = tree(jnp.maximum, mc)
            st[b][:, tile(0)] = mm_
            lc = [None] * NC
            sc = scale[...]
            for t in range(NT):
                e = jnp.exp2((sp[b][rows(0), tile(t)] - mm_) * sc)
                p[b][:, tile(t)] = e
                lc[t % NC] = e if t < NC else lc[t % NC] + e
                if t == NT - 1:
                    st[b][:, tile(1)] = tree(jnp.add, lc)
                yield

        def pv_tiles(xu, nbands):
            return [(h, b0, range(len(range(b0 // CB, xu, KP)), NT))
                    for h in range(2) for b0 in range(h * NB // 2, (h + 1) * NB // 2, nbands)]

        def pv_steps(i, b, xu, xt, xo, nbands, gb):
            for h, b0, tiles in pv_tiles(xu, nbands):
                npk = len(tiles) - xt
                order = sorted(tiles, key=lambda t: ((t - tiles[0] + 0.5) / npk if t < NT - xt
                                                     else (t - (NT - xt) + 0.5) / xt))
                groups = range(b0, b0 + nbands, gb)
                acc = {}
                for pos, t in enumerate(order):
                    pb = p[b][h:h + 1, tile(t)]
                    for g0 in groups:
                        u = vbuf[i, g0:g0 + gb, :, tile(t)]
                        if t < NT - xt:
                            lo, hi = _split(u)
                        else:
                            lo, hi = vlo[xo + NT - 1 - t, g0:g0 + gb], u
                        term = pltpu.bitcast(jnp.concatenate([lo, hi], axis=1), F32) * pb
                        acc[g0] = term if pos == 0 else acc[g0] + term
                        if pos == len(order) - 1:
                            for k in range(gb):
                                acca[b][:, tile(g0 + k)] = pltpu.bitcast(acc[g0][k].astype(BF16), U32)
                    yield

        def rewrite_v(i):
            def lookup(table):
                if isinstance(i, int):
                    return table[i]
                v = jnp.int32(table[0])
                for k in range(1, NP):
                    v = jnp.where(i == k, table[k], v)
                return v

            xo = lookup(XO)

            def transpose(u_, carry):
                blk = (i, pl.ds(pl.multiple_of(u_ % KP * CB, CB), CB), slice(None),
                       pl.ds(pl.multiple_of(u_ // KP * LANES, LANES), LANES))
                v32 = pltpu.bitcast(jnp.concatenate(_split(vbuf[blk]), axis=1), F32)
                w = pltpu.bitcast(v32.reshape(LANES, LANES).astype(BF16).T, U32)
                vbuf[blk] = w.reshape(CB, ROWS, LANES)
                return carry

            def unpack(k, carry):
                blk = (i, slice(None), slice(None),
                       pl.ds(pl.multiple_of((NT - 1 - k) * LANES, LANES), LANES))
                lo, hi = _split(vbuf[blk])
                vbuf[blk] = hi
                vlo[xo + k] = lo
                return carry

            lax.fori_loop(0, lookup(XU), transpose, 0)
            lax.fori_loop(0, lookup(XT), unpack, 0)

        def step(j, b, first):
            nb = 1 - b
            static = isinstance(j, int)

            def live(i):
                return not static or 0 <= i < NP

            def at(i):
                return i if static else jnp.clip(i, 0, NP - 1)

            def xu(i):
                return 0 if first or not live(i) else XU[i]

            opn = [0, 0, (NP - 4) // 2, (NP - 4) // 2] if first else OPN
            ops = {NP - 4 + k: (sum(opn[:k]), n) for k, n in enumerate(opn) if n}
            extra = []
            if live(j - 1):
                extra.append(lambda: lane_weights(nb, xu(j - 1)))
            if live(j - 3):
                extra.append(lambda: o_pack(at(j - 3), nb, xu(j - 3)))
            if live(j + 3):
                extra.append(lambda: q_pack(nb))
            if static and j - 1 in ops:
                i0, n = ops[j - 1]
                for k in range(n):
                    def acc_op(k=k):
                        s_ = sum_rows(op[nb], KP, off=k * KP)
                        att[...] = s_ if i0 + k == 0 else att[...] + s_
                    extra.append(acc_op)
            if live(j + 1):
                sm = softmax_steps(nb)
                assert NT > 6
                short, extra = extra, [lambda: next(sm)] * (2 * NT)
                for k, f in enumerate(short):
                    extra.insert(6 + 5 * k, f)
            extra = [lambda: None] * 3 + extra
            xt, xo, nbands, gb = (0, 0, NB // 2, NB // 4) if first else (XT[j], XO[j], *PV_BANDS)
            nsteps = sum(len(tiles) for _, _, tiles in pv_tiles(xu(j), nbands))
            done = 0
            for k, _ in enumerate(pv_steps(j, b, xu(j), xt, xo, nbands, gb)):
                upto = (k + 1) * len(extra) // nsteps
                for f in extra[done:upto]:
                    f()
                done = upto
            if live(j + 2):
                qk(j + 2, b)
            if live(j - 2):
                combine(at(j - 2), b, xu(j - 2))
            if live(j + 4):
                q_proj(at(j + 4), b)
            if static and j in ops:
                o_proj(*ops[j], b)
            if live(j - 1):
                accb[nb][...] = pltpu.bitcast(packed_acc(nb).T, U32)
            row_max(b)
            if live(j - 2):
                den[b][...] = row_sum(b)

        state = {}

        def attention(x, first):
            mean, rstd = _ln_stats(x)
            xnpk[...] = _pack(x - mean)
            scale[...] = jnp.broadcast_to(rstd * exp2_scale, (ROWS, LANES))
            if first:
                for ref in (gpk[0].at[:, tile(0)], accb[0], acca[1], oraw[1].at[0:PROWS]):
                    ref[...] = jnp.zeros(ref.shape, ref.dtype)
                for ref in (st[1], gl[0], den[1]):
                    ref[...] = jnp.ones(ref.shape, ref.dtype)
            qpk[0][...] = _pack(jnp.where(diag, _centered_dot(x, mean, wqb[0]), 0.0))
            if first:
                for cp in k0_cps + [wo_cp]:
                    cp.wait()
            qk(0, 0, (0,))
            q_proj(1, 1)
            q_pack(1)
            qk(0, 0, range(1, KP))
            qk(1, 1)
            q_proj(2, 0)
            q_pack(0)
            q_proj(3, 1)
            for _ in softmax_steps(0):
                pass
            if first:
                def reorder_wo(i, carry):
                    for band in range(NB):
                        wobuf[i, rows(band)] = _deinterleave(wobuf[i, rows(band)])
                    return carry
                lax.fori_loop(0, NP, reorder_wo, 0)

            def stream(j):
                if not first:
                    return
                if isinstance(j, int):
                    for cp in group_copies(j, False):
                        cp.wait()
                    w2_cps[j - (NP - 3)].start()
                    return
                for cp in group_copies(j, True):
                    cp.wait()

                @pl.when(j + NRING < NP - 2)
                def _():
                    for cp in group_copies(j + NRING, True):
                        cp.start()

                @pl.when(jnp.logical_and(j + NRING >= NP - 2, j + NRING < NP))
                def _():
                    for cp in group_copies(j + NRING, False):
                        cp.start()

                @pl.when(j + NRING == NP - 1)
                def _():
                    w1_cp.start()
                    w2_cps[0].start()

            def run(j, b, cond):
                stream(j)

                @pl.when(cond)
                def _():
                    step(j, b, first)
                if first:
                    rewrite_v(j)

            if first:
                def body(_, j):
                    for b in range(2):
                        run(j + b, b, ((j + b) & 1) == b)
                    return j + 2
                state['zero'] = lax.fori_loop(0, NP // 2 - 1, body, 0) - (NP - 2)
            for j in range(NP - 2 if first else 0, NP):
                run(j, j % 2, state['zero'] + j == j)

            lane_weights(1, 0)
            o2 = combine_parts(NP - 2, 0, 0)
            o1 = combine_parts(NP - 1, 1, 0, transposed=False)
            n_last = (NP - 4) // 2 if first else OPN[-1]
            a = x + att[...] + sum_rows(op[1], n_last * KP)
            a = a + mm(_unpack(opk[NP - 4]), wob[NP - 4])
            a = a + mm(_unpack(normalise(stored_parts(1, 0 if first else XU[NP - 3]), den[1][...])), wob[NP - 3])
            a = a + mm(_unpack(normalise(o2, row_sum(0))), wob[NP - 2])
            a = a + mm(_unpack(normalise(o1, row_sum(1))), wob[NP - 1])
            return _round_bf16(a)

        def ffn(x, first):
            mean, rstd = _ln_stats(x)
            if first:
                w1_cp.wait()
                w2_cps[-1].start()
            b1 = b1buf[...].reshape(1, FF).astype(F32)
            b2 = b2buf[...].reshape(1, D).astype(F32)
            h = _centered_dot(x, mean, w1b[...]) * rstd
            h = _gelu_tanh(h + b1).astype(BF16)
            y = x + b2
            bounds = W2B if first else list(range(0, FF + 1, 128))
            for c in range(len(bounds) - 1):
                if first:
                    w2_cps[c].wait()
                yc = jnp.dot(h[:, bounds[c]:bounds[c + 1]], w2b[bounds[c]:bounds[c + 1], :],
                             preferred_element_type=F32)
                y = y + yc
            return _round_bf16(y)

        for cp in wq_cps + small:
            cp.wait()
        x = jnp.broadcast_to(xbuf[0].astype(F32), (ROWS, D))
        for first in (True, False):
            x = attention(x, first)
            x = ffn(x, first)
        o_ref[0] = x[0:1].astype(o_ref.dtype)

    any_spec = pl.BlockSpec(memory_space=pl.ANY)
    return pl.pallas_call(
        kernel,
        out_shape=jax.ShapeDtypeStruct((B, SQ, D), A_x.dtype),
        in_specs=[any_spec] * 9,
        out_specs=pl.BlockSpec(memory_space=pltpu.VMEM),
        scratch_shapes=[
            pltpu.VMEM((NP, NB, ROWS, W), U32),
            pltpu.VMEM((NP, NB, ROWS, W), U32),
            pltpu.VMEM((NP, D // 2, PD), U32),
            pltpu.VMEM((NP, DH, D), U32),
            pltpu.VMEM((D // 2, FF), U32),
            pltpu.VMEM((FF // 2, D), U32),
            pltpu.VMEM((ROWS, D), U32),
            pltpu.VMEM((ROWS, D), F32),
            pltpu.VMEM((NP, ROWS, PD), U32),
            pltpu.VMEM((ROWS, LANES), F32),
            pltpu.VMEM((sum(XT), NB, ROWS, LANES), U32),
            pltpu.SemaphoreType.DMA((2 + NRING,)),
        ] + [pltpu.VMEM(*pingpong[n]) for n in names for _ in range(2)] + [
            pltpu.VMEM((B, SQ, D), BF16),
            pltpu.VMEM((FF,), BF16),
            pltpu.VMEM((D,), BF16),
        ],
        compiler_params=pltpu.CompilerParams(vmem_limit_bytes=511 * 256 * 1024),
    )(A_x, kt, vt, A_wq, wo3, B_w1, B_b1, B_w2, B_b2)
```

```python
import math

import jax
import jax.numpy as jnp
from jax import lax
import jax.experimental.pallas as pl
import jax.experimental.pallas.tpu as pltpu

F32 = jnp.float32
BF16 = jnp.bfloat16
U32 = jnp.uint32

LANES = 128
ROWS = 8
PROWS = 16
NT_DIMS = (((1,), (1,)), ((), ()))


def _ln_stats(x, eps=1e-5):
    m = jnp.mean(x, axis=-1, keepdims=True)
    c = x - m
    v = jnp.mean(c * c, axis=-1, keepdims=True)
    return m, 1.0 / jnp.sqrt(v + eps)


def _centered_dot(x, m, w):
    lhs = jnp.concatenate([x, jnp.ones_like(x)], axis=0).astype(BF16)
    y = jnp.dot(lhs, w, preferred_element_type=F32)
    return y[0:ROWS] - m * y[ROWS:PROWS]


def _round_bf16(x):
    return x.astype(BF16).astype(F32)


def _gelu_tanh(x):
    c = math.sqrt(2.0 / math.pi)
    return 0.5 * x * (1.0 + jnp.tanh(c * (x + 0.044715 * (x * x * x))))


def _pack(x, y=None):
    y = jnp.zeros_like(x) if y is None else y
    return pltpu.bitcast(jnp.concatenate([x, y], axis=0).astype(BF16), U32)


def _unpack(u):
    return pltpu.bitcast(u, BF16)


def _split(u):
    return u << 16, u & U32(0xFFFF0000)


def _deinterleave(u):
    rows16 = pltpu.bitcast(jnp.concatenate(_split(u), axis=0), F32)
    return pltpu.bitcast(rows16.astype(BF16), U32)


@jax.jit
def pallas_interleave_layers__sliding_block_cached__dense_activation_gelu__decode_kernel(
    A_x: jax.Array,
    A_k_cache: jax.Array,
    A_v_cache: jax.Array,
    A_wq: jax.Array,
    A_wo: jax.Array,
    B_x: jax.Array,
    B_w1: jax.Array,
    B_b1: jax.Array,
    B_w2: jax.Array,
    B_b2: jax.Array,
):
    B, SQ, D = A_x.shape
    _, H, SK, DH = A_k_cache.shape
    FF = B_w1.shape[1]
    assert B == 1 and SQ == 1 and A_wq.shape[1] == H * DH and H % 4 == 0
    W = min(4096, max(256, SK // 4))
    NP = H // 2
    PD = 2 * DH
    NT = W // LANES
    KQ = D // LANES
    KP = PD // LANES
    W2B = [0, FF - 8 * LANES, FF - 4 * LANES, FF - LANES, FF]
    XU = [10, 10, 10, 10, 10, 10, 10, 10, 2, 2, 13, 13, 23, 19, 0, 0]
    XT = [8, 9, 4, 4, 4, 4, 4, 4, 10, 10, 5, 5, 0, 2, 16, 16]
    OPN = [0, 0, 6, 6]
    assert len(XU) == len(XT) == NP and XU[-1] == XU[-2] == 0 and sum(OPN) == NP - 4
    XO = [sum(XT[:i]) for i in range(NP)]
    XN = -(-max(XU) // KP)
    CB = LANES // PROWS
    ND = max(OPN + [(NP - 4) // 2])
    PV_BANDS = (4, 2)
    NRING = 2
    exp2_scale = float(DH) ** -0.5 * math.log2(math.e)

    NB = PD // PROWS
    kt = jnp.transpose(A_k_cache, (0, 1, 3, 2)).reshape(NP, NB, 2, ROWS, SK)
    vt = jnp.transpose(A_v_cache, (0, 1, 3, 2)).reshape(NP, NB, 2, ROWS, SK)
    wo3 = A_wo.reshape(NP, PD, D)

    pingpong = dict(
        qp=((KQ * ROWS, PD), F32),
        qpk=((ROWS, PD), U32),
        sp=((KP * ROWS, W), F32),
        p=((ROWS, W), F32),
        st=((ROWS, 3 * LANES), F32),
        gl=((PROWS, LANES), F32),
        den=((PROWS, LANES), F32),
        acca=((ROWS, NB * LANES), U32),
        accb=((LANES // 2, PD), U32),
        gpk=((ROWS, (1 + XN) * LANES), U32),
        oraw=(((1 + XN) * PROWS, PD), F32),
        op=((ND * KP * ROWS, D), F32),
    )
    names = list(pingpong)

    def kernel(x_hbm, k_hbm, v_hbm, wq_hbm, wo_hbm, w1_hbm, b1_hbm, w2_hbm, b2_hbm,
               o_ref,
               kbuf, vbuf, wqbuf, wobuf, w1buf, w2buf, xnpk, att, opk, scale, vlo, sems, cut, *pp):
        xbuf, b1buf, b2buf = pp[-3:]
        bufs = {n: (pp[2 * k], pp[2 * k + 1]) for k, n in enumerate(names)}
        qp, qpk, sp, p, st, gl, den, acca, accb, gpk, oraw, op = (bufs[n] for n in names)
        kb = kbuf.bitcast(BF16)
        vb = vbuf.bitcast(BF16)
        wqb = wqbuf.bitcast(BF16)
        wob = wobuf.bitcast(BF16)
        w1b = w1buf.bitcast(BF16)
        w2b = w2buf.bitcast(BF16)

        S_A, S_B, S_RING = 0, 1, 2

        def window_copies(hbm, buf, start, n, sem):
            return [pltpu.make_async_copy(
                hbm.at[pl.ds(start, n), :, h, :, pl.ds(SK - W, W)],
                buf.at[pl.ds(start, n), :, pl.ds(h * ROWS, ROWS), :], sem) for h in range(2)]

        def group_copies(j, with_k):
            sem = sems.at[S_RING + j % NRING]
            return ((window_copies(k_hbm, kb, j + 2, 1, sem) if with_k else [])
                    + window_copies(v_hbm, vb, j, 1, sem))

        small = [pltpu.make_async_copy(x_hbm, xbuf, sems.at[S_A]),
                 pltpu.make_async_copy(b1_hbm, b1buf, sems.at[S_A]),
                 pltpu.make_async_copy(b2_hbm, b2buf, sems.at[S_A])]
        wq_cps = [pltpu.make_async_copy(wq_hbm.at[:, i * PD:(i + 1) * PD], wqb.at[i], sems.at[S_A])
                  for i in range(NP)]
        k0_cps = window_copies(k_hbm, kb, 0, 2, sems.at[S_B])
        wo_cp = pltpu.make_async_copy(wo_hbm, wob, sems.at[S_B])
        w1_cp = pltpu.make_async_copy(w1_hbm, w1b, sems.at[S_A])
        w2_cps = [pltpu.make_async_copy(w2_hbm.at[W2B[c]:W2B[c + 1]], w2b.at[W2B[c]:W2B[c + 1]],
                                        sems.at[sem])
                  for c, sem in enumerate((S_B, S_RING + NP % NRING, S_RING + (NP + 1) % NRING, S_A))]

        for cp in wq_cps:
            cp.start()
        for cp in small:
            cp.start()
        for cp in k0_cps:
            cp.start()
        wo_cp.start()
        for j in range(NRING):
            for cp in group_copies(j, True):
                cp.start()

        row_id = lax.broadcasted_iota(jnp.int32, (ROWS, PD), 0)
        col = lax.broadcasted_iota(jnp.int32, (ROWS, PD), 1)
        first_head = col < DH
        diag = jnp.where(first_head, 0, 1) == row_id

        def tile(t):
            return slice(t * LANES, (t + 1) * LANES)

        def rows(t):
            return slice(t * ROWS, (t + 1) * ROWS)

        def mm(a, b_):
            return jnp.dot(a, b_, preferred_element_type=F32)[0:ROWS]

        def q_proj(i, b):
            for c in range(KQ):
                qp[b][rows(c)] = mm(_unpack(xnpk[:, tile(c)]), wqb[i, tile(c), :])

        def qk(i, b, cs=range(KP)):
            for c in cs:
                sp[b][rows(c)] = mm(_unpack(qpk[b][:, tile(c)]), kb[i, rows(c)].reshape(LANES, W))

        def nt(a, b_):
            return lax.dot_general(a, b_, NT_DIMS, preferred_element_type=F32)

        def packed_acc(b):
            return _unpack(jnp.concatenate([acca[b][:, tile(k)] for k in range(NB)], axis=0))

        def combine_parts(i, b, xu, transposed=True):
            g = _unpack(gpk[b][:, tile(0)])
            parts = [jnp.dot(g, _unpack(accb[b][...]), preferred_element_type=F32) if transposed
                     else nt(g, packed_acc(b))]
            for t in range(-(-xu // KP)):
                w = jnp.concatenate([vbuf[i, c * CB:(c + 1) * CB, :, tile(t)].reshape(LANES // 2, LANES)
                                     for c in range(min(KP, xu - t * KP))], axis=1)
                parts.append(jnp.dot(_unpack(gpk[b][:, tile(1 + t)]), _unpack(w),
                                     preferred_element_type=F32))
            return parts

        def combine(i, b, xu):
            for k, part in enumerate(combine_parts(i, b, xu)):
                oraw[b][k * PROWS:(k + 1) * PROWS, 0:part.shape[1]] = part

        def o_proj(i0, n, b):
            for k in range(n):
                for c in range(KP):
                    op[b][rows(k * KP + c)] = mm(_unpack(opk[i0 + k, :, tile(c)]), wob[i0 + k, tile(c), :])

        def row_max(b):
            st[b][:, tile(2)] = jnp.broadcast_to(
                jnp.max(st[b][:, tile(0)], axis=1, keepdims=True), (ROWS, LANES))

        def row_sum(b):
            return jnp.broadcast_to(jnp.sum(gl[b][...], axis=1, keepdims=True), (PROWS, LANES))

        def sum_rows(ref, n, cols=slice(None), off=0):
            s = ref[rows(off), cols]
            for c in range(1, n):
                s = s + ref[rows(off + c), cols]
            return s

        def q_pack(b):
            qpk[b][...] = _pack(jnp.where(diag, sum_rows(qp[b], KQ), 0.0))

        def row(ref, r, cols=slice(None)):
            v = ref[r:r + 1, cols]
            return jnp.broadcast_to(v, (ROWS, v.shape[1]))

        def lane_weights(b, xu):
            g = []
            for r in range(2):
                g.append(_round_bf16(jnp.exp2((row(st[b], r, tile(0)) - row(st[b], r, tile(2))) * scale[...])))
                gl[b][rows(r)] = g[r] * row(st[b], r, tile(1))
            gpk[b][:, tile(0)] = _pack(g[0], g[1])
            for t in range(-(-xu // KP)):
                gpk[b][:, tile(1 + t)] = _pack(g[0] * row(p[b], 0, tile(t)), g[1] * row(p[b], 1, tile(t)))

        def normalise(parts, dn):
            o = parts[0]
            for part in parts[1:]:
                n = part.shape[1]
                o = o + part if n == PD else jnp.concatenate([o[:, :n] + part, o[:, n:]], axis=1)
            o = o * jnp.concatenate([1.0 / dn] * KP, axis=1)
            return _pack(jnp.where(first_head, o[0:ROWS], o[ROWS:PROWS]))

        def stored_parts(b, xu):
            return [oraw[b][k * PROWS:(k + 1) * PROWS, 0:min(KP, xu - (k - 1) * KP) * LANES]
                    for k in range(1 - (-xu // KP))]

        def o_pack(i, b, xu):
            opk[i] = normalise(stored_parts(b, xu), den[b][...])

        def softmax_steps(b):
            NC = 4

            def tree(f, xs):
                while len(xs) > 1:
                    xs = [f(xs[k], xs[k + 1]) for k in range(0, len(xs), 2)]
                return xs[0]

            mc = [None] * NC
            for t in range(NT):
                s = sum_rows(sp[b], KP, tile(t))
                sp[b][rows(0), tile(t)] = s
                mc[t % NC] = s if t < NC else jnp.maximum(mc[t % NC], s)
                yield
            mm_ = tree(jnp.maximum, mc)
            st[b][:, tile(0)] = mm_
            lc = [None] * NC
            sc = scale[...]
            for t in range(NT):
                e = jnp.exp2((sp[b][rows(0), tile(t)] - mm_) * sc)
                p[b][:, tile(t)] = e
                lc[t % NC] = e if t < NC else lc[t % NC] + e
                if t == NT - 1:
                    st[b][:, tile(1)] = tree(jnp.add, lc)
                yield

        def pv_tiles(xu, nbands):
            return [(h, b0, range(len(range(b0 // CB, xu, KP)), NT))
                    for h in range(2) for b0 in range(h * NB // 2, (h + 1) * NB // 2, nbands)]

        def pv_steps(i, b, xu, xt, xo, nbands, gb):
            for h, b0, tiles in pv_tiles(xu, nbands):
                npk = len(tiles) - xt
                order = sorted(tiles, key=lambda t: ((t - tiles[0] + 0.5) / npk if t < NT - xt
                                                     else (t - (NT - xt) + 0.5) / xt))
                groups = range(b0, b0 + nbands, gb)
                acc = {}
                for pos, t in enumerate(order):
                    pb = p[b][h:h + 1, tile(t)]
                    for g0 in groups:
                        u = vbuf[i, g0:g0 + gb, :, tile(t)]
                        if t < NT - xt:
                            lo, hi = _split(u)
                        else:
                            lo, hi = vlo[xo + NT - 1 - t, g0:g0 + gb], u
                        term = pltpu.bitcast(jnp.concatenate([lo, hi], axis=1), F32) * pb
                        acc[g0] = term if pos == 0 else acc[g0] + term
                        if pos == len(order) - 1:
                            for k in range(gb):
                                acca[b][:, tile(g0 + k)] = pltpu.bitcast(acc[g0][k].astype(BF16), U32)
                    yield

        def rewrite_v(i):
            def lookup(table):
                if isinstance(i, int):
                    return table[i]
                v = jnp.int32(table[0])
                for k in range(1, NP):
                    v = jnp.where(i == k, table[k], v)
                return v

            xo = lookup(XO)

            def transpose(u_, carry):
                blk = (i, pl.ds(pl.multiple_of(u_ % KP * CB, CB), CB), slice(None),
                       pl.ds(pl.multiple_of(u_ // KP * LANES, LANES), LANES))
                v32 = pltpu.bitcast(jnp.concatenate(_split(vbuf[blk]), axis=1), F32)
                w = pltpu.bitcast(v32.reshape(LANES, LANES).astype(BF16).T, U32)
                vbuf[blk] = w.reshape(CB, ROWS, LANES)
                return carry

            def unpack(k, carry):
                blk = (i, slice(None), slice(None),
                       pl.ds(pl.multiple_of((NT - 1 - k) * LANES, LANES), LANES))
                lo, hi = _split(vbuf[blk])
                vbuf[blk] = hi
                vlo[xo + k] = lo
                return carry

            lax.fori_loop(0, lookup(XU), transpose, 0)
            lax.fori_loop(0, lookup(XT), unpack, 0)

        def step(j, b, first):
            nb = 1 - b
            static = isinstance(j, int)

            def live(i):
                return not static or 0 <= i < NP

            def at(i):
                return i if static else jnp.clip(i, 0, NP - 1)

            def xu(i):
                return 0 if first or not live(i) else XU[i]

            opn = [0, 0, (NP - 4) // 2, (NP - 4) // 2] if first else OPN
            ops = {NP - 4 + k: (sum(opn[:k]), n) for k, n in enumerate(opn) if n}
            extra = []
            if live(j - 1):
                extra.append(lambda: lane_weights(nb, xu(j - 1)))
            if live(j - 3):
                extra.append(lambda: o_pack(at(j - 3), nb, xu(j - 3)))
            if live(j + 3):
                extra.append(lambda: q_pack(nb))
            if static and j - 1 in ops:
                i0, n = ops[j - 1]
                for k in range(n):
                    def acc_op(k=k):
                        s_ = sum_rows(op[nb], KP, off=k * KP)
                        att[...] = s_ if i0 + k == 0 else att[...] + s_
                    extra.append(acc_op)
            if live(j + 1):
                sm = softmax_steps(nb)
                assert NT > 6
                short, extra = extra, [lambda: next(sm)] * (2 * NT)
                for k, f in enumerate(short):
                    extra.insert(6 + 5 * k, f)
            extra = [lambda: None] * 3 + extra
            xt, xo, nbands, gb = (0, 0, NB // 2, NB // 4) if first else (XT[j], XO[j], *PV_BANDS)
            nsteps = sum(len(tiles) for _, _, tiles in pv_tiles(xu(j), nbands))
            done = 0
            for k, _ in enumerate(pv_steps(j, b, xu(j), xt, xo, nbands, gb)):
                upto = (k + 1) * len(extra) // nsteps
                for f in extra[done:upto]:
                    f()
                done = upto
            if live(j + 2):
                qk(j + 2, b)
            if live(j - 2):
                combine(at(j - 2), b, xu(j - 2))
            if live(j + 4):
                q_proj(at(j + 4), b)
            if static and j in ops:
                o_proj(*ops[j], b)
            if live(j - 1):
                accb[nb][...] = pltpu.bitcast(packed_acc(nb).T, U32)
            row_max(b)
            if live(j - 2):
                den[b][...] = row_sum(b)

        def attention(x, first):
            mean, rstd = _ln_stats(x)
            xnpk[...] = _pack(x - mean)
            scale[...] = jnp.broadcast_to(rstd * exp2_scale, (ROWS, LANES))
            if first:
                for ref in (gpk[0].at[:, tile(0)], accb[0], acca[1], oraw[1].at[0:PROWS]):
                    ref[...] = jnp.zeros(ref.shape, ref.dtype)
                for ref in (st[1], gl[0], den[1]):
                    ref[...] = jnp.ones(ref.shape, ref.dtype)
            qpk[0][...] = _pack(jnp.where(diag, _centered_dot(x, mean, wqb[0]), 0.0))
            if first:
                for cp in k0_cps + [wo_cp]:
                    cp.wait()
            qk(0, 0, (0,))
            q_proj(1, 1)
            q_pack(1)
            qk(0, 0, range(1, KP))
            qk(1, 1)
            q_proj(2, 0)
            q_pack(0)
            q_proj(3, 1)
            for _ in softmax_steps(0):
                pass
            if first:
                def reorder_wo(i, carry):
                    for band in range(NB):
                        wobuf[i, rows(band)] = _deinterleave(wobuf[i, rows(band)])
                    return carry
                lax.fori_loop(0, NP, reorder_wo, 0)

            def stream(j):
                if isinstance(j, int):
                    for cp in group_copies(j, False):
                        cp.wait()
                    w2_cps[j - (NP - 3)].start()
                    return
                for cp in group_copies(j, True):
                    cp.wait()

                @pl.when(j + NRING < NP - 2)
                def _():
                    for cp in group_copies(j + NRING, True):
                        cp.start()

                @pl.when(jnp.logical_and(j + NRING >= NP - 2, j + NRING < NP))
                def _():
                    for cp in group_copies(j + NRING, False):
                        cp.start()

                @pl.when(j + NRING == NP - 1)
                def _():
                    w1_cp.start()
                    w2_cps[0].start()

            if first:
                def run(j, b, always):
                    stream(j)

                    @pl.when(always)
                    def _():
                        step(j, b, first)
                    rewrite_v(j)

                def body(_, j):
                    for b in range(2):
                        run(j + b, b, ((j + b) & 1) == b)
                    return j + 2
                j_end = lax.fori_loop(0, NP // 2 - 1, body, 0)
                for b in range(2):
                    run(NP - 2 + b, b, j_end + b == NP - 2 + b)
            else:
                for j in range(NP):
                    pl.semaphore_signal(cut, 1)
                    step(j, j % 2, first)
                pl.semaphore_wait(cut, NP)

            lane_weights(1, 0)
            o2 = combine_parts(NP - 2, 0, 0)
            o1 = combine_parts(NP - 1, 1, 0, transposed=False)
            n_last = (NP - 4) // 2 if first else OPN[-1]
            a = x + att[...] + sum_rows(op[1], n_last * KP)
            a = a + mm(_unpack(opk[NP - 4]), wob[NP - 4])
            a = a + mm(_unpack(normalise(stored_parts(1, 0 if first else XU[NP - 3]), den[1][...])), wob[NP - 3])
            a = a + mm(_unpack(normalise(o2, row_sum(0))), wob[NP - 2])
            a = a + mm(_unpack(normalise(o1, row_sum(1))), wob[NP - 1])
            return _round_bf16(a)

        def ffn(x, first):
            mean, rstd = _ln_stats(x)
            if first:
                w1_cp.wait()
                w2_cps[-1].start()
            b1 = b1buf[...].reshape(1, FF).astype(F32)
            b2 = b2buf[...].reshape(1, D).astype(F32)
            h = _centered_dot(x, mean, w1b[...]) * rstd
            h = _gelu_tanh(h + b1).astype(BF16)
            y = x + b2
            bounds = W2B if first else list(range(0, FF + 1, 128))
            for c in range(len(bounds) - 1):
                if first:
                    w2_cps[c].wait()
                yc = jnp.dot(h[:, bounds[c]:bounds[c + 1]], w2b[bounds[c]:bounds[c + 1], :],
                             preferred_element_type=F32)
                y = y + yc
            return _round_bf16(y)

        for cp in wq_cps + small:
            cp.wait()
        x = jnp.broadcast_to(xbuf[0].astype(F32), (ROWS, D))
        for first in (True, False):
            x = attention(x, first)
            x = ffn(x, first)
        o_ref[0] = x[0:1].astype(o_ref.dtype)

    any_spec = pl.BlockSpec(memory_space=pl.ANY)
    return pl.pallas_call(
        kernel,
        out_shape=jax.ShapeDtypeStruct((B, SQ, D), A_x.dtype),
        in_specs=[any_spec] * 9,
        out_specs=pl.BlockSpec(memory_space=pltpu.VMEM),
        scratch_shapes=[
            pltpu.VMEM((NP, NB, ROWS, W), U32),
            pltpu.VMEM((NP, NB, ROWS, W), U32),
            pltpu.VMEM((NP, D // 2, PD), U32),
            pltpu.VMEM((NP, DH, D), U32),
            pltpu.VMEM((D // 2, FF), U32),
            pltpu.VMEM((FF // 2, D), U32),
            pltpu.VMEM((ROWS, D), U32),
            pltpu.VMEM((ROWS, D), F32),
            pltpu.VMEM((NP, ROWS, PD), U32),
            pltpu.VMEM((ROWS, LANES), F32),
            pltpu.VMEM((sum(XT), NB, ROWS, LANES), U32),
            pltpu.SemaphoreType.DMA((2 + NRING,)),
            pltpu.SemaphoreType.REGULAR,
        ] + [pltpu.VMEM(*pingpong[n]) for n in names for _ in range(2)] + [
            pltpu.VMEM((B, SQ, D), BF16),
            pltpu.VMEM((FF,), BF16),
            pltpu.VMEM((D,), BF16),
        ],
        compiler_params=pltpu.CompilerParams(vmem_limit_bytes=511 * 256 * 1024),
    )(A_x, kt, vt, A_wq, wo3, B_w1, B_b1, B_w2, B_b2)
```

```python
import math

import jax
import jax.numpy as jnp
from jax import lax
import jax.experimental.pallas as pl
import jax.experimental.pallas.tpu as pltpu

F32 = jnp.float32
BF16 = jnp.bfloat16
U32 = jnp.uint32

LANES = 128
ROWS = 8
PROWS = 16
NT_DIMS = (((1,), (1,)), ((), ()))


def _ln_stats(x, eps=1e-5):
    m = jnp.mean(x, axis=-1, keepdims=True)
    c = x - m
    v = jnp.mean(c * c, axis=-1, keepdims=True)
    return m, 1.0 / jnp.sqrt(v + eps)


def _centered_dot(x, m, w):
    lhs = jnp.concatenate([x, jnp.ones_like(x)], axis=0).astype(BF16)
    y = jnp.dot(lhs, w, preferred_element_type=F32)
    return y[0:ROWS] - m * y[ROWS:PROWS]


def _round_bf16(x):
    return x.astype(BF16).astype(F32)


def _gelu_tanh(x):
    c = math.sqrt(2.0 / math.pi)
    return 0.5 * x * (1.0 + jnp.tanh(c * (x + 0.044715 * (x * x * x))))


def _pack(x, y=None):
    y = jnp.zeros_like(x) if y is None else y
    return pltpu.bitcast(jnp.concatenate([x, y], axis=0).astype(BF16), U32)


def _unpack(u):
    return pltpu.bitcast(u, BF16)


def _split(u):
    return u << 16, u & U32(0xFFFF0000)


def _deinterleave(u):
    rows16 = pltpu.bitcast(jnp.concatenate(_split(u), axis=0), F32)
    return pltpu.bitcast(rows16.astype(BF16), U32)


@jax.jit
def pallas_interleave_layers__sliding_block_cached__dense_activation_gelu__decode_kernel(
    A_x: jax.Array,
    A_k_cache: jax.Array,
    A_v_cache: jax.Array,
    A_wq: jax.Array,
    A_wo: jax.Array,
    B_x: jax.Array,
    B_w1: jax.Array,
    B_b1: jax.Array,
    B_w2: jax.Array,
    B_b2: jax.Array,
):
    B, SQ, D = A_x.shape
    _, H, SK, DH = A_k_cache.shape
    FF = B_w1.shape[1]
    assert B == 1 and SQ == 1 and A_wq.shape[1] == H * DH and H % 4 == 0
    W = min(4096, max(256, SK // 4))
    NP = H // 2
    PD = 2 * DH
    NT = W // LANES
    KQ = D // LANES
    KP = PD // LANES
    W2B = [0, FF - 8 * LANES, FF - 4 * LANES, FF - LANES, FF]
    XU = [17, 17, 17, 10, 10, 10, 10, 10, 2, 2, 13, 13, 23, 19, 0, 0]
    XT = [1, 2, 2, 9, 9, 4, 4, 4, 10, 10, 5, 5, 0, 2, 16, 16]
    OPN = [0, 0, 6, 6]
    assert len(XU) == len(XT) == NP and XU[-1] == XU[-2] == 0 and sum(OPN) == NP - 4
    XO = [sum(XT[:i]) for i in range(NP)]
    VQ = [3, 6, 7, 8]
    VF = 4
    assert 3 in VQ
    XN = -(-max(XU) // KP)
    CB = LANES // PROWS
    ND = max(OPN + [(NP - 4) // 2])
    PV_BANDS = (4, 2)
    NRING = 2
    exp2_scale = float(DH) ** -0.5 * math.log2(math.e)

    NB = PD // PROWS
    kt = jnp.transpose(A_k_cache, (0, 1, 3, 2)).reshape(NP, NB, 2, ROWS, SK)
    vt = jnp.transpose(A_v_cache, (0, 1, 3, 2)).reshape(NP, NB, 2, ROWS, SK)
    wo3 = A_wo.reshape(NP, PD, D)

    pingpong = dict(
        qp=(((KQ + (len(VQ) + 1) // 2) * ROWS, PD), F32),
        qpk=((ROWS, PD), U32),
        sp=((KP * ROWS, W), F32),
        p=((ROWS, W), F32),
        st=((ROWS, 3 * LANES), F32),
        gl=((PROWS, LANES), F32),
        den=((PROWS, LANES), F32),
        acca=((ROWS, NB * LANES), U32),
        accb=((LANES // 2, PD), U32),
        gpk=((ROWS, (1 + XN) * LANES), U32),
        oraw=(((1 + XN) * PROWS, PD), F32),
        op=((ND * KP * ROWS, D), F32),
    )
    names = list(pingpong)

    def kernel(x_hbm, k_hbm, v_hbm, wq_hbm, wo_hbm, w1_hbm, b1_hbm, w2_hbm, b2_hbm,
               o_ref,
               kbuf, vbuf, wqbuf, wobuf, w1buf, w2buf, xnpk, att, opk, scale, vlo, xcol, sems, cut, *pp):
        q2pk = opk.at[NP - 1]
        xbuf, b1buf, b2buf = pp[-3:]
        bufs = {n: (pp[2 * k], pp[2 * k + 1]) for k, n in enumerate(names)}
        qp, qpk, sp, p, st, gl, den, acca, accb, gpk, oraw, op = (bufs[n] for n in names)
        kb = kbuf.bitcast(BF16)
        vb = vbuf.bitcast(BF16)
        wqb = wqbuf.bitcast(BF16)
        wob = wobuf.bitcast(BF16)
        w1b = w1buf.bitcast(BF16)
        w2b = w2buf.bitcast(BF16)

        S_A, S_B, S_RING = 0, 1, 2

        def window_copies(hbm, buf, start, n, sem):
            return [pltpu.make_async_copy(
                hbm.at[pl.ds(start, n), :, h, :, pl.ds(SK - W, W)],
                buf.at[pl.ds(start, n), :, pl.ds(h * ROWS, ROWS), :], sem) for h in range(2)]

        def group_copies(j, with_k):
            sem = sems.at[S_RING + j % NRING]
            return ((window_copies(k_hbm, kb, j + 2, 1, sem) if with_k else [])
                    + window_copies(v_hbm, vb, j, 1, sem))

        small = [pltpu.make_async_copy(x_hbm, xbuf, sems.at[S_A]),
                 pltpu.make_async_copy(b1_hbm, b1buf, sems.at[S_A]),
                 pltpu.make_async_copy(b2_hbm, b2buf, sems.at[S_A])]
        wq_cps = [pltpu.make_async_copy(wq_hbm.at[:, i * PD:(i + 1) * PD], wqb.at[i], sems.at[S_A])
                  for i in range(NP)]
        k0_cps = window_copies(k_hbm, kb, 0, 2, sems.at[S_B])
        wo_cp = pltpu.make_async_copy(wo_hbm, wob, sems.at[S_B])
        w1_cp = pltpu.make_async_copy(w1_hbm, w1b, sems.at[S_A])
        w2_cps = [pltpu.make_async_copy(w2_hbm.at[W2B[c]:W2B[c + 1]], w2b.at[W2B[c]:W2B[c + 1]],
                                        sems.at[sem])
                  for c, sem in enumerate((S_B, S_RING + NP % NRING, S_RING + (NP + 1) % NRING, S_A))]

        for cp in wq_cps:
            cp.start()
        for cp in small:
            cp.start()
        for cp in k0_cps:
            cp.start()
        wo_cp.start()
        for j in range(NRING):
            for cp in group_copies(j, True):
                cp.start()

        row_id = lax.broadcasted_iota(jnp.int32, (ROWS, PD), 0)
        col = lax.broadcasted_iota(jnp.int32, (ROWS, PD), 1)
        first_head = col < DH
        diag = jnp.where(first_head, 0, 1) == row_id

        def tile(t):
            return slice(t * LANES, (t + 1) * LANES)

        def rows(t):
            return slice(t * ROWS, (t + 1) * ROWS)

        def mm(a, b_):
            return jnp.dot(a, b_, preferred_element_type=F32)[0:ROWS]

        def q_proj(i, b):
            for c in range(KQ):
                qp[b][rows(c)] = mm(_unpack(xnpk[:, tile(c)]), wqb[i, tile(c), :])

        def qk(i, b, cs=range(KP), q_ref=None):
            q_ref = qpk[b] if q_ref is None else q_ref
            for c in cs:
                sp[b][rows(c)] = mm(_unpack(q_ref[:, tile(c)]), kb[i, rows(c)].reshape(LANES, W))

        def columns(xpk):
            return pltpu.bitcast(jnp.concatenate([_unpack(xpk)] * CB, axis=0).T, U32)

        def nt(a, b_):
            return lax.dot_general(a, b_, NT_DIMS, preferred_element_type=F32)

        def packed_acc(b):
            return _unpack(jnp.concatenate([acca[b][:, tile(k)] for k in range(NB)], axis=0))

        def combine_parts(i, b, xu, transposed=True):
            g = _unpack(gpk[b][:, tile(0)])
            parts = [jnp.dot(g, _unpack(accb[b][...]), preferred_element_type=F32) if transposed
                     else nt(g, packed_acc(b))]
            for t in range(-(-xu // KP)):
                w = jnp.concatenate([vbuf[i, c * CB:(c + 1) * CB, :, tile(t)].reshape(LANES // 2, LANES)
                                     for c in range(min(KP, xu - t * KP))], axis=1)
                parts.append(jnp.dot(_unpack(gpk[b][:, tile(1 + t)]), _unpack(w),
                                     preferred_element_type=F32))
            return parts

        def combine(i, b, xu):
            for k, part in enumerate(combine_parts(i, b, xu)):
                oraw[b][k * PROWS:(k + 1) * PROWS, 0:part.shape[1]] = part

        def o_proj(i0, n, b):
            for k in range(n):
                for c in range(KP):
                    op[b][rows(k * KP + c)] = mm(_unpack(opk[i0 + k, :, tile(c)]), wob[i0 + k, tile(c), :])

        def row_max(b):
            st[b][:, tile(2)] = jnp.broadcast_to(
                jnp.max(st[b][:, tile(0)], axis=1, keepdims=True), (ROWS, LANES))

        def row_sum(b):
            return jnp.broadcast_to(jnp.sum(gl[b][...], axis=1, keepdims=True), (PROWS, LANES))

        def sum_rows(ref, n, cols=slice(None), off=0):
            s = ref[rows(off), cols]
            for c in range(1, n):
                s = s + ref[rows(off + c), cols]
            return s

        def q_pack(b):
            qpk[b][...] = _pack(jnp.where(diag, sum_rows(qp[b], KQ), 0.0))

        def row(ref, r, cols=slice(None)):
            v = ref[r:r + 1, cols]
            return jnp.broadcast_to(v, (ROWS, v.shape[1]))

        def lane_weights(b, xu):
            g = []
            for r in range(2):
                g.append(_round_bf16(jnp.exp2((row(st[b], r, tile(0)) - row(st[b], r, tile(2))) * scale[...])))
                gl[b][rows(r)] = g[r] * row(st[b], r, tile(1))
            gpk[b][:, tile(0)] = _pack(g[0], g[1])
            for t in range(-(-xu // KP)):
                gpk[b][:, tile(1 + t)] = _pack(g[0] * row(p[b], 0, tile(t)), g[1] * row(p[b], 1, tile(t)))

        def normalise(parts, dn):
            o = parts[0]
            for part in parts[1:]:
                n = part.shape[1]
                o = o + part if n == PD else jnp.concatenate([o[:, :n] + part, o[:, n:]], axis=1)
            o = o * jnp.concatenate([1.0 / dn] * KP, axis=1)
            o = jnp.where(first_head, o[0:ROWS], o[ROWS:PROWS])
            return _pack(o, o)

        def vector_matvec(xpk, w_ref):
            acc = None
            for c in range(xpk.shape[1] // LANES):
                cols = [pltpu.bitcast(v, F32) for v in _split(columns(xpk[:, tile(c)]))]
                for r in range(CB):
                    w = [pltpu.bitcast(v, F32) for v in _split(w_ref[rows(c * CB + r), :])]
                    reps = w[0].shape[1] // LANES
                    term = (w[0] * jnp.concatenate([cols[0][rows(r)]] * reps, axis=1)
                            + w[1] * jnp.concatenate([cols[1][rows(r)]] * reps, axis=1))
                    acc = term if acc is None else acc + term
            return jnp.broadcast_to(jnp.sum(acc, axis=0, keepdims=True), acc.shape)

        def vector_q(items, other=iter(())):
            acc = {}
            for band in range(D // PROWS):
                next(other, None)
                ce, co = (jnp.concatenate([pltpu.bitcast(v, F32)] * KP, axis=1)
                          for v in _split(xcol[rows(band)]))
                for i in items:
                    we, wo_ = (pltpu.bitcast(v, F32) for v in _split(wqbuf[i, rows(band)]))
                    term = we * ce + wo_ * co
                    acc[i] = term if band == 0 else acc[i] + term
            return acc

        def vector_q_slot(i):
            k = VQ.index(i)
            return qp[k % 2], (KQ + k // 2) * ROWS

        def vector_q_pack(i, b):
            ref, r0 = vector_q_slot(i)
            q = []
            for c in range(KP):
                q.append(row(ref, r0, tile(c)))
                for r in range(1, ROWS):
                    q[c] = q[c] + row(ref, r0 + r, tile(c))
            qpk[b][...] = _pack(jnp.where(diag, jnp.concatenate(q, axis=1), 0.0))

        def stored_parts(b, xu):
            return [oraw[b][k * PROWS:(k + 1) * PROWS, 0:min(KP, xu - (k - 1) * KP) * LANES]
                    for k in range(1 - (-xu // KP))]

        def o_pack(i, b, xu):
            opk[i] = normalise(stored_parts(b, xu), den[b][...])

        def softmax_steps(b):
            NC = 4

            def tree(f, xs):
                while len(xs) > 1:
                    xs = [f(xs[k], xs[k + 1]) for k in range(0, len(xs), 2)]
                return xs[0]

            mc = [None] * NC
            for t in range(NT):
                s = sum_rows(sp[b], KP, tile(t))
                sp[b][rows(0), tile(t)] = s
                mc[t % NC] = s if t < NC else jnp.maximum(mc[t % NC], s)
                yield
            mm_ = tree(jnp.maximum, mc)
            st[b][:, tile(0)] = mm_
            lc = [None] * NC
            sc = scale[...]
            for t in range(NT):
                e = jnp.exp2((sp[b][rows(0), tile(t)] - mm_) * sc)
                p[b][:, tile(t)] = e
                lc[t % NC] = e if t < NC else lc[t % NC] + e
                if t == NT - 1:
                    st[b][:, tile(1)] = tree(jnp.add, lc)
                yield

        def pv_tiles(xu, nbands):
            return [(h, b0, range(len(range(b0 // CB, xu, KP)), NT))
                    for h in range(2) for b0 in range(h * NB // 2, (h + 1) * NB // 2, nbands)]

        def pv_steps(i, b, xu, xt, xo, nbands, gb):
            for h, b0, tiles in pv_tiles(xu, nbands):
                npk = len(tiles) - xt
                order = sorted(tiles, key=lambda t: ((t - tiles[0] + 0.5) / npk if t < NT - xt
                                                     else (t - (NT - xt) + 0.5) / xt))
                groups = range(b0, b0 + nbands, gb)
                acc = {}
                for pos, t in enumerate(order):
                    pb = p[b][h:h + 1, tile(t)]
                    for g0 in groups:
                        u = vbuf[i, g0:g0 + gb, :, tile(t)]
                        if t < NT - xt:
                            lo, hi = _split(u)
                        else:
                            lo, hi = vlo[xo + NT - 1 - t, g0:g0 + gb], u
                        term = pltpu.bitcast(jnp.concatenate([lo, hi], axis=1), F32) * pb
                        acc[g0] = term if pos == 0 else acc[g0] + term
                        if pos == len(order) - 1:
                            for k in range(gb):
                                acca[b][:, tile(g0 + k)] = pltpu.bitcast(acc[g0][k].astype(BF16), U32)
                    yield

        def rewrite_v(i):
            def lookup(table):
                if isinstance(i, int):
                    return table[i]
                v = jnp.int32(table[0])
                for k in range(1, NP):
                    v = jnp.where(i == k, table[k], v)
                return v

            xo = lookup(XO)

            def transpose(u_, carry):
                blk = (i, pl.ds(pl.multiple_of(u_ % KP * CB, CB), CB), slice(None),
                       pl.ds(pl.multiple_of(u_ // KP * LANES, LANES), LANES))
                v32 = pltpu.bitcast(jnp.concatenate(_split(vbuf[blk]), axis=1), F32)
                w = pltpu.bitcast(v32.reshape(LANES, LANES).astype(BF16).T, U32)
                vbuf[blk] = w.reshape(CB, ROWS, LANES)
                return carry

            def unpack(k, carry):
                blk = (i, slice(None), slice(None),
                       pl.ds(pl.multiple_of((NT - 1 - k) * LANES, LANES), LANES))
                lo, hi = _split(vbuf[blk])
                vbuf[blk] = hi
                vlo[xo + k] = lo
                return carry

            lax.fori_loop(0, lookup(XU), transpose, 0)
            lax.fori_loop(0, lookup(XT), unpack, 0)

        def step(j, b, first):
            nb = 1 - b
            static = isinstance(j, int)

            def live(i):
                return not static or 0 <= i < NP

            def at(i):
                return i if static else jnp.clip(i, 0, NP - 1)

            def xu(i):
                return 0 if first or not live(i) else XU[i]

            opn = [0, 0, (NP - 4) // 2, (NP - 4) // 2] if first else OPN
            ops = {NP - 4 + k: (sum(opn[:k]), n) for k, n in enumerate(opn) if n}
            extra = []
            if live(j - 1):
                extra.append(lambda: lane_weights(nb, xu(j - 1)))
            if live(j - 3):
                extra.append(lambda: o_pack(at(j - 3), nb, xu(j - 3)))
            if live(j + 3):
                extra.append(lambda: q_pack(nb) if first or j + 3 not in VQ
                             else vector_q_pack(j + 3, nb))
            if static and j - 1 in ops:
                i0, n = ops[j - 1]
                for k in range(n):
                    def acc_op(k=k):
                        s_ = sum_rows(op[nb], KP, off=k * KP)
                        att[...] = s_ if i0 + k == 0 else att[...] + s_
                    extra.append(acc_op)
            if live(j + 1):
                sm = softmax_steps(nb)
                assert NT > 6
                short, extra = extra, [lambda: next(sm)] * (2 * NT)
                for k, f in enumerate(short):
                    extra.insert(6 + 5 * k, f)
            extra = [lambda: None] * 3 + extra
            xt, xo, nbands, gb = (0, 0, NB // 2, NB // 4) if first else (XT[j], XO[j], *PV_BANDS)
            nsteps = sum(len(tiles) for _, _, tiles in pv_tiles(xu(j), nbands))
            done = 0
            for k, _ in enumerate(pv_steps(j, b, xu(j), xt, xo, nbands, gb)):
                upto = (k + 1) * len(extra) // nsteps
                for f in extra[done:upto]:
                    f()
                done = upto
            if live(j + 2):
                qk(j + 2, b, q_ref=q2pk if not first and j == 0 else None)
            if live(j - 2):
                combine(at(j - 2), b, xu(j - 2))
            if live(j + 4) and (first or j + 4 not in VQ):
                q_proj(at(j + 4), b)
            if static and j in ops:
                o_proj(*ops[j], b)
            if live(j - 1):
                accb[nb][...] = pltpu.bitcast(packed_acc(nb).T, U32)
            row_max(b)
            if live(j - 2):
                den[b][...] = row_sum(b)

        def attention(x, first):
            mean, rstd = _ln_stats(x)
            xnpk[...] = _pack(x - mean, x - mean)
            scale[...] = jnp.broadcast_to(rstd * exp2_scale, (ROWS, LANES))
            if first:
                for ref in (gpk[0].at[:, tile(0)], accb[0], acca[1], oraw[1].at[0:PROWS]):
                    ref[...] = jnp.zeros(ref.shape, ref.dtype)
                for ref in (st[1], gl[0], den[1]):
                    ref[...] = jnp.ones(ref.shape, ref.dtype)
            qpk[0][...] = _pack(jnp.where(diag, _centered_dot(x, mean, wqb[0]), 0.0))
            if first:
                for cp in k0_cps + [wo_cp]:
                    cp.wait()
                qk(0, 0)
                q_proj(1, 1)
                q_pack(1)
                qk(1, 1)
                q_proj(2, 0)
                q_pack(0)
                q_proj(3, 1)
                for _ in softmax_steps(0):
                    pass

                def reorder_wo(i, carry):
                    for band in range(NB):
                        wobuf[i, rows(band)] = _deinterleave(wobuf[i, rows(band)])
                    return carry
                lax.fori_loop(0, NP, reorder_wo, 0)
            else:
                qpk[1][...] = _pack(jnp.where(diag, _centered_dot(x, mean, wqb[1]), 0.0))
                for c in range(KQ):
                    xcol[c * LANES // 2:(c + 1) * LANES // 2] = columns(xnpk[:, tile(c)])
                qk(0, 0)
                q = jnp.sum(vector_q([2])[2], axis=0, keepdims=True)
                q2pk[...] = _pack(jnp.where(diag, jnp.broadcast_to(q, (ROWS, PD)), 0.0))
                pl.semaphore_signal(cut, 1)
                sm = softmax_steps(0)
                for k in range(0, len(VQ), 2):
                    for i, acc in vector_q(VQ[k:k + 2], sm).items():
                        ref, r0 = vector_q_slot(i)
                        ref[r0:r0 + ROWS] = acc
                for _ in sm:
                    pass
                qk(1, 1)

            def stream(j):
                if isinstance(j, int):
                    for cp in group_copies(j, False):
                        cp.wait()
                    w2_cps[j - (NP - 3)].start()
                    return
                for cp in group_copies(j, True):
                    cp.wait()

                @pl.when(j + NRING < NP - 2)
                def _():
                    for cp in group_copies(j + NRING, True):
                        cp.start()

                @pl.when(jnp.logical_and(j + NRING >= NP - 2, j + NRING < NP))
                def _():
                    for cp in group_copies(j + NRING, False):
                        cp.start()

                @pl.when(j + NRING == NP - 1)
                def _():
                    w1_cp.start()
                    w2_cps[0].start()

            if first:
                def run(j, b, always):
                    stream(j)

                    @pl.when(always)
                    def _():
                        step(j, b, first)
                    rewrite_v(j)

                def body(_, j):
                    for b in range(2):
                        run(j + b, b, ((j + b) & 1) == b)
                    return j + 2
                j_end = lax.fori_loop(0, NP // 2 - 1, body, 0)
                for b in range(2):
                    run(NP - 2 + b, b, j_end + b == NP - 2 + b)
            else:
                for j in range(NP):
                    pl.semaphore_signal(cut, 1)
                    step(j, j % 2, first)
                pl.semaphore_wait(cut, NP + 1)

            lane_weights(1, 0)
            o2 = combine_parts(NP - 2, 0, 0)
            o1 = combine_parts(NP - 1, 1, 0, transposed=False)
            n_last = (NP - 4) // 2 if first else OPN[-1]
            a = x + att[...] + sum_rows(op[1], n_last * KP)
            a = a + vector_matvec(opk[NP - 4], wobuf.at[NP - 4])
            a = a + mm(_unpack(normalise(stored_parts(1, 0 if first else XU[NP - 3]), den[1][...])), wob[NP - 3])
            a = a + mm(_unpack(normalise(o2, row_sum(0))), wob[NP - 2])
            a = a + mm(_unpack(normalise(o1, row_sum(1))), wob[NP - 1])
            return _round_bf16(a)

        def ffn(x, first):
            mean, rstd = _ln_stats(x)
            if first:
                w1_cp.wait()
                w2_cps[-1].start()
            b1 = b1buf[...].reshape(1, FF).astype(F32)
            b2 = b2buf[...].reshape(1, D).astype(F32)
            h = _centered_dot(x, mean, w1b[...]) * rstd
            h32 = _gelu_tanh(h + b1)
            h = h32.astype(BF16)
            y = x + b2
            bounds = W2B if first else list(range(VF * LANES, FF + 1, LANES))
            if not first:
                hv = h32[:, 0:VF * LANES]
                y = y + vector_matvec(_pack(hv, hv), w2buf.at[0:VF * LANES // 2])
            for c in range(len(bounds) - 1):
                if first:
                    w2_cps[c].wait()
                yc = jnp.dot(h[:, bounds[c]:bounds[c + 1]], w2b[bounds[c]:bounds[c + 1], :],
                             preferred_element_type=F32)
                y = y + yc
            return _round_bf16(y)

        for cp in wq_cps + small:
            cp.wait()
        x = jnp.broadcast_to(xbuf[0].astype(F32), (ROWS, D))
        for first in (True, False):
            x = attention(x, first)
            x = ffn(x, first)
        o_ref[0] = x[0:1].astype(o_ref.dtype)

    any_spec = pl.BlockSpec(memory_space=pl.ANY)
    return pl.pallas_call(
        kernel,
        out_shape=jax.ShapeDtypeStruct((B, SQ, D), A_x.dtype),
        in_specs=[any_spec] * 9,
        out_specs=pl.BlockSpec(memory_space=pltpu.VMEM),
        scratch_shapes=[
            pltpu.VMEM((NP, NB, ROWS, W), U32),
            pltpu.VMEM((NP, NB, ROWS, W), U32),
            pltpu.VMEM((NP, D // 2, PD), U32),
            pltpu.VMEM((NP, DH, D), U32),
            pltpu.VMEM((D // 2, FF), U32),
            pltpu.VMEM((FF // 2, D), U32),
            pltpu.VMEM((ROWS, D), U32),
            pltpu.VMEM((ROWS, D), F32),
            pltpu.VMEM((NP, ROWS, PD), U32),
            pltpu.VMEM((ROWS, LANES), F32),
            pltpu.VMEM((sum(XT), NB, ROWS, LANES), U32),
            pltpu.VMEM((D // 2, LANES), U32),
            pltpu.SemaphoreType.DMA((2 + NRING,)),
            pltpu.SemaphoreType.REGULAR,
        ] + [pltpu.VMEM(*pingpong[n]) for n in names for _ in range(2)] + [
            pltpu.VMEM((B, SQ, D), BF16),
            pltpu.VMEM((FF,), BF16),
            pltpu.VMEM((D,), BF16),
        ],
        compiler_params=pltpu.CompilerParams(vmem_limit_bytes=2047 * 64 * 1024),
    )(A_x, kt, vt, A_wq, wo3, B_w1, B_b1, B_w2, B_b2)
```

```python
import math

import jax
import jax.numpy as jnp
from jax import lax
import jax.experimental.pallas as pl
import jax.experimental.pallas.tpu as pltpu

F32 = jnp.float32
BF16 = jnp.bfloat16
U32 = jnp.uint32

LANES = 128
ROWS = 8
PROWS = 16
NT_DIMS = (((1,), (1,)), ((), ()))


def _ln_stats(x, eps=1e-5):
    m = jnp.mean(x, axis=-1, keepdims=True)
    c = x - m
    v = jnp.mean(c * c, axis=-1, keepdims=True)
    return m, 1.0 / jnp.sqrt(v + eps)


def _centered_dot(x, m, w):
    lhs = jnp.concatenate([x, jnp.ones_like(x)], axis=0).astype(BF16)
    y = jnp.dot(lhs, w, preferred_element_type=F32)
    return y[0:ROWS] - m * y[ROWS:PROWS]


def _round_bf16(x):
    return x.astype(BF16).astype(F32)


def _gelu_tanh(x):
    c = math.sqrt(2.0 / math.pi)
    return 0.5 * x * (1.0 + jnp.tanh(c * (x + 0.044715 * (x * x * x))))


def _pack(x, y=None):
    y = jnp.zeros_like(x) if y is None else y
    return pltpu.bitcast(jnp.concatenate([x, y], axis=0).astype(BF16), U32)


def _unpack(u):
    return pltpu.bitcast(u, BF16)


def _split(u):
    return u << 16, u & U32(0xFFFF0000)


def _deinterleave(u):
    rows16 = pltpu.bitcast(jnp.concatenate(_split(u), axis=0), F32)
    return pltpu.bitcast(rows16.astype(BF16), U32)


@jax.jit
def pallas_interleave_layers__sliding_block_cached__dense_activation_gelu__decode_kernel(
    A_x: jax.Array,
    A_k_cache: jax.Array,
    A_v_cache: jax.Array,
    A_wq: jax.Array,
    A_wo: jax.Array,
    B_x: jax.Array,
    B_w1: jax.Array,
    B_b1: jax.Array,
    B_w2: jax.Array,
    B_b2: jax.Array,
):
    B, SQ, D = A_x.shape
    _, H, SK, DH = A_k_cache.shape
    FF = B_w1.shape[1]
    assert B == 1 and SQ == 1 and A_wq.shape[1] == H * DH and H % 4 == 0
    W = min(4096, max(256, SK // 4))
    NP = H // 2
    PD = 2 * DH
    NT = W // LANES
    KQ = D // LANES
    KP = PD // LANES
    W2B = [0, FF - 8 * LANES, FF - 4 * LANES, FF - LANES, FF]
    XU = [17, 17, 17, 10, 10, 10, 10, 10, 2, 2, 13, 13, 23, 19, 0, 0]
    XT = [1, 2, 2, 9, 9, 4, 4, 4, 10, 10, 5, 5, 0, 2, 16, 16]
    OPN = [0, 0, 6, 6]
    assert len(XU) == len(XT) == NP and XU[-1] == XU[-2] == 0 and sum(OPN) == NP - 4
    XO = [sum(XT[:i]) for i in range(NP)]
    VQ = [3, 6, 7, 8]
    VF = 4
    assert 3 in VQ
    XN = -(-max(XU) // KP)
    CB = LANES // PROWS
    ND = max(OPN + [(NP - 4) // 2])
    PV_BANDS = (4, 2)
    NRING = 2
    exp2_scale = float(DH) ** -0.5 * math.log2(math.e)

    NB = PD // PROWS
    kt = jnp.transpose(A_k_cache, (0, 1, 3, 2)).reshape(NP, NB, 2, ROWS, SK)
    vt = jnp.transpose(A_v_cache, (0, 1, 3, 2)).reshape(NP, NB, 2, ROWS, SK)
    wo3 = A_wo.reshape(NP, PD, D)

    pingpong = dict(
        qp=(((KQ + (len(VQ) + 1) // 2) * ROWS, PD), F32),
        qpk=((ROWS, PD), U32),
        sp=((KP * ROWS, W), F32),
        p=((ROWS, W), F32),
        st=((ROWS, 3 * LANES), F32),
        gl=((PROWS, LANES), F32),
        den=((PROWS, LANES), F32),
        acca=((ROWS, NB * LANES), U32),
        accb=((LANES // 2, PD), U32),
        gpk=((ROWS, (1 + XN) * LANES), U32),
        oraw=(((1 + XN) * PROWS, PD), F32),
        op=((ND * KP * ROWS, D), F32),
    )
    names = list(pingpong)

    def kernel(x_hbm, k_hbm, v_hbm, wq_hbm, wo_hbm, w1_hbm, b1_hbm, w2_hbm, b2_hbm,
               o_ref,
               kbuf, vbuf, wqbuf, wobuf, w1buf, w2buf, xnpk, att, opk, scale, vlo, xcol, sems, cut, *pp):
        q2pk = opk.at[NP - 1]
        xbuf, b1buf, b2buf = pp[-3:]
        bufs = {n: (pp[2 * k], pp[2 * k + 1]) for k, n in enumerate(names)}
        qp, qpk, sp, p, st, gl, den, acca, accb, gpk, oraw, op = (bufs[n] for n in names)
        kb = kbuf.bitcast(BF16)
        vb = vbuf.bitcast(BF16)
        wqb = wqbuf.bitcast(BF16)
        wob = wobuf.bitcast(BF16)
        w1b = w1buf.bitcast(BF16)
        w2b = w2buf.bitcast(BF16)

        S_A, S_B, S_RING = 0, 1, 2

        def window_copies(hbm, buf, start, n, sem):
            return [pltpu.make_async_copy(
                hbm.at[pl.ds(start, n), :, h, :, pl.ds(SK - W, W)],
                buf.at[pl.ds(start, n), :, pl.ds(h * ROWS, ROWS), :], sem) for h in range(2)]

        def group_copies(j, with_k):
            sem = sems.at[S_RING + j % NRING]
            return ((window_copies(k_hbm, kb, j + 2, 1, sem) if with_k else [])
                    + window_copies(v_hbm, vb, j, 1, sem))

        small = [pltpu.make_async_copy(x_hbm, xbuf, sems.at[S_A]),
                 pltpu.make_async_copy(b1_hbm, b1buf, sems.at[S_A]),
                 pltpu.make_async_copy(b2_hbm, b2buf, sems.at[S_A])]
        wq_cps = [pltpu.make_async_copy(wq_hbm.at[:, i * PD:(i + 1) * PD], wqb.at[i], sems.at[S_A])
                  for i in range(NP)]
        k0_cps = window_copies(k_hbm, kb, 0, 2, sems.at[S_B])
        wo_cp = pltpu.make_async_copy(wo_hbm, wob, sems.at[S_B])
        w1_cp = pltpu.make_async_copy(w1_hbm, w1b, sems.at[S_A])
        w2_cps = [pltpu.make_async_copy(w2_hbm.at[W2B[c]:W2B[c + 1]], w2b.at[W2B[c]:W2B[c + 1]],
                                        sems.at[sem])
                  for c, sem in enumerate((S_B, S_RING + NP % NRING, S_RING + (NP + 1) % NRING, S_A))]

        for cp in wq_cps:
            cp.start()
        for cp in small:
            cp.start()
        for cp in k0_cps:
            cp.start()
        wo_cp.start()
        for j in range(NRING):
            for cp in group_copies(j, True):
                cp.start()

        row_id = lax.broadcasted_iota(jnp.int32, (ROWS, PD), 0)
        col = lax.broadcasted_iota(jnp.int32, (ROWS, PD), 1)
        first_head = col < DH
        diag = jnp.where(first_head, 0, 1) == row_id

        def tile(t):
            return slice(t * LANES, (t + 1) * LANES)

        def rows(t):
            return slice(t * ROWS, (t + 1) * ROWS)

        def mm(a, b_):
            return jnp.dot(a, b_, preferred_element_type=F32)[0:ROWS]

        def q_proj(i, b):
            for c in range(KQ):
                qp[b][rows(c)] = mm(_unpack(xnpk[:, tile(c)]), wqb[i, tile(c), :])

        def qk(i, b, cs=range(KP), q_ref=None):
            q_ref = qpk[b] if q_ref is None else q_ref
            for c in cs:
                sp[b][rows(c)] = mm(_unpack(q_ref[:, tile(c)]), kb[i, rows(c)].reshape(LANES, W))

        def columns(xpk):
            return pltpu.bitcast(jnp.concatenate([_unpack(xpk)] * CB, axis=0).T, U32)

        def nt(a, b_):
            return lax.dot_general(a, b_, NT_DIMS, preferred_element_type=F32)

        def packed_acc(b):
            return _unpack(jnp.concatenate([acca[b][:, tile(k)] for k in range(NB)], axis=0))

        def combine_parts(i, b, xu, transposed=True):
            g = _unpack(gpk[b][:, tile(0)])
            parts = [jnp.dot(g, _unpack(accb[b][...]), preferred_element_type=F32) if transposed
                     else nt(g, packed_acc(b))]
            for t in range(-(-xu // KP)):
                w = jnp.concatenate([vbuf[i, c * CB:(c + 1) * CB, :, tile(t)].reshape(LANES // 2, LANES)
                                     for c in range(min(KP, xu - t * KP))], axis=1)
                parts.append(jnp.dot(_unpack(gpk[b][:, tile(1 + t)]), _unpack(w),
                                     preferred_element_type=F32))
            return parts

        def combine(i, b, xu):
            for k, part in enumerate(combine_parts(i, b, xu)):
                oraw[b][k * PROWS:(k + 1) * PROWS, 0:part.shape[1]] = part

        def o_proj(i0, n, b):
            for k in range(n):
                for c in range(KP):
                    op[b][rows(k * KP + c)] = mm(_unpack(opk[i0 + k, :, tile(c)]), wob[i0 + k, tile(c), :])

        def row_max(b):
            st[b][:, tile(2)] = jnp.broadcast_to(
                jnp.max(st[b][:, tile(0)], axis=1, keepdims=True), (ROWS, LANES))

        def row_sum(b):
            return jnp.broadcast_to(jnp.sum(gl[b][...], axis=1, keepdims=True), (PROWS, LANES))

        def sum_rows(ref, n, cols=slice(None), off=0):
            s = ref[rows(off), cols]
            for c in range(1, n):
                s = s + ref[rows(off + c), cols]
            return s

        def q_pack(b):
            qpk[b][...] = _pack(jnp.where(diag, sum_rows(qp[b], KQ), 0.0))

        def row(ref, r, cols=slice(None)):
            v = ref[r:r + 1, cols]
            return jnp.broadcast_to(v, (ROWS, v.shape[1]))

        def lane_weights(b, xu):
            g = []
            for r in range(2):
                g.append(_round_bf16(jnp.exp2((row(st[b], r, tile(0)) - row(st[b], r, tile(2))) * scale[...])))
                gl[b][rows(r)] = g[r] * row(st[b], r, tile(1))
            gpk[b][:, tile(0)] = _pack(g[0], g[1])
            for t in range(-(-xu // KP)):
                gpk[b][:, tile(1 + t)] = _pack(g[0] * row(p[b], 0, tile(t)), g[1] * row(p[b], 1, tile(t)))

        def normalise(parts, dn):
            o = parts[0]
            for part in parts[1:]:
                n = part.shape[1]
                o = o + part if n == PD else jnp.concatenate([o[:, :n] + part, o[:, n:]], axis=1)
            o = o * jnp.concatenate([1.0 / dn] * KP, axis=1)
            o = jnp.where(first_head, o[0:ROWS], o[ROWS:PROWS])
            return _pack(o, o)

        def column_pairs(xpk):
            out = []
            for c in range(xpk.shape[1] // LANES):
                ce, co = (pltpu.bitcast(v, F32) for v in _split(columns(xpk[:, tile(c)])))
                out += [(ce[rows(r)], co[rows(r)]) for r in range(CB)]
            return out

        def vector_matvec(cols, w_ref):
            acc = None
            for band, (ce, co) in enumerate(cols):
                we, wo_ = (pltpu.bitcast(v, F32) for v in _split(w_ref[rows(band), :]))
                reps = we.shape[1] // LANES
                term = (we * jnp.concatenate([ce] * reps, axis=1)
                        + wo_ * jnp.concatenate([co] * reps, axis=1))
                acc = term if acc is None else acc + term
            return jnp.broadcast_to(jnp.sum(acc, axis=0, keepdims=True), acc.shape)

        def vector_q(items, other=iter(())):
            acc = {}
            for band in range(D // PROWS):
                next(other, None)
                ce, co = (jnp.concatenate([pltpu.bitcast(v, F32)] * KP, axis=1)
                          for v in _split(xcol[rows(band)]))
                for i in items:
                    we, wo_ = (pltpu.bitcast(v, F32) for v in _split(wqbuf[i, rows(band)]))
                    term = we * ce + wo_ * co
                    acc[i] = term if band == 0 else acc[i] + term
            return acc

        def vector_q_slot(i):
            k = VQ.index(i)
            return qp[k % 2], (KQ + k // 2) * ROWS

        def vector_q_pack(i, b):
            ref, r0 = vector_q_slot(i)
            q = []
            for c in range(KP):
                q.append(row(ref, r0, tile(c)))
                for r in range(1, ROWS):
                    q[c] = q[c] + row(ref, r0 + r, tile(c))
            qpk[b][...] = _pack(jnp.where(diag, jnp.concatenate(q, axis=1), 0.0))

        def stored_parts(b, xu):
            return [oraw[b][k * PROWS:(k + 1) * PROWS, 0:min(KP, xu - (k - 1) * KP) * LANES]
                    for k in range(1 - (-xu // KP))]

        def o_pack(i, b, xu):
            opk[i] = normalise(stored_parts(b, xu), den[b][...])

        def softmax_steps(b):
            NC = 4

            def tree(f, xs):
                while len(xs) > 1:
                    xs = [f(xs[k], xs[k + 1]) for k in range(0, len(xs), 2)]
                return xs[0]

            mc = [None] * NC
            for t in range(NT):
                s = sum_rows(sp[b], KP, tile(t))
                sp[b][rows(0), tile(t)] = s
                mc[t % NC] = s if t < NC else jnp.maximum(mc[t % NC], s)
                yield
            mm_ = tree(jnp.maximum, mc)
            st[b][:, tile(0)] = mm_
            lc = [None] * NC
            sc = scale[...]
            for t in range(NT):
                e = jnp.exp2((sp[b][rows(0), tile(t)] - mm_) * sc)
                p[b][:, tile(t)] = e
                lc[t % NC] = e if t < NC else lc[t % NC] + e
                if t == NT - 1:
                    st[b][:, tile(1)] = tree(jnp.add, lc)
                yield

        def pv_tiles(xu, nbands):
            return [(h, b0, range(len(range(b0 // CB, xu, KP)), NT))
                    for h in range(2) for b0 in range(h * NB // 2, (h + 1) * NB // 2, nbands)]

        def pv_steps(i, b, xu, xt, xo, nbands, gb):
            for h, b0, tiles in pv_tiles(xu, nbands):
                npk = len(tiles) - xt
                order = sorted(tiles, key=lambda t: ((t - tiles[0] + 0.5) / npk if t < NT - xt
                                                     else (t - (NT - xt) + 0.5) / xt))
                groups = range(b0, b0 + nbands, gb)
                acc = {}
                for pos, t in enumerate(order):
                    pb = p[b][h:h + 1, tile(t)]
                    for g0 in groups:
                        u = vbuf[i, g0:g0 + gb, :, tile(t)]
                        if t < NT - xt:
                            lo, hi = _split(u)
                        else:
                            lo, hi = vlo[xo + NT - 1 - t, g0:g0 + gb], u
                        term = pltpu.bitcast(jnp.concatenate([lo, hi], axis=1), F32) * pb
                        acc[g0] = term if pos == 0 else acc[g0] + term
                        if pos == len(order) - 1:
                            for k in range(gb):
                                acca[b][:, tile(g0 + k)] = pltpu.bitcast(acc[g0][k].astype(BF16), U32)
                    yield

        def rewrite_v(i):
            def lookup(table):
                if isinstance(i, int):
                    return table[i]
                v = jnp.int32(table[0])
                for k in range(1, NP):
                    v = jnp.where(i == k, table[k], v)
                return v

            xo = lookup(XO)

            def transpose(u_, carry):
                blk = (i, pl.ds(pl.multiple_of(u_ % KP * CB, CB), CB), slice(None),
                       pl.ds(pl.multiple_of(u_ // KP * LANES, LANES), LANES))
                v32 = pltpu.bitcast(jnp.concatenate(_split(vbuf[blk]), axis=1), F32)
                w = pltpu.bitcast(v32.reshape(LANES, LANES).astype(BF16).T, U32)
                vbuf[blk] = w.reshape(CB, ROWS, LANES)
                return carry

            def unpack(k, carry):
                blk = (i, slice(None), slice(None),
                       pl.ds(pl.multiple_of((NT - 1 - k) * LANES, LANES), LANES))
                lo, hi = _split(vbuf[blk])
                vbuf[blk] = hi
                vlo[xo + k] = lo
                return carry

            lax.fori_loop(0, lookup(XU), transpose, 0)
            lax.fori_loop(0, lookup(XT), unpack, 0)

        def step(j, b, first):
            nb = 1 - b
            static = isinstance(j, int)

            def live(i):
                return not static or 0 <= i < NP

            def at(i):
                return i if static else jnp.clip(i, 0, NP - 1)

            def xu(i):
                return 0 if first or not live(i) else XU[i]

            opn = [0, 0, (NP - 4) // 2, (NP - 4) // 2] if first else OPN
            ops = {NP - 4 + k: (sum(opn[:k]), n) for k, n in enumerate(opn) if n}
            extra = []
            if live(j - 1):
                extra.append(lambda: lane_weights(nb, xu(j - 1)))
            if live(j - 3):
                extra.append(lambda: o_pack(at(j - 3), nb, xu(j - 3)))
            if live(j + 3):
                extra.append(lambda: q_pack(nb) if first or j + 3 not in VQ
                             else vector_q_pack(j + 3, nb))
            if static and j - 1 in ops:
                i0, n = ops[j - 1]
                for k in range(n):
                    def acc_op(k=k):
                        s_ = sum_rows(op[nb], KP, off=k * KP)
                        att[...] = s_ if i0 + k == 0 else att[...] + s_
                    extra.append(acc_op)
            if live(j + 1):
                sm = softmax_steps(nb)
                assert NT > 6
                short, extra = extra, [lambda: next(sm)] * (2 * NT)
                for k, f in enumerate(short):
                    extra.insert(6 + 5 * k, f)
            extra = [lambda: None] * 3 + extra
            xt, xo, nbands, gb = (0, 0, NB // 2, NB // 4) if first else (XT[j], XO[j], *PV_BANDS)
            nsteps = sum(len(tiles) for _, _, tiles in pv_tiles(xu(j), nbands))
            done = 0
            for k, _ in enumerate(pv_steps(j, b, xu(j), xt, xo, nbands, gb)):
                upto = (k + 1) * len(extra) // nsteps
                for f in extra[done:upto]:
                    f()
                done = upto
            if live(j + 2):
                qk(j + 2, b, q_ref=q2pk if not first and j == 0 else None)
            if live(j - 2):
                combine(at(j - 2), b, xu(j - 2))
            if live(j + 4) and (first or j + 4 not in VQ):
                q_proj(at(j + 4), b)
            if static and j in ops:
                o_proj(*ops[j], b)
            if live(j - 1):
                accb[nb][...] = pltpu.bitcast(packed_acc(nb).T, U32)
            row_max(b)
            if live(j - 2):
                den[b][...] = row_sum(b)

        def attention(x, first):
            mean, rstd = _ln_stats(x)
            xnpk[...] = _pack(x - mean, x - mean)
            scale[...] = jnp.broadcast_to(rstd * exp2_scale, (ROWS, LANES))
            if first:
                for ref in (gpk[0].at[:, tile(0)], accb[0], acca[1], oraw[1].at[0:PROWS]):
                    ref[...] = jnp.zeros(ref.shape, ref.dtype)
                for ref in (st[1], gl[0], den[1]):
                    ref[...] = jnp.ones(ref.shape, ref.dtype)
            qpk[0][...] = _pack(jnp.where(diag, _centered_dot(x, mean, wqb[0]), 0.0))
            if first:
                for cp in k0_cps + [wo_cp]:
                    cp.wait()
                qk(0, 0)
                q_proj(1, 1)
                q_pack(1)
                qk(1, 1)
                q_proj(2, 0)
                q_pack(0)
                q_proj(3, 1)
                for _ in softmax_steps(0):
                    pass

                def reorder_wo(i, carry):
                    for band in range(NB):
                        wobuf[i, rows(band)] = _deinterleave(wobuf[i, rows(band)])
                    return carry
                lax.fori_loop(0, NP, reorder_wo, 0)
            else:
                qpk[1][...] = _pack(jnp.where(diag, _centered_dot(x, mean, wqb[1]), 0.0))
                for c in range(KQ):
                    xcol[c * LANES // 2:(c + 1) * LANES // 2] = columns(xnpk[:, tile(c)])
                qk(0, 0)
                q = jnp.sum(vector_q([2])[2], axis=0, keepdims=True)
                q2pk[...] = _pack(jnp.where(diag, jnp.broadcast_to(q, (ROWS, PD)), 0.0))
                pl.semaphore_signal(cut, 1)
                sm = softmax_steps(0)
                for k in range(0, len(VQ), 2):
                    for i, acc in vector_q(VQ[k:k + 2], sm).items():
                        ref, r0 = vector_q_slot(i)
                        ref[r0:r0 + ROWS] = acc
                for _ in sm:
                    pass
                qk(1, 1)

            def stream(j):
                if isinstance(j, int):
                    for cp in group_copies(j, False):
                        cp.wait()
                    w2_cps[j - (NP - 3)].start()
                    return
                for cp in group_copies(j, True):
                    cp.wait()

                @pl.when(j + NRING < NP - 2)
                def _():
                    for cp in group_copies(j + NRING, True):
                        cp.start()

                @pl.when(jnp.logical_and(j + NRING >= NP - 2, j + NRING < NP))
                def _():
                    for cp in group_copies(j + NRING, False):
                        cp.start()

                @pl.when(j + NRING == NP - 1)
                def _():
                    w1_cp.start()
                    w2_cps[0].start()

            if first:
                def run(j, b, always):
                    stream(j)

                    @pl.when(always)
                    def _():
                        step(j, b, first)
                    rewrite_v(j)

                def body(_, j):
                    for b in range(2):
                        run(j + b, b, ((j + b) & 1) == b)
                    return j + 2
                j_end = lax.fori_loop(0, NP // 2 - 1, body, 0)
                for b in range(2):
                    run(NP - 2 + b, b, j_end + b == NP - 2 + b)
            else:
                for j in range(NP):
                    pl.semaphore_signal(cut, 1)
                    step(j, j % 2, first)
                pl.semaphore_wait(cut, NP + 1)

            lane_weights(1, 0)
            o2 = combine_parts(NP - 2, 0, 0)
            o1 = combine_parts(NP - 1, 1, 0, transposed=False)
            n_last = (NP - 4) // 2 if first else OPN[-1]
            a = x + att[...] + sum_rows(op[1], n_last * KP)
            a = a + vector_matvec(column_pairs(opk[NP - 4]), wobuf.at[NP - 4])
            a = a + mm(_unpack(normalise(stored_parts(1, 0 if first else XU[NP - 3]), den[1][...])), wob[NP - 3])
            a = a + mm(_unpack(normalise(o2, row_sum(0))), wob[NP - 2])
            a = a + mm(_unpack(normalise(o1, row_sum(1))), wob[NP - 1])
            return _round_bf16(a)

        def ffn(x, first):
            mean, rstd = _ln_stats(x)
            if first:
                w1_cp.wait()
                w2_cps[-1].start()
            b1 = b1buf[...].reshape(1, FF).astype(F32)
            b2 = b2buf[...].reshape(1, D).astype(F32)
            h = _centered_dot(x, mean, w1b[...]) * rstd
            h32 = _gelu_tanh(h + b1)
            h = h32.astype(BF16)
            y = x + b2
            if first:
                bounds = W2B[:-1]
                hv = h32[:, W2B[-2]:]
                cols = column_pairs(_pack(hv, hv))
            else:
                bounds = list(range(VF * LANES, FF + 1, LANES))
                hv = h32[:, 0:VF * LANES]
                y = y + vector_matvec(column_pairs(_pack(hv, hv)), w2buf.at[0:VF * LANES // 2])
            for c in range(len(bounds) - 1):
                if first:
                    w2_cps[c].wait()
                yc = jnp.dot(h[:, bounds[c]:bounds[c + 1]], w2b[bounds[c]:bounds[c + 1], :],
                             preferred_element_type=F32)
                y = y + yc
            if first:
                w2_cps[-1].wait()
                y = y + vector_matvec(cols, w2buf.at[W2B[-2] // 2:FF // 2])
            return _round_bf16(y)

        for cp in wq_cps + small:
            cp.wait()
        x = jnp.broadcast_to(xbuf[0].astype(F32), (ROWS, D))
        for first in (True, False):
            x = attention(x, first)
            x = ffn(x, first)
        o_ref[0] = x[0:1].astype(o_ref.dtype)

    any_spec = pl.BlockSpec(memory_space=pl.ANY)
    return pl.pallas_call(
        kernel,
        out_shape=jax.ShapeDtypeStruct((B, SQ, D), A_x.dtype),
        in_specs=[any_spec] * 9,
        out_specs=pl.BlockSpec(memory_space=pltpu.VMEM),
        scratch_shapes=[
            pltpu.VMEM((NP, NB, ROWS, W), U32),
            pltpu.VMEM((NP, NB, ROWS, W), U32),
            pltpu.VMEM((NP, D // 2, PD), U32),
            pltpu.VMEM((NP, DH, D), U32),
            pltpu.VMEM((D // 2, FF), U32),
            pltpu.VMEM((FF // 2, D), U32),
            pltpu.VMEM((ROWS, D), U32),
            pltpu.VMEM((ROWS, D), F32),
            pltpu.VMEM((NP, ROWS, PD), U32),
            pltpu.VMEM((ROWS, LANES), F32),
            pltpu.VMEM((sum(XT), NB, ROWS, LANES), U32),
            pltpu.VMEM((D // 2, LANES), U32),
            pltpu.SemaphoreType.DMA((2 + NRING,)),
            pltpu.SemaphoreType.REGULAR,
        ] + [pltpu.VMEM(*pingpong[n]) for n in names for _ in range(2)] + [
            pltpu.VMEM((B, SQ, D), BF16),
            pltpu.VMEM((FF,), BF16),
            pltpu.VMEM((D,), BF16),
        ],
        compiler_params=pltpu.CompilerParams(vmem_limit_bytes=2047 * 64 * 1024),
    )(A_x, kt, vt, A_wq, wo3, B_w1, B_b1, B_w2, B_b2)
```
